```python
import jax
import jax.numpy as jnp

def _softmax(x, axis=-1):
    return jax.nn.softmax(x, axis=axis)

def _gelu(x):
    return jax.nn.gelu(x, approximate=True)

def _silu(x):
    return jax.nn.silu(x)

def _sigmoid(x):
    return jax.nn.sigmoid(x)

def _layernorm(x, axis=-1, eps=1e-05):
    m = jnp.mean(x, axis=axis, keepdims=True)
    v = jnp.var(x, axis=axis, keepdims=True)
    return (x - m) / jnp.sqrt(v + eps)

def _scatter_add(tgt, idx, src, axis=0):
    return tgt.at[idx].add(src)

def _segment_sum(src, seg, n):
    return jax.ops.segment_sum(src, seg, n)

class _Rng:

    def __init__(self, key):
        self._k = key

    def _next(self):
        self._k, sub = jax.random.split(self._k)
        return sub

    def normal(self, shape):
        return jax.random.normal(self._next(), shape, dtype=jnp.bfloat16)

    def randint(self, lo, hi, shape):
        return jax.random.randint(self._next(), shape, lo, hi, dtype=jnp.int32)

    def uniform(self, shape, lo=0.0, hi=1.0):
        return jax.random.uniform(self._next(), shape, jnp.bfloat16, lo, hi)

    def permutation(self, n):
        return jax.random.permutation(self._next(), n)
kernel_name = 'concat_heads__memory_aug_recurrent_mem_tr__ssm_conv_s4__prompt'

def setup_inputs():
    _rng = _Rng(jax.random.key(int.from_bytes(__import__("os").urandom(4), "little")))
    _w = lambda a: (lambda t: t.astype(jnp.bfloat16) if jnp.issubdtype(t.dtype, jnp.floating) else t)(jnp.asarray(a))

    def _A_setup():
        B, S, Dm = (1, 2048, 1024)
        H, Dh = (32, 128)
        M, seg = (8, 32)
        seg = min(seg, S)
        S = S // seg * seg
        return {'x': _w((lambda *s: _rng.normal(s) * 0.05)(B, S, Dm)), 'mem0': _w((lambda *s: _rng.normal(s) * 0.05)(B, M, Dm)), 'Wq': _w((lambda *s: _rng.normal(s) * 0.05)(Dm, H, Dh) * Dm ** (-0.5)), 'Wk': _w((lambda *s: _rng.normal(s) * 0.05)(Dm, H, Dh) * Dm ** (-0.5)), 'Wv': _w((lambda *s: _rng.normal(s) * 0.05)(Dm, H, Dh) * Dm ** (-0.5)), 'Wo': _w((lambda *s: _rng.normal(s) * 0.05)(H, Dh, Dm) * (H * Dh) ** (-0.5)), 'seg_len': seg}
    _A_in = _A_setup()

    def _B_setup():
        B, L, D, N = (1, 2048, 1024, 128)
        A_re = -jnp.exp((lambda *s: _rng.normal(s) * 0.05)(D, N))
        A_im = jnp.pi * (lambda *s: _rng.normal(s) * 0.05)(D, N)
        B_re = (lambda *s: _rng.normal(s) * 0.05)(D, N)
        B_im = (lambda *s: _rng.normal(s) * 0.05)(D, N)
        C_re = (lambda *s: _rng.normal(s) * 0.05)(D, N)
        C_im = (lambda *s: _rng.normal(s) * 0.05)(D, N)
        log_dt = (lambda *s: _rng.normal(s) * 0.05)(D) * 0.5 - 4.0
        Dskip = (lambda *s: _rng.normal(s) * 0.05)(D)
        return {'u': _w((lambda *s: _rng.normal(s) * 0.05)(B, L, D)), 'A_re': _w(A_re), 'A_im': _w(A_im), 'B_re': _w(B_re), 'B_im': _w(B_im), 'C_re': _w(C_re), 'C_im': _w(C_im), 'log_dt': _w(log_dt), 'Dskip': _w(Dskip)}
    _B_in = _B_setup()
    return {'A_x': _A_in['x'], 'A_mem0': _A_in['mem0'], 'A_Wq': _A_in['Wq'], 'A_Wk': _A_in['Wk'], 'A_Wv': _A_in['Wv'], 'A_Wo': _A_in['Wo'], 'A_seg_len': _A_in['seg_len'], 'B_u': _B_in['u'], 'B_A_re': _B_in['A_re'], 'B_A_im': _B_in['A_im'], 'B_B_re': _B_in['B_re'], 'B_B_im': _B_in['B_im'], 'B_C_re': _B_in['C_re'], 'B_C_im': _B_in['C_im'], 'B_log_dt': _B_in['log_dt'], 'B_Dskip': _B_in['Dskip']}

def reference(A_x, A_mem0, A_Wq, A_Wk, A_Wv, A_Wo, A_seg_len, B_u, B_A_re, B_A_im, B_B_re, B_B_im, B_C_re, B_C_im, B_log_dt, B_Dskip):

    def _A_ref(x, mem0, Wq, Wk, Wv, Wo, seg_len):
        B, S, Dm = x.shape
        H, Dh = (Wq.shape[1], Wq.shape[2])
        M = mem0.shape[1]
        scale = Dh ** (-0.5)
        n_seg = S // seg_len
        L = M + seg_len
        idx = jnp.arange(L)
        mask = (idx[:, None] < M) | (idx[:, None] >= idx[None, :])
        mem = mem0
        outs = []
        for s in range(n_seg):
            xs = x[:, s * seg_len:(s + 1) * seg_len, :].copy()
            h = jnp.concatenate([mem, xs], axis=1)
            q = jnp.einsum('btd,dhe->bhte', h, Wq)
            k = jnp.einsum('btd,dhe->bhte', h, Wk)
            v = jnp.einsum('btd,dhe->bhte', h, Wv)
            scores = jnp.einsum('bhqe,bhke->bhqk', q, k) * scale
            scores = jnp.where(mask[None, None], scores, -1000000000.0)
            p = _softmax(scores, axis=-1)
            o = jnp.einsum('bhqk,bhke->bhqe', p, v)
            o = jnp.einsum('bhte,hed->btd', o, Wo)
            mem = o[:, :M, :].copy()
            outs.append(o[:, M:, :])
        return jnp.concatenate(outs, axis=1)

    def _B_ref(u, A_re, A_im, B_re, B_im, C_re, C_im, log_dt, Dskip):
        Bsz, L, D = u.shape
        dt = jnp.exp(log_dt)[:, None]
        A = A_re + 1j * A_im
        Bc = B_re + 1j * B_im
        Cc = C_re + 1j * C_im
        logdA = dt * A
        dB = dt * Bc
        l = (lambda x, dt: x.astype(dt))(jnp.arange(L), A_re.dtype)
        P = jnp.exp(logdA[:, :, None] * l[None, None, :])
        K = jnp.einsum('dn,dnl,dn->dl', Cc, P, dB).real
        L2 = 2 * L
        Kp = jnp.pad(K, ((0, 0), (0, L)))
        up = (lambda x, *d: x.transpose(*d))(u, 0, 2, 1)
        up = jnp.pad(up, ((0, 0), (0, 0), (0, L)))
        Kf = (lambda x, axes=(-2, -1): jnp.fft.rfft2(x.astype(jnp.float32), axes=axes))(Kp[:, None, :], axes=(-2, -1))
        Uf = (lambda x, axes=(-2, -1): jnp.fft.rfft2(x.astype(jnp.float32), axes=axes))(up[:, :, None, :], axes=(-2, -1))
        Yf = Uf * Kf[None, :, :, :]
        y = (lambda x, s, axes=(-2, -1): jnp.fft.irfft2(x, s=s, axes=axes).astype(jnp.bfloat16))(Yf, (1, L2), axes=(-2, -1))[:, :, 0, :L]
        y = (lambda x, *d: x.transpose(*d))(y, 0, 2, 1) + u * Dskip[None, None, :]
        return y
    a = _A_ref(A_x, A_mem0, A_Wq, A_Wk, A_Wv, A_Wo, A_seg_len)
    b = _B_ref(B_u, B_A_re, B_A_im, B_B_re, B_B_im, B_C_re, B_C_im, B_log_dt, B_Dskip)
    return jnp.concatenate([a, b], axis=-1)
```

```python
import functools

import jax
import jax.numpy as jnp
from jax import lax
import jax.experimental.pallas as pl
import jax.experimental.pallas.tpu as pltpu

_NN = (((1,), (0,)), ((), ()))
_NT = (((1,), (1,)), ((), ()))
_LANES = 128
_T = 64
_CB = 128
_F32 = jnp.float32
_BF16 = jnp.bfloat16
_U32 = jnp.uint32


def _cmul(ar, ai, br, bi):
    return ar * br - ai * bi, ar * bi + ai * br


def _csqrt(x, y):
    big = jnp.sqrt(0.5 * (jnp.sqrt(x * x + y * y) + jnp.abs(x)))
    small = jnp.where(big > 0, 0.5 * y / big, 0.0)
    pos = x >= 0
    return jnp.where(pos, big, jnp.abs(small)), jnp.where(pos, small, jnp.where(y < 0, -big, big))


def _make_kernel(S, Dm, H, Dh, M, seg, L, D, N):
    n_seg = S // seg
    LA = M + seg
    scale = Dh ** (-0.5)
    NC = L // _T
    NB = D // (2 * _CB)
    SG = 17
    RING = 16
    LAG = 20
    CPI = NC // (2 * _CB // 16)
    SU = _CB + 1
    SW = Dm // 2 + 1
    DC = Dm // NB
    NPOW = 11
    HP = H // 2

    def kernel(x_hbm, mem0_hbm, wq_hbm, wk_hbm, wv_hbm, wo_hbm, u_hbm,
               are_hbm, aim_hbm, bre_hbm, bim_hbm, cre_hbm, cim_hbm, ldt_hbm, dsk_hbm,
               out_hbm,
               x_v, mem0_v, wraw_v, wf_v, wo_v, u_v, par_v, ldt_v, dsk_v, dt_v, dk_v,
               ut_v, yt_v, pr_v, pi_v, aux_v, ob_v,
               h_v, o_v, oa_v,
               sem_par, sem_u, sem_w, sem_wo, sem_x, sem_oa, sem_ob, *ring):
        par_hbm = (are_hbm, aim_hbm, bre_hbm, bim_hbm, cre_hbm, cim_hbm)
        par_cp = [pltpu.make_async_copy(par_hbm[i], par_v.at[i], sem_par.at[i]) for i in range(6)]
        par_cp.append(pltpu.make_async_copy(ldt_hbm, ldt_v, sem_par.at[6]))
        par_cp.append(pltpu.make_async_copy(dsk_hbm, dsk_v, sem_par.at[7]))
        mem_cp = pltpu.make_async_copy(mem0_hbm, mem0_v, sem_par.at[8])
        w_hbm = (wq_hbm, wk_hbm, wv_hbm)

        def u_cp(cb):
            return pltpu.make_async_copy(
                u_hbm.at[:, pl.ds(pl.multiple_of(cb * _CB, _CB), _CB)], u_v.at[cb], sem_u.at[cb])

        def w_cp(t, cb):
            rows = pl.ds(pl.multiple_of(cb * (DC * H), DC * H), DC * H)
            return pltpu.make_async_copy(w_hbm[t].at[rows], wraw_v.at[t, rows], sem_w.at[t * NB + cb])

        def wo_cp(j):
            return pltpu.make_async_copy(wo_hbm.at[:, pl.ds(j * _LANES, _LANES)], wo_v.at[j], sem_wo.at[j])

        def ob_cp(cb):
            return pltpu.make_async_copy(
                ob_v.at[cb], out_hbm.at[:, pl.ds(pl.multiple_of(Dm + cb * _CB, _CB), _CB)], sem_ob)

        x_cp = pltpu.make_async_copy(x_hbm, x_v, sem_x)

        for cp in par_cp:
            cp.start()
        for cb in range(2 * NB):
            u_cp(cb).start()
        for cb in range(NB):
            for t in range(3):
                w_cp(t, cb).start()
        mem_cp.start()
        x_cp.start()
        for j in range(Dm // _LANES):
            wo_cp(j).start()
        for cp in par_cp:
            cp.wait()

        dt_all = jnp.exp(ldt_v[...].astype(_F32)).astype(_BF16).astype(_F32).reshape(1, D)
        dk_all = dsk_v[...].astype(_F32).reshape(1, D)
        for cb in range(2 * NB):
            dt_v[cb] = jnp.broadcast_to(dt_all[:, cb * _CB:(cb + 1) * _CB], (8, _CB))
            dk_v[cb] = jnp.broadcast_to(dk_all[:, cb * _CB:(cb + 1) * _CB], (8, _CB))

        flip8 = 7 - lax.broadcasted_iota(jnp.int32, (8, _LANES), 0)
        lane8 = lax.broadcasted_iota(jnp.int32, (8, _LANES), 1)
        sub8 = lax.broadcasted_iota(jnp.int32, (8, _LANES), 0)
        lo_c = lax.broadcasted_iota(jnp.int32, (NC, _LANES), 1) < _T
        first_c = lax.broadcasted_iota(jnp.int32, (NC, _LANES), 0) == 0
        raw32 = wraw_v.bitcast(_U32)
        s_ring = [(ring[4 * i], ring[4 * i + 1]) for i in range(RING)]
        z_ring = [(ring[4 * i + 2], ring[4 * i + 3]) for i in range(RING)]

        def block(sb, carry):
            for hf in range(2):
                aux_v[0, hf] = jnp.broadcast_to(dt_v[2 * sb + hf][0:1, :], (_CB, _CB)).T
            u_cp(2 * sb).wait()
            u_cp(2 * sb + 1).wait()

            def prepare(g, c):
                hf = g // (_CB // 16)
                g16 = (g % (_CB // 16)) * 16
                r = pl.ds(pl.multiple_of(g16, 16), 16)
                rg = pl.ds(pl.multiple_of(sb * 2 * _CB + g * 16, 16), 16)
                dt = aux_v[0, hf, r, :]
                a = dt * par_v[0, rg, :].astype(_F32)
                b = dt * par_v[1, rg, :].astype(_F32)
                mag = jnp.exp(a)
                l1 = (mag * jnp.cos(b), mag * jnp.sin(b))
                w = _cmul(par_v[4, rg, :].astype(_F32), par_v[5, rg, :].astype(_F32),
                          dt * par_v[2, rg, :].astype(_F32), dt * par_v[3, rg, :].astype(_F32))
                l2 = _cmul(*l1, *l1)
                l4 = _cmul(*l2, *l2)
                l8 = _cmul(*l4, *l4)
                l16 = _cmul(*l8, *l8)
                l32 = _cmul(*l16, *l16)
                l64 = _cmul(*l32, *l32)
                pw = [_csqrt(*_cmul(*w, *l1))]
                pw.append(_cmul(*pw[0], *l1))
                pw += [_cmul(*q, *l2) for q in pw]
                pw += [_cmul(*q, *l4) for q in pw]
                pw += [l8, l16, l32]
                for j in range(NPOW):
                    pr_v[hf, pl.ds(j * SU + g16, 16), :] = pw[j][0]
                    pi_v[hf, pl.ds(j * SU + g16, 16), :] = pw[j][1]
                aux_v[1, hf, r, :] = l64[0]
                aux_v[2, hf, r, :] = l64[1]
                aux_v[3, hf, r, :] = jnp.broadcast_to(jnp.sum(w[0], axis=-1, keepdims=True), (16, N))
                aux_v[4, hf, r, :] = pw[0][0]
                aux_v[5, hf, r, :] = -pw[0][1]
                for k in range(CPI):
                    ck = g * CPI + k
                    rows = pl.ds(pl.multiple_of(ck * _T, _T), _T)
                    fl = []
                    for q in range(2):
                        tile = u_v[2 * sb + q, rows, :].astype(_F32)
                        fl += [jnp.take_along_axis(tile[_T - 8 * (i + 1):_T - 8 * i], flip8, axis=0)
                               for i in range(_T // 8)]
                    ut_v[pl.ds(ck * SU, _CB), :] = jnp.concatenate(fl, axis=0).T
                return c
            lax.fori_loop(0, 2 * _CB // 16, prepare, 0)

            def states(p):
                vr, vi = [], []
                for hf in range(2):
                    ar = [pr_v[hf, pl.ds(p, 8, stride=SU), :]]
                    ai = [pi_v[hf, pl.ds(p, 8, stride=SU), :]]
                    for lvl in range(3):
                        mr = jnp.broadcast_to(pr_v[hf, pl.ds((8 + lvl) * SU + p, 1), :], (8, N))
                        mi = jnp.broadcast_to(pi_v[hf, pl.ds((8 + lvl) * SU + p, 1), :], (8, N))
                        for i in range(len(ar)):
                            nr, ni = _cmul(ar[i], ai[i], mr, mi)
                            ar.append(nr)
                            ai.append(ni)
                    vr += ar
                    vi += ai
                v = jnp.concatenate(
                    [jnp.concatenate(vr, axis=0), jnp.concatenate(vi, axis=0)], axis=1).astype(_BF16)
                uf = ut_v[pl.ds(p, NC, stride=SU), :]
                lhs = jnp.concatenate([jnp.where(lo_c, uf, 0.0), jnp.where(lo_c, 0.0, uf)], axis=0)
                st = lax.dot_general(lhs, v, _NN, preferred_element_type=_F32)
                s_r, s_i = st[:, :N], st[:, N:]
                sr, si = s_ring[(p // 8) % RING]
                for hf in range(2):
                    rows = pl.ds(hf * 8 + p % 8, NC, stride=SG)
                    sr[rows, :] = s_r[hf * NC:(hf + 1) * NC]
                    si[rows, :] = s_i[hf * NC:(hf + 1) * NC]
                return v

            def scan(g):
                sr, si = s_ring[g % RING]
                zr, zi = z_ring[g % RING]
                cat = lambda i: jnp.concatenate([aux_v[i, hf, pl.ds(g * 8, 8), :] for hf in range(2)], axis=0)
                lr, li = cat(1), cat(2)
                zr[0:16, :] = cat(4)
                zi[0:16, :] = cat(5)
                xr = xi = None
                for c in range(1, NC):
                    s_r = sr[pl.ds((c - 1) * SG, 16), :]
                    s_i = si[pl.ds((c - 1) * SG, 16), :]
                    if xr is None:
                        xr, xi = s_r, -s_i
                    else:
                        xr, xi = (xr * lr + s_r) + xi * li, (xi * lr - s_i) - xr * li
                    zr[pl.ds(c * SG, 16), :] = xr
                    zi[pl.ds(c * SG, 16), :] = xi
                    if c % (NC // 8) == NC // 8 - 1:
                        yield

            def inter(p, v):
                zr, zi = z_ring[(p // 8) % RING]
                lhs_r = jnp.concatenate([zr[pl.ds(hf * 8 + p % 8, NC, stride=SG), :] for hf in range(2)], axis=0)
                lhs_i = jnp.concatenate([zi[pl.ds(hf * 8 + p % 8, NC, stride=SG), :] for hf in range(2)], axis=0)
                y = lax.dot_general(jnp.concatenate([lhs_r, lhs_i], axis=1), v, _NT,
                                    preferred_element_type=_F32)
                return jnp.where(lo_c, y[:NC], y[NC:])

            def intra(p, y):
                kk = jnp.broadcast_to(y[0:1, :], (8, _LANES))
                g1 = pltpu.roll(kk, 1, 1, stride=1, stride_axis=0)
                g1 = jnp.where((lane8 & (_T - 1)) > sub8, g1, 0.0)
                g1 = jnp.take_along_axis(g1, flip8, axis=0)
                g0 = jnp.where((lane8 & (_T - 1)) >= 8, pltpu.roll(g1, 8, 1), 0.0)
                top = pltpu.bitcast(jnp.concatenate([g0, g1], axis=0).astype(_BF16), _U32)
                gs = [(i, pltpu.roll(top, 16 * i, 1) if i else top) for i in range(_T // 16 - 1, -1, -1)]
                hs = [jnp.where((lane8 >= 16 * i) & (lane8 < _T), gv, _U32(0)) for i, gv in gs]
                hs += [jnp.where(lane8 >= _T + 16 * i, gv, _U32(0)) for i, gv in gs]
                hk = pltpu.bitcast(jnp.concatenate(hs, axis=0), _BF16)
                rows = pl.ds(p, NC, stride=SU)
                yd = lax.dot_general(ut_v[rows, :], hk, _NN, preferred_element_type=_F32)
                yt_v[rows, :] = jnp.where(first_c, 0.0, y) + yd

            def relayout(t, j):
                src = raw32.at[t, pl.ds(pl.multiple_of(sb * (DC * HP), DC * HP), DC * HP), :]
                for half in range(HP // 8):
                    a = src[pl.ds(j * 2 * HP + half * 8, 8), :]
                    b = src[pl.ds(j * 2 * HP + HP + half * 8, 8), :]
                    even = (a & _U32(0xFFFF)) | (b << 16)
                    odd = (a >> 16) | (b & _U32(0xFFFF0000))
                    j0 = sb * (DC // 2) + j
                    wf_v[t, pl.ds(half * 8 * SW + j0, 8, stride=SW), :] = even
                    wf_v[t, pl.ds((HP + half * 8) * SW + j0, 8, stride=SW), :] = odd

            NG = _CB // 8
            jobs = [(t, j) for t in range(3) for j in range(DC // 2)]
            n_jobs = len(jobs)
            ys = {}
            for g0 in range(0, NG, RING):
                ps = range(g0 * 8, (g0 + RING) * 8)
                vs = {p: states(p) for p in ps}
                scs = [scan(g) for g in range(g0, g0 + RING)]
                for i in range(0, RING, 2):
                    for _ in range(8):
                        next(scs[i])
                        next(scs[i + 1])
                if g0 == 0:
                    for t in range(3):
                        w_cp(t, sb).wait()
                for p in ps:
                    ys[p] = inter(p, vs.pop(p))
                    while jobs and len(jobs) * _CB > (_CB - 1 - p) * n_jobs:
                        relayout(*jobs.pop(0))
                for p in sorted(ys):
                    intra(p, ys.pop(p))

            for hf in range(2):
                dk_v[2 * sb + hf] = dk_v[2 * sb + hf] + aux_v[3, hf].T[0:8]

            def tr_out(g, carry):
                for k in range(8):
                    ck = g * 8 + k
                    rows = pl.ds(pl.multiple_of(ck * _T, _T), _T)
                    y = yt_v[pl.ds(ck * SU, _CB), :].T
                    for q in range(2):
                        skip = u_v[2 * sb + q, rows, :].astype(_F32) * dk_v[2 * sb + q][0:1, :]
                        ob_v[2 * sb + q, rows, :] = (y[q * _T:(q + 1) * _T] + skip).astype(_BF16)
                return carry
            lax.fori_loop(0, NC // 8, tr_out, 0)
            ob_cp(2 * sb).start()
            ob_cp(2 * sb + 1).start()
            return carry
        lax.fori_loop(0, NB, block, 0)

        mem_cp.wait()
        x_cp.wait()
        for j in range(Dm // _LANES):
            wo_cp(j).wait()
        h_v[0:M, :] = mem0_v[...].astype(_F32)
        row = lax.broadcasted_iota(jnp.int32, (LA, LA), 0)
        col = lax.broadcasted_iota(jnp.int32, (LA, LA), 1)
        mask = (row < M) | (row >= col)
        wo32 = wo_v.bitcast(_U32)

        def step(s, carry):
            rows = pl.ds(pl.multiple_of(s * seg, seg), seg)
            h_v[M:LA, :] = x_v[rows, :].astype(_F32)

            def proj(hd):
                h = h_v[...]
                r0 = ((hd % 2) * HP + hd // 2) * SW
                return [lax.dot_general(h, pltpu.bitcast(wf_v[t, pl.ds(r0, Dm // 2), :], _BF16), _NN,
                                        preferred_element_type=_F32) for t in range(3)]

            def probs(q, k):
                sc = lax.dot_general(q, k, _NT, preferred_element_type=_F32) * scale
                sc = jnp.where(mask, sc, -1e9)
                p = jnp.exp(sc - jnp.max(sc, axis=-1, keepdims=True))
                return p * pl.reciprocal(jnp.sum(p, axis=-1, keepdims=True), approx=False)

            qkv, pr = {}, {}
            done = [0, 0]

            def do_q():
                pr[done[0]] = probs(*qkv[done[0]][:2])
                done[0] += 1

            def do_v():
                hd = done[1]
                o_v[:, hd * Dh:(hd + 1) * Dh] = lax.dot_general(
                    pr[hd], qkv[hd][2], _NN, preferred_element_type=_F32)
                done[1] += 1

            for hd in range(H):
                qkv[hd] = proj(hd)
                if done[0] <= hd - 1:
                    do_q()
                if done[1] <= hd - 3:
                    do_v()
            h0, acc = 0, None
            for nh in (H - H // 4, H // 4):
                while done[1] < h0 + nh:
                    if done[0] < H:
                        do_q()
                    do_v()
                o = o_v[:, h0 * Dh:(h0 + nh) * Dh]
                res = []
                for j in range(Dm // _LANES):
                    w = pltpu.bitcast(wo32[j, h0 * Dh // 2:(h0 + nh) * Dh // 2, :], _BF16)
                    res.append(lax.dot_general(o, w, _NN, preferred_element_type=_F32))
                    if done[0] < H:
                        do_q()
                    elif done[1] < H:
                        do_v()
                acc = res if acc is None else [a + b for a, b in zip(acc, res)]
                h0 += nh
            out = jnp.concatenate(acc, axis=1)
            h_v[0:M, :] = out[0:M]
            oa_v[rows, :] = out[M:].astype(_BF16)
            pltpu.make_async_copy(oa_v.at[rows], out_hbm.at[rows, pl.ds(0, Dm)], sem_oa).start()
            return carry
        lax.fori_loop(0, n_seg, step, 0)

        pltpu.make_async_copy(oa_v, out_hbm.at[:, pl.ds(0, Dm)], sem_oa).wait()
        for cb in range(2 * NB):
            ob_cp(cb).wait()

    scratch = [
        pltpu.VMEM((S, Dm), _BF16),
        pltpu.VMEM((M, Dm), _BF16),
        pltpu.VMEM((3, Dm * H, Dh), _BF16),
        pltpu.VMEM((3, H * SW, Dh), _U32),
        pltpu.VMEM((Dm // _LANES, H * Dh, _LANES), _BF16),
        pltpu.VMEM((2 * NB, L, _CB), _BF16),
        pltpu.VMEM((6, D, N), _BF16),
        pltpu.VMEM((D,), _BF16),
        pltpu.VMEM((D,), _BF16),
        pltpu.VMEM((2 * NB, 8, _CB), _F32),
        pltpu.VMEM((2 * NB, 8, _CB), _F32),
        pltpu.VMEM((NC * SU, _LANES), _F32),
        pltpu.VMEM((NC * SU, _LANES), _F32),
        pltpu.VMEM((2, NPOW * SU + 5, N), _F32),
        pltpu.VMEM((2, NPOW * SU + 5, N), _F32),
        pltpu.VMEM((6, 2, _CB, N), _F32),
        pltpu.VMEM((2 * NB, L, _CB), _BF16),
        pltpu.VMEM((LA, Dm), _F32),
        pltpu.VMEM((LA, H * Dh), _F32),
        pltpu.VMEM((S, Dm), _BF16),
        pltpu.SemaphoreType.DMA((9,)),
        pltpu.SemaphoreType.DMA((2 * NB,)),
        pltpu.SemaphoreType.DMA((3 * NB,)),
        pltpu.SemaphoreType.DMA((Dm // _LANES,)),
        pltpu.SemaphoreType.DMA(()),
        pltpu.SemaphoreType.DMA(()),
        pltpu.SemaphoreType.DMA(()),
    ] + [pltpu.VMEM((NC * SG, N), _F32)] * (4 * RING)
    return kernel, scratch


@functools.partial(jax.jit, static_argnames=("A_seg_len",))
def pallas_concat_heads__memory_aug_recurrent_mem_tr__ssm_conv_s4__prompt_kernel(
    A_x: jax.Array,
    A_mem0: jax.Array,
    A_Wq: jax.Array,
    A_Wk: jax.Array,
    A_Wv: jax.Array,
    A_Wo: jax.Array,
    A_seg_len: int,
    B_u: jax.Array,
    B_A_re: jax.Array,
    B_A_im: jax.Array,
    B_B_re: jax.Array,
    B_B_im: jax.Array,
    B_C_re: jax.Array,
    B_C_im: jax.Array,
    B_log_dt: jax.Array,
    B_Dskip: jax.Array,
):
    B, S, Dm = A_x.shape
    H, Dh = A_Wq.shape[1], A_Wq.shape[2]
    M = A_mem0.shape[1]
    seg = int(A_seg_len)
    _, L, D = B_u.shape
    N = B_A_re.shape[1]
    assert B == 1 and S == L and S % seg == 0 and Dh == _LANES and N == _LANES

    kernel, scratch = _make_kernel(S, Dm, H, Dh, M, seg, L, D, N)
    out = pl.pallas_call(
        kernel,
        out_shape=jax.ShapeDtypeStruct((S, Dm + D), _BF16),
        in_specs=[pl.BlockSpec(memory_space=pl.ANY)] * 15,
        out_specs=pl.BlockSpec(memory_space=pl.ANY),
        scratch_shapes=scratch,
        compiler_params=pltpu.CompilerParams(vmem_limit_bytes=120 * 1024 * 1024),
    )(
        A_x.reshape(S, Dm), A_mem0.reshape(M, Dm),
        A_Wq.reshape(Dm * H, Dh), A_Wk.reshape(Dm * H, Dh), A_Wv.reshape(Dm * H, Dh),
        A_Wo.reshape(H * Dh, Dm), B_u.reshape(L, D),
        B_A_re, B_A_im, B_B_re, B_B_im, B_C_re, B_C_im, B_log_dt, B_Dskip,
    )
    return out.reshape(B, S, Dm + D)
```

```python
import functools

import jax
import jax.numpy as jnp
from jax import lax
import jax.experimental.pallas as pl
import jax.experimental.pallas.tpu as pltpu

_NN = (((1,), (0,)), ((), ()))
_NT = (((1,), (1,)), ((), ()))
_LANES = 128
_T = 64
_CB = 128
_F32 = jnp.float32
_BF16 = jnp.bfloat16
_U32 = jnp.uint32


def _cmul(ar, ai, br, bi):
    return ar * br - ai * bi, ar * bi + ai * br


def _csqrt(x, y):
    big = jnp.sqrt(0.5 * (jnp.sqrt(x * x + y * y) + jnp.abs(x)))
    small = jnp.where(big > 0, 0.5 * y / big, 0.0)
    pos = x >= 0
    return jnp.where(pos, big, jnp.abs(small)), jnp.where(pos, small, jnp.where(y < 0, -big, big))


def _make_kernel(S, Dm, H, Dh, M, seg, L, D, N):
    n_seg = S // seg
    LA = M + seg
    scale = Dh ** (-0.5)
    NC = L // _T
    NB = D // (2 * _CB)
    SG = 17
    DC = Dm // NB
    RING = 16
    TPI = 8
    JPI = DC // 2 // (NC // TPI)
    PPI = 4
    XR = 4
    LAG = 20
    CPI = NC // (2 * _CB // 16)
    SU = _CB + 1
    SW = Dm // 2 + 1
    NPOW = 11
    HP = H // 2

    def kernel(x_hbm, mem0_hbm, wq_hbm, wk_hbm, wv_hbm, wo_hbm, u_hbm,
               are_hbm, aim_hbm, bre_hbm, bim_hbm, cre_hbm, cim_hbm, ldt_hbm, dsk_hbm,
               out_hbm,
               x_v, mem0_v, wraw_v, wf_v, wo_v, u_v, par_v, ldt_v, dsk_v, dt_v, dk_v,
               ut_v, yt_v, pr_v, pi_v, aux_v, ob_v,
               h_v, o_v, acc_v, oa_v,
               sem_par, sem_u, sem_w, sem_wo, sem_x, sem_oa, sem_ob, *ring):
        par_hbm = (are_hbm, aim_hbm, bre_hbm, bim_hbm, cre_hbm, cim_hbm)
        par_cp = [pltpu.make_async_copy(par_hbm[i], par_v.at[i], sem_par.at[i]) for i in range(6)]
        par_cp.append(pltpu.make_async_copy(ldt_hbm, ldt_v, sem_par.at[6]))
        par_cp.append(pltpu.make_async_copy(dsk_hbm, dsk_v, sem_par.at[7]))
        mem_cp = pltpu.make_async_copy(mem0_hbm, mem0_v, sem_par.at[8])
        w_hbm = (wq_hbm, wk_hbm, wv_hbm)

        def u_cp(cb):
            return pltpu.make_async_copy(
                u_hbm.at[:, pl.ds(pl.multiple_of(cb * _CB, _CB), _CB)], u_v.at[cb], sem_u.at[cb])

        def w_cp(t, cb):
            rows = pl.ds(pl.multiple_of(cb * (DC * H), DC * H), DC * H)
            return pltpu.make_async_copy(w_hbm[t].at[rows], wraw_v.at[t, rows], sem_w.at[t * NB + cb])

        def wo_cp(j):
            return pltpu.make_async_copy(
                wo_hbm.at[:, pl.ds(pl.multiple_of(j * _LANES, _LANES), _LANES)], wo_v.at[j], sem_wo.at[j])

        def ob_cp(cb):
            return pltpu.make_async_copy(
                ob_v.at[cb], out_hbm.at[:, pl.ds(pl.multiple_of(Dm + cb * _CB, _CB), _CB)], sem_ob)

        def x_cp(s):
            src = pl.ds(pl.multiple_of(jnp.minimum(s, n_seg - 1) * seg, seg), seg)
            return pltpu.make_async_copy(x_hbm.at[src], x_v.at[s % XR], sem_x.at[s % XR])

        for cp in par_cp:
            cp.start()
        u_cp(0).start()
        u_cp(1).start()
        for t in range(3):
            w_cp(t, 0).start()
        for cp in par_cp:
            cp.wait()
        mem_cp.start()
        for s in range(XR - 1):
            x_cp(s).start()

        dt_all = jnp.exp(ldt_v[...].astype(_F32)).astype(_BF16).astype(_F32).reshape(1, D)
        dk_all = dsk_v[...].astype(_F32).reshape(1, D)
        for cb in range(2 * NB):
            dt_v[cb] = jnp.broadcast_to(dt_all[:, cb * _CB:(cb + 1) * _CB], (8, _CB))
            dk_v[cb] = jnp.broadcast_to(dk_all[:, cb * _CB:(cb + 1) * _CB], (8, _CB))

        flip8 = 7 - lax.broadcasted_iota(jnp.int32, (8, _LANES), 0)
        lane8 = lax.broadcasted_iota(jnp.int32, (8, _LANES), 1)
        sub8 = lax.broadcasted_iota(jnp.int32, (8, _LANES), 0)
        lo_c = lax.broadcasted_iota(jnp.int32, (NC, _LANES), 1) < _T
        first_c = lax.broadcasted_iota(jnp.int32, (NC, _LANES), 0) == 0
        raw32 = wraw_v.bitcast(_U32)
        s_ring = [(ring[4 * i], ring[4 * i + 1]) for i in range(RING)]
        z_ring = [(ring[4 * i + 2], ring[4 * i + 3]) for i in range(RING)]

        def block(sb, carry):
            @pl.when(sb < NB - 1)
            def _():
                u_cp(2 * sb + 2).start()
                u_cp(2 * sb + 3).start()
                for t in range(3):
                    w_cp(t, sb + 1).start()

            wo_cp(2 * sb).start()
            wo_cp(2 * sb + 1).start()

            for hf in range(2):
                aux_v[0, hf] = jnp.broadcast_to(dt_v[2 * sb + hf][0:1, :], (_CB, _CB)).T
            u_cp(2 * sb).wait()
            u_cp(2 * sb + 1).wait()

            def prepare1(g):
                hf = g // (_CB // 16)
                g16 = (g % (_CB // 16)) * 16
                r = pl.ds(pl.multiple_of(g16, 16), 16)
                rg = pl.ds(pl.multiple_of(sb * 2 * _CB + g * 16, 16), 16)
                dt = aux_v[0, hf, r, :]
                a = dt * par_v[0, rg, :].astype(_F32)
                b = dt * par_v[1, rg, :].astype(_F32)
                mag = jnp.exp(a)
                l1 = (mag * jnp.cos(b), mag * jnp.sin(b))
                w = _cmul(par_v[4, rg, :].astype(_F32), par_v[5, rg, :].astype(_F32),
                          dt * par_v[2, rg, :].astype(_F32), dt * par_v[3, rg, :].astype(_F32))
                l2 = _cmul(*l1, *l1)
                l4 = _cmul(*l2, *l2)
                l8 = _cmul(*l4, *l4)
                l16 = _cmul(*l8, *l8)
                l32 = _cmul(*l16, *l16)
                l64 = _cmul(*l32, *l32)
                pw = [_csqrt(*_cmul(*w, *l1))]
                pw.append(_cmul(*pw[0], *l1))
                pw += [_cmul(*q, *l2) for q in pw]
                pw += [_cmul(*q, *l4) for q in pw]
                pw += [l8, l16, l32]
                for j in range(NPOW):
                    pr_v[hf, pl.ds(j * SU + g16, 16), :] = pw[j][0]
                    pi_v[hf, pl.ds(j * SU + g16, 16), :] = pw[j][1]
                aux_v[1, hf, r, :] = l64[0]
                aux_v[2, hf, r, :] = l64[1]
                aux_v[3, hf, r, :] = jnp.broadcast_to(jnp.sum(w[0], axis=-1, keepdims=True), (16, N))
                aux_v[4, hf, r, :] = pw[0][0]
                aux_v[5, hf, r, :] = -pw[0][1]
                for k in range(CPI):
                    ck = g * CPI + k
                    rows = pl.ds(pl.multiple_of(ck * _T, _T), _T)
                    fl = []
                    for q in range(2):
                        tile = u_v[2 * sb + q, rows, :].astype(_F32)
                        fl += [jnp.take_along_axis(tile[_T - 8 * (i + 1):_T - 8 * i], flip8, axis=0)
                               for i in range(_T // 8)]
                    ut_v[pl.ds(ck * SU, _CB), :] = jnp.concatenate(fl, axis=0).T

            def prepare(i, c):
                for k in range(PPI):
                    prepare1(i * PPI + k)
                return c
            lax.fori_loop(0, 2 * _CB // 16 // PPI, prepare, 0)

            def states(p):
                vr, vi = [], []
                for hf in range(2):
                    ar = [pr_v[hf, pl.ds(p, 8, stride=SU), :]]
                    ai = [pi_v[hf, pl.ds(p, 8, stride=SU), :]]
                    for lvl in range(3):
                        mr = jnp.broadcast_to(pr_v[hf, pl.ds((8 + lvl) * SU + p, 1), :], (8, N))
                        mi = jnp.broadcast_to(pi_v[hf, pl.ds((8 + lvl) * SU + p, 1), :], (8, N))
                        for i in range(len(ar)):
                            nr, ni = _cmul(ar[i], ai[i], mr, mi)
                            ar.append(nr)
                            ai.append(ni)
                    vr += ar
                    vi += ai
                v = jnp.concatenate(
                    [jnp.concatenate(vr, axis=0), jnp.concatenate(vi, axis=0)], axis=1).astype(_BF16)
                uf = ut_v[pl.ds(p, NC, stride=SU), :]
                lhs = jnp.concatenate([jnp.where(lo_c, uf, 0.0), jnp.where(lo_c, 0.0, uf)], axis=0)
                st = lax.dot_general(lhs, v, _NN, preferred_element_type=_F32)
                s_r, s_i = st[:, :N], st[:, N:]
                sr, si = s_ring[(p // 8) % RING]
                for hf in range(2):
                    rows = pl.ds(hf * 8 + p % 8, NC, stride=SG)
                    sr[rows, :] = s_r[hf * NC:(hf + 1) * NC]
                    si[rows, :] = s_i[hf * NC:(hf + 1) * NC]
                return v

            def scan(g):
                sr, si = s_ring[g % RING]
                zr, zi = z_ring[g % RING]
                cat = lambda i: jnp.concatenate([aux_v[i, hf, pl.ds(g * 8, 8), :] for hf in range(2)], axis=0)
                lr, li = cat(1), cat(2)
                zr[0:16, :] = cat(4)
                zi[0:16, :] = cat(5)
                xr = xi = None
                for c in range(1, NC):
                    s_r = sr[pl.ds((c - 1) * SG, 16), :]
                    s_i = si[pl.ds((c - 1) * SG, 16), :]
                    if xr is None:
                        xr, xi = s_r, -s_i
                    else:
                        xr, xi = (xr * lr + s_r) + xi * li, (xi * lr - s_i) - xr * li
                    zr[pl.ds(c * SG, 16), :] = xr
                    zi[pl.ds(c * SG, 16), :] = xi
                    if c % (NC // 8) == NC // 8 - 1:
                        yield

            def inter(p, v):
                zr, zi = z_ring[(p // 8) % RING]
                lhs_r = jnp.concatenate([zr[pl.ds(hf * 8 + p % 8, NC, stride=SG), :] for hf in range(2)], axis=0)
                lhs_i = jnp.concatenate([zi[pl.ds(hf * 8 + p % 8, NC, stride=SG), :] for hf in range(2)], axis=0)
                y = lax.dot_general(jnp.concatenate([lhs_r, lhs_i], axis=1), v, _NT,
                                    preferred_element_type=_F32)
                return jnp.where(lo_c, y[:NC], y[NC:])

            def intra(p, y):
                kk = jnp.broadcast_to(y[0:1, :], (8, _LANES))
                g1 = pltpu.roll(kk, 1, 1, stride=1, stride_axis=0)
                g1 = jnp.where((lane8 & (_T - 1)) > sub8, g1, 0.0)
                g1 = jnp.take_along_axis(g1, flip8, axis=0)
                g0 = jnp.where((lane8 & (_T - 1)) >= 8, pltpu.roll(g1, 8, 1), 0.0)
                top = pltpu.bitcast(jnp.concatenate([g0, g1], axis=0).astype(_BF16), _U32)
                gs = [(i, pltpu.roll(top, 16 * i, 1) if i else top) for i in range(_T // 16 - 1, -1, -1)]
                hs = [jnp.where((lane8 >= 16 * i) & (lane8 < _T), gv, _U32(0)) for i, gv in gs]
                hs += [jnp.where(lane8 >= _T + 16 * i, gv, _U32(0)) for i, gv in gs]
                hk = pltpu.bitcast(jnp.concatenate(hs, axis=0), _BF16)
                rows = pl.ds(p, NC, stride=SU)
                yd = lax.dot_general(ut_v[rows, :], hk, _NN, preferred_element_type=_F32)
                yt_v[rows, :] = jnp.where(first_c, 0.0, y) + yd

            NG = _CB // 8
            ys = {}
            for g0 in range(0, NG, RING):
                ps = range(g0 * 8, (g0 + RING) * 8)
                vs = {p: states(p) for p in ps}
                scs = [scan(g) for g in range(g0, g0 + RING)]
                for i in range(0, RING, 2):
                    for _ in range(8):
                        next(scs[i])
                        next(scs[i + 1])
                for p in ps:
                    ys[p] = inter(p, vs.pop(p))
                for p in sorted(ys):
                    intra(p, ys.pop(p))

            for hf in range(2):
                dk_v[2 * sb + hf] = dk_v[2 * sb + hf] + aux_v[3, hf].T[0:8]

            for t in range(3):
                w_cp(t, sb).wait()

            def finish(g, carry):
                for k in range(TPI):
                    ck = g * TPI + k
                    rows = pl.ds(pl.multiple_of(ck * _T, _T), _T)
                    y = yt_v[pl.ds(ck * SU, _CB), :].T
                    for q in range(2):
                        skip = u_v[2 * sb + q, rows, :].astype(_F32) * dk_v[2 * sb + q][0:1, :]
                        ob_v[2 * sb + q, rows, :] = (y[q * _T:(q + 1) * _T] + skip).astype(_BF16)
                j0 = sb * (DC // 2) + g * JPI
                for t in range(3):
                    src = raw32.at[t, pl.ds(pl.multiple_of(j0 * H, JPI * H), JPI * H), :]
                    for j in range(JPI):
                        for half in range(HP // 8):
                            a = src[pl.ds(j * H + half * 8, 8), :]
                            b = src[pl.ds(j * H + HP + half * 8, 8), :]
                            even = (a & _U32(0xFFFF)) | (b << 16)
                            odd = (a >> 16) | (b & _U32(0xFFFF0000))
                            wf_v[t, pl.ds(j0 + (half * 8 * SW + j), 8, stride=SW), :] = even
                            wf_v[t, pl.ds(j0 + ((HP + half * 8) * SW + j), 8, stride=SW), :] = odd
                return carry
            lax.fori_loop(0, NC // TPI, finish, 0)
            return carry
        lax.fori_loop(0, NB, block, 0)

        mem_cp.wait()
        for j in range(Dm // _LANES):
            wo_cp(j).wait()
        for cb in range(2 * NB):
            ob_cp(cb).start()
        h_v[0:M, :] = mem0_v[...].astype(_F32)
        row = lax.broadcasted_iota(jnp.int32, (LA, LA), 0)
        col = lax.broadcasted_iota(jnp.int32, (LA, LA), 1)
        mask = (row < M) | (row >= col)
        wo32 = wo_v.bitcast(_U32)

        def step(s, carry):
            rows = pl.ds(pl.multiple_of(s * seg, seg), seg)
            x_cp(s).wait()
            h_v[M:LA, :] = x_v[s % XR].astype(_F32)
            x_cp(s + XR - 1).start()

            def proj(hd):
                h = h_v[...]
                r0 = ((hd % 2) * HP + hd // 2) * SW
                return [lax.dot_general(h, pltpu.bitcast(wf_v[t, pl.ds(r0, Dm // 2), :], _BF16), _NN,
                                        preferred_element_type=_F32) for t in range(3)]

            def probs(q, k):
                sc = lax.dot_general(q, k, _NT, preferred_element_type=_F32) * scale
                sc = jnp.where(mask, sc, -1e9)
                p = jnp.exp(sc - jnp.max(sc, axis=-1, keepdims=True))
                return p / jnp.sum(p, axis=-1, keepdims=True)

            qkv, pr = {}, {}
            done = [0, 0]

            def do_q():
                pr[done[0]] = probs(*qkv[done[0]][:2])
                done[0] += 1

            def do_v():
                hd = done[1]
                o_v[:, hd * Dh:(hd + 1) * Dh] = lax.dot_general(
                    pr[hd], qkv[hd][2], _NN, preferred_element_type=_F32)
                done[1] += 1

            for hd in range(H):
                qkv[hd] = proj(hd)
                if done[0] <= hd - 1:
                    do_q()
                if done[1] <= hd - 3:
                    do_v()
            n1 = H - H // 4
            o = o_v[:, 0:n1 * Dh]
            for j in range(Dm // _LANES):
                w = pltpu.bitcast(wo32[j, 0:n1 * Dh // 2, :], _BF16)
                acc_v[:, j * _LANES:(j + 1) * _LANES] = lax.dot_general(o, w, _NN, preferred_element_type=_F32)
                if done[0] < H:
                    do_q()
                elif done[1] < H and j >= 2:
                    do_v()
            while done[1] < H:
                do_v()
            o = o_v[:, n1 * Dh:]
            for j in range(Dm // _LANES):
                cols = slice(j * _LANES, (j + 1) * _LANES)
                w = pltpu.bitcast(wo32[j, n1 * Dh // 2:, :], _BF16)
                res = lax.dot_general(o, w, _NN, preferred_element_type=_F32) + acc_v[:, cols]
                h_v[0:M, cols] = res[0:M]
                oa_v[rows, cols] = res[M:].astype(_BF16)
            pltpu.make_async_copy(oa_v.at[rows], out_hbm.at[rows, pl.ds(0, Dm)], sem_oa).start()
            return carry
        lax.fori_loop(0, n_seg, step, 0)

        for s in range(n_seg, n_seg + XR - 1):
            x_cp(s).wait()
        pltpu.make_async_copy(oa_v, out_hbm.at[:, pl.ds(0, Dm)], sem_oa).wait()
        for cb in range(2 * NB):
            ob_cp(cb).wait()

    scratch = [
        pltpu.VMEM((XR, seg, Dm), _BF16),
        pltpu.VMEM((M, Dm), _BF16),
        pltpu.VMEM((3, Dm * H, Dh), _BF16),
        pltpu.VMEM((3, H * SW, Dh), _U32),
        pltpu.VMEM((Dm // _LANES, H * Dh, _LANES), _BF16),
        pltpu.VMEM((2 * NB, L, _CB), _BF16),
        pltpu.VMEM((6, D, N), _BF16),
        pltpu.VMEM((D,), _BF16),
        pltpu.VMEM((D,), _BF16),
        pltpu.VMEM((2 * NB, 8, _CB), _F32),
        pltpu.VMEM((2 * NB, 8, _CB), _F32),
        pltpu.VMEM((NC * SU, _LANES), _F32),
        pltpu.VMEM((NC * SU, _LANES), _F32),
        pltpu.VMEM((2, NPOW * SU + 5, N), _F32),
        pltpu.VMEM((2, NPOW * SU + 5, N), _F32),
        pltpu.VMEM((6, 2, _CB, N), _F32),
        pltpu.VMEM((2 * NB, L, _CB), _BF16),
        pltpu.VMEM((LA, Dm), _F32),
        pltpu.VMEM((LA, H * Dh), _F32),
        pltpu.VMEM((LA, Dm), _F32),
        pltpu.VMEM((S, Dm), _BF16),
        pltpu.SemaphoreType.DMA((9,)),
        pltpu.SemaphoreType.DMA((2 * NB,)),
        pltpu.SemaphoreType.DMA((3 * NB,)),
        pltpu.SemaphoreType.DMA((Dm // _LANES,)),
        pltpu.SemaphoreType.DMA((XR,)),
        pltpu.SemaphoreType.DMA(()),
        pltpu.SemaphoreType.DMA(()),
    ] + [pltpu.VMEM((NC * SG, N), _F32)] * (4 * RING)
    return kernel, scratch


@functools.partial(jax.jit, static_argnames=("A_seg_len",))
def pallas_concat_heads__memory_aug_recurrent_mem_tr__ssm_conv_s4__prompt_kernel(
    A_x: jax.Array,
    A_mem0: jax.Array,
    A_Wq: jax.Array,
    A_Wk: jax.Array,
    A_Wv: jax.Array,
    A_Wo: jax.Array,
    A_seg_len: int,
    B_u: jax.Array,
    B_A_re: jax.Array,
    B_A_im: jax.Array,
    B_B_re: jax.Array,
    B_B_im: jax.Array,
    B_C_re: jax.Array,
    B_C_im: jax.Array,
    B_log_dt: jax.Array,
    B_Dskip: jax.Array,
):
    B, S, Dm = A_x.shape
    H, Dh = A_Wq.shape[1], A_Wq.shape[2]
    M = A_mem0.shape[1]
    seg = int(A_seg_len)
    _, L, D = B_u.shape
    N = B_A_re.shape[1]
    assert B == 1 and S == L and S % seg == 0 and Dh == _LANES and N == _LANES

    kernel, scratch = _make_kernel(S, Dm, H, Dh, M, seg, L, D, N)
    out = pl.pallas_call(
        kernel,
        out_shape=jax.ShapeDtypeStruct((S, Dm + D), _BF16),
        in_specs=[pl.BlockSpec(memory_space=pl.ANY)] * 15,
        out_specs=pl.BlockSpec(memory_space=pl.ANY),
        scratch_shapes=scratch,
        compiler_params=pltpu.CompilerParams(vmem_limit_bytes=120 * 1024 * 1024),
    )(
        A_x.reshape(S, Dm), A_mem0.reshape(M, Dm),
        A_Wq.reshape(Dm * H, Dh), A_Wk.reshape(Dm * H, Dh), A_Wv.reshape(Dm * H, Dh),
        A_Wo.reshape(H * Dh, Dm), B_u.reshape(L, D),
        B_A_re, B_A_im, B_B_re, B_B_im, B_C_re, B_C_im, B_log_dt, B_Dskip,
    )
    return out.reshape(B, S, Dm + D)
```

```python
import functools

import jax
import jax.numpy as jnp
from jax import lax
import jax.experimental.pallas as pl
import jax.experimental.pallas.tpu as pltpu

_NN = (((1,), (0,)), ((), ()))
_NT = (((1,), (1,)), ((), ()))
_LANES = 128
_T = 64
_CB = 128
_F32 = jnp.float32
_BF16 = jnp.bfloat16
_U32 = jnp.uint32


def _cmul(ar, ai, br, bi):
    return ar * br - ai * bi, ar * bi + ai * br


def _csqrt(x, y):
    big = jnp.sqrt(0.5 * (jnp.sqrt(x * x + y * y) + jnp.abs(x)))
    small = jnp.where(big > 0, 0.5 * y / big, 0.0)
    pos = x >= 0
    return jnp.where(pos, big, jnp.abs(small)), jnp.where(pos, small, jnp.where(y < 0, -big, big))


def _make_kernel(S, Dm, H, Dh, M, seg, L, D, N):
    n_seg = S // seg
    LA = M + seg
    scale = Dh ** (-0.5)
    NC = L // _T
    NB = D // (2 * _CB)
    SG = 17
    DC = Dm // NB
    RING = 16
    TPI = 8
    JPI = DC // 2 // (NC // TPI)
    PPI = 4
    XR = 4
    LAG = 20
    CPI = NC // (2 * _CB // 16)
    SU = _CB + 1
    SW = Dm // 2 + 1
    NPOW = 11
    HP = H // 2

    def kernel(x_hbm, mem0_hbm, wq_hbm, wk_hbm, wv_hbm, wo_hbm, u_hbm,
               are_hbm, aim_hbm, bre_hbm, bim_hbm, cre_hbm, cim_hbm, ldt_hbm, dsk_hbm,
               out_hbm,
               x_v, mem0_v, wraw_v, wf_v, wo_v, u_v, par_v, ldt_v, dsk_v, dt_v, dk_v,
               ut_v, yt_v, pr_v, pi_v, aux_v, ob_v,
               h_v, o_v, acc_v, oa_v,
               sem_par, sem_u, sem_w, sem_wo, sem_x, sem_oa, sem_ob, *ring):
        par_hbm = (are_hbm, aim_hbm, bre_hbm, bim_hbm, cre_hbm, cim_hbm)
        par_cp = [pltpu.make_async_copy(par_hbm[i], par_v.at[i], sem_par.at[i]) for i in range(6)]
        par_cp.append(pltpu.make_async_copy(ldt_hbm, ldt_v, sem_par.at[6]))
        par_cp.append(pltpu.make_async_copy(dsk_hbm, dsk_v, sem_par.at[7]))
        mem_cp = pltpu.make_async_copy(mem0_hbm, mem0_v, sem_par.at[8])
        w_hbm = (wq_hbm, wk_hbm, wv_hbm)

        def u_cp(cb):
            return pltpu.make_async_copy(
                u_hbm.at[:, pl.ds(pl.multiple_of(cb * _CB, _CB), _CB)], u_v.at[cb], sem_u.at[cb])

        def w_cp(t, cb):
            rows = pl.ds(pl.multiple_of(cb * (DC * H), DC * H), DC * H)
            return pltpu.make_async_copy(w_hbm[t].at[rows], wraw_v.at[t, rows], sem_w.at[t * NB + cb])

        def wo_cp(j):
            return pltpu.make_async_copy(
                wo_hbm.at[:, pl.ds(pl.multiple_of(j * _LANES, _LANES), _LANES)], wo_v.at[j], sem_wo.at[j])

        def ob_cp(cb):
            return pltpu.make_async_copy(
                ob_v.at[cb], out_hbm.at[:, pl.ds(pl.multiple_of(Dm + cb * _CB, _CB), _CB)], sem_ob)

        def x_cp(s):
            src = pl.ds(pl.multiple_of(jnp.minimum(s, n_seg - 1) * seg, seg), seg)
            return pltpu.make_async_copy(x_hbm.at[src], x_v.at[s % XR], sem_x.at[s % XR])

        for cp in par_cp:
            cp.start()
        u_cp(0).start()
        u_cp(1).start()
        for cp in par_cp:
            cp.wait()
        mem_cp.start()
        for s in range(XR - 1):
            x_cp(s).start()

        dt_all = jnp.exp(ldt_v[...].astype(_F32)).astype(_BF16).astype(_F32).reshape(1, D)
        dk_all = dsk_v[...].astype(_F32).reshape(1, D)
        for cb in range(2 * NB):
            dt_v[cb] = jnp.broadcast_to(dt_all[:, cb * _CB:(cb + 1) * _CB], (8, _CB))
            dk_v[cb] = jnp.broadcast_to(dk_all[:, cb * _CB:(cb + 1) * _CB], (8, _CB))

        flip8 = 7 - lax.broadcasted_iota(jnp.int32, (8, _LANES), 0)
        lane8 = lax.broadcasted_iota(jnp.int32, (8, _LANES), 1)
        sub8 = lax.broadcasted_iota(jnp.int32, (8, _LANES), 0)
        lo_c = lax.broadcasted_iota(jnp.int32, (NC, _LANES), 1) < _T
        first_c = lax.broadcasted_iota(jnp.int32, (NC, _LANES), 0) == 0
        raw32 = wraw_v.bitcast(_U32)
        s_ring = [(ring[4 * i], ring[4 * i + 1]) for i in range(RING)]
        z_ring = [(ring[4 * i + 2], ring[4 * i + 3]) for i in range(RING)]

        def block(sb, carry):
            for t in range(3):
                w_cp(t, sb).start()

            @pl.when(sb < NB - 1)
            def _():
                u_cp(2 * sb + 2).start()
                u_cp(2 * sb + 3).start()

            for hf in range(2):
                aux_v[0, hf] = jnp.broadcast_to(dt_v[2 * sb + hf][0:1, :], (_CB, _CB)).T
            u_cp(2 * sb).wait()
            u_cp(2 * sb + 1).wait()

            def prepare1(g):
                hf = g // (_CB // 16)
                g16 = (g % (_CB // 16)) * 16
                r = pl.ds(pl.multiple_of(g16, 16), 16)
                rg = pl.ds(pl.multiple_of(sb * 2 * _CB + g * 16, 16), 16)
                dt = aux_v[0, hf, r, :]
                a = dt * par_v[0, rg, :].astype(_F32)
                b = dt * par_v[1, rg, :].astype(_F32)
                mag = jnp.exp(a)
                l1 = (mag * jnp.cos(b), mag * jnp.sin(b))
                w = _cmul(par_v[4, rg, :].astype(_F32), par_v[5, rg, :].astype(_F32),
                          dt * par_v[2, rg, :].astype(_F32), dt * par_v[3, rg, :].astype(_F32))
                l2 = _cmul(*l1, *l1)
                l4 = _cmul(*l2, *l2)
                l8 = _cmul(*l4, *l4)
                l16 = _cmul(*l8, *l8)
                l32 = _cmul(*l16, *l16)
                l64 = _cmul(*l32, *l32)
                pw = [_csqrt(*_cmul(*w, *l1))]
                pw.append(_cmul(*pw[0], *l1))
                pw += [_cmul(*q, *l2) for q in pw]
                pw += [_cmul(*q, *l4) for q in pw]
                pw += [l8, l16, l32]
                for j in range(NPOW):
                    pr_v[hf, pl.ds(j * SU + g16, 16), :] = pw[j][0]
                    pi_v[hf, pl.ds(j * SU + g16, 16), :] = pw[j][1]
                aux_v[1, hf, r, :] = l64[0]
                aux_v[2, hf, r, :] = l64[1]
                aux_v[3, hf, r, :] = jnp.broadcast_to(jnp.sum(w[0], axis=-1, keepdims=True), (16, N))
                aux_v[4, hf, r, :] = pw[0][0]
                aux_v[5, hf, r, :] = -pw[0][1]
                for k in range(CPI):
                    ck = g * CPI + k
                    rows = pl.ds(pl.multiple_of(ck * _T, _T), _T)
                    fl = []
                    for q in range(2):
                        tile = u_v[2 * sb + q, rows, :].astype(_F32)
                        fl += [jnp.take_along_axis(tile[_T - 8 * (i + 1):_T - 8 * i], flip8, axis=0)
                               for i in range(_T // 8)]
                    ut_v[pl.ds(ck * SU, _CB), :] = jnp.concatenate(fl, axis=0).T

            def prepare(i, c):
                for k in range(PPI):
                    prepare1(i * PPI + k)
                return c
            lax.fori_loop(0, 2 * _CB // 16 // PPI, prepare, 0)

            def states(p):
                vr, vi = [], []
                for hf in range(2):
                    ar = [pr_v[hf, pl.ds(p, 8, stride=SU), :]]
                    ai = [pi_v[hf, pl.ds(p, 8, stride=SU), :]]
                    for lvl in range(3):
                        mr = jnp.broadcast_to(pr_v[hf, pl.ds((8 + lvl) * SU + p, 1), :], (8, N))
                        mi = jnp.broadcast_to(pi_v[hf, pl.ds((8 + lvl) * SU + p, 1), :], (8, N))
                        for i in range(len(ar)):
                            nr, ni = _cmul(ar[i], ai[i], mr, mi)
                            ar.append(nr)
                            ai.append(ni)
                    vr += ar
                    vi += ai
                v = jnp.concatenate(
                    [jnp.concatenate(vr, axis=0), jnp.concatenate(vi, axis=0)], axis=1).astype(_BF16)
                uf = ut_v[pl.ds(p, NC, stride=SU), :]
                lhs = jnp.concatenate([jnp.where(lo_c, uf, 0.0), jnp.where(lo_c, 0.0, uf)], axis=0)
                st = lax.dot_general(lhs, v, _NN, preferred_element_type=_F32)
                s_r, s_i = st[:, :N], st[:, N:]
                sr, si = s_ring[(p // 8) % RING]
                for hf in range(2):
                    rows = pl.ds(hf * 8 + p % 8, NC, stride=SG)
                    sr[rows, :] = s_r[hf * NC:(hf + 1) * NC]
                    si[rows, :] = s_i[hf * NC:(hf + 1) * NC]
                return v

            def scan(g):
                sr, si = s_ring[g % RING]
                zr, zi = z_ring[g % RING]
                cat = lambda i: jnp.concatenate([aux_v[i, hf, pl.ds(g * 8, 8), :] for hf in range(2)], axis=0)
                lr, li = cat(1), cat(2)
                zr[0:16, :] = cat(4)
                zi[0:16, :] = cat(5)
                xr = xi = None
                for c in range(1, NC):
                    s_r = sr[pl.ds((c - 1) * SG, 16), :]
                    s_i = si[pl.ds((c - 1) * SG, 16), :]
                    if xr is None:
                        xr, xi = s_r, -s_i
                    else:
                        xr, xi = (xr * lr + s_r) + xi * li, (xi * lr - s_i) - xr * li
                    zr[pl.ds(c * SG, 16), :] = xr
                    zi[pl.ds(c * SG, 16), :] = xi
                    if c % (NC // 8) == NC // 8 - 1:
                        yield

            def inter(p, v):
                zr, zi = z_ring[(p // 8) % RING]
                lhs_r = jnp.concatenate([zr[pl.ds(hf * 8 + p % 8, NC, stride=SG), :] for hf in range(2)], axis=0)
                lhs_i = jnp.concatenate([zi[pl.ds(hf * 8 + p % 8, NC, stride=SG), :] for hf in range(2)], axis=0)
                y = lax.dot_general(jnp.concatenate([lhs_r, lhs_i], axis=1), v, _NT,
                                    preferred_element_type=_F32)
                return jnp.where(lo_c, y[:NC], y[NC:])

            def intra(p, y):
                kk = jnp.broadcast_to(y[0:1, :], (8, _LANES))
                g1 = pltpu.roll(kk, 1, 1, stride=1, stride_axis=0)
                g1 = jnp.where((lane8 & (_T - 1)) > sub8, g1, 0.0)
                g1 = jnp.take_along_axis(g1, flip8, axis=0)
                g0 = jnp.where((lane8 & (_T - 1)) >= 8, pltpu.roll(g1, 8, 1), 0.0)
                top = pltpu.bitcast(jnp.concatenate([g0, g1], axis=0).astype(_BF16), _U32)
                gs = [(i, pltpu.roll(top, 16 * i, 1) if i else top) for i in range(_T // 16 - 1, -1, -1)]
                hs = [jnp.where((lane8 >= 16 * i) & (lane8 < _T), gv, _U32(0)) for i, gv in gs]
                hs += [jnp.where(lane8 >= _T + 16 * i, gv, _U32(0)) for i, gv in gs]
                hk = pltpu.bitcast(jnp.concatenate(hs, axis=0), _BF16)
                rows = pl.ds(p, NC, stride=SU)
                yd = lax.dot_general(ut_v[rows, :], hk, _NN, preferred_element_type=_F32)
                yt_v[rows, :] = jnp.where(first_c, 0.0, y) + yd

            NG = _CB // 8
            ys = {}
            for g0 in range(0, NG, RING):
                ps = range(g0 * 8, (g0 + RING) * 8)
                vs = {p: states(p) for p in ps}
                scs = [scan(g) for g in range(g0, g0 + RING)]
                for i in range(0, RING, 2):
                    for _ in range(8):
                        next(scs[i])
                        next(scs[i + 1])
                if g0 == 0:
                    wo_cp(2 * sb).start()
                    wo_cp(2 * sb + 1).start()
                for p in ps:
                    ys[p] = inter(p, vs.pop(p))
                for p in sorted(ys):
                    intra(p, ys.pop(p))

            for hf in range(2):
                dk_v[2 * sb + hf] = dk_v[2 * sb + hf] + aux_v[3, hf].T[0:8]

            for t in range(3):
                w_cp(t, sb).wait()

            def finish(g, carry):
                for k in range(TPI):
                    ck = g * TPI + k
                    rows = pl.ds(pl.multiple_of(ck * _T, _T), _T)
                    y = yt_v[pl.ds(ck * SU, _CB), :].T
                    for q in range(2):
                        skip = u_v[2 * sb + q, rows, :].astype(_F32) * dk_v[2 * sb + q][0:1, :]
                        ob_v[2 * sb + q, rows, :] = (y[q * _T:(q + 1) * _T] + skip).astype(_BF16)
                j0 = sb * (DC // 2) + g * JPI
                for t in range(3):
                    src = raw32.at[t, pl.ds(pl.multiple_of(j0 * H, JPI * H), JPI * H), :]
                    for j in range(JPI):
                        for half in range(HP // 8):
                            a = src[pl.ds(j * H + half * 8, 8), :]
                            b = src[pl.ds(j * H + HP + half * 8, 8), :]
                            even = (a & _U32(0xFFFF)) | (b << 16)
                            odd = (a >> 16) | (b & _U32(0xFFFF0000))
                            wf_v[t, pl.ds(j0 + (half * 8 * SW + j), 8, stride=SW), :] = even
                            wf_v[t, pl.ds(j0 + ((HP + half * 8) * SW + j), 8, stride=SW), :] = odd
                return carry
            lax.fori_loop(0, NC // TPI, finish, 0)
            return carry
        lax.fori_loop(0, NB, block, 0)

        mem_cp.wait()
        for j in range(Dm // _LANES):
            wo_cp(j).wait()
        for cb in range(2 * NB):
            ob_cp(cb).start()
        h_v[0:M, :] = mem0_v[...].astype(_F32)
        row = lax.broadcasted_iota(jnp.int32, (LA, LA), 0)
        col = lax.broadcasted_iota(jnp.int32, (LA, LA), 1)
        mask = (row < M) | (row >= col)
        wo32 = wo_v.bitcast(_U32)

        def step(s, carry):
            rows = pl.ds(pl.multiple_of(s * seg, seg), seg)
            x_cp(s).wait()
            h_v[M:LA, :] = x_v[s % XR].astype(_F32)
            x_cp(s + XR - 1).start()

            def proj(hd):
                h = h_v[...]
                r0 = ((hd % 2) * HP + hd // 2) * SW
                return [lax.dot_general(h, pltpu.bitcast(wf_v[t, pl.ds(r0, Dm // 2), :], _BF16), _NN,
                                        preferred_element_type=_F32) for t in range(3)]

            def probs(q, k):
                sc = lax.dot_general(q, k, _NT, preferred_element_type=_F32) * scale
                sc = jnp.where(mask, sc, -1e9)
                p = jnp.exp(sc - jnp.max(sc, axis=-1, keepdims=True))
                return p / jnp.sum(p, axis=-1, keepdims=True)

            qkv, pr = {}, {}
            done = [0, 0]

            def do_q():
                pr[done[0]] = probs(*qkv[done[0]][:2])
                done[0] += 1

            def do_v():
                hd = done[1]
                o_v[:, hd * Dh:(hd + 1) * Dh] = lax.dot_general(
                    pr[hd], qkv[hd][2], _NN, preferred_element_type=_F32)
                done[1] += 1

            for hd in range(H):
                qkv[hd] = proj(hd)
                if done[0] <= hd - 1:
                    do_q()
                if done[1] <= hd - 3:
                    do_v()
            n1 = H - H // 4
            o = o_v[:, 0:n1 * Dh]
            for j in range(Dm // _LANES):
                w = pltpu.bitcast(wo32[j, 0:n1 * Dh // 2, :], _BF16)
                acc_v[:, j * _LANES:(j + 1) * _LANES] = lax.dot_general(o, w, _NN, preferred_element_type=_F32)
                if done[0] < H:
                    do_q()
                elif done[1] < H and j >= 2:
                    do_v()
            while done[1] < H:
                do_v()
            o = o_v[:, n1 * Dh:]
            for j in range(Dm // _LANES):
                cols = slice(j * _LANES, (j + 1) * _LANES)
                w = pltpu.bitcast(wo32[j, n1 * Dh // 2:, :], _BF16)
                res = lax.dot_general(o, w, _NN, preferred_element_type=_F32) + acc_v[:, cols]
                h_v[0:M, cols] = res[0:M]
                oa_v[rows, cols] = res[M:].astype(_BF16)
            pltpu.make_async_copy(oa_v.at[rows], out_hbm.at[rows, pl.ds(0, Dm)], sem_oa).start()
            return carry
        lax.fori_loop(0, n_seg, step, 0)

        for s in range(n_seg, n_seg + XR - 1):
            x_cp(s).wait()
        pltpu.make_async_copy(oa_v, out_hbm.at[:, pl.ds(0, Dm)], sem_oa).wait()
        for cb in range(2 * NB):
            ob_cp(cb).wait()

    scratch = [
        pltpu.VMEM((XR, seg, Dm), _BF16),
        pltpu.VMEM((M, Dm), _BF16),
        pltpu.VMEM((3, Dm * H, Dh), _BF16),
        pltpu.VMEM((3, H * SW, Dh), _U32),
        pltpu.VMEM((Dm // _LANES, H * Dh, _LANES), _BF16),
        pltpu.VMEM((2 * NB, L, _CB), _BF16),
        pltpu.VMEM((6, D, N), _BF16),
        pltpu.VMEM((D,), _BF16),
        pltpu.VMEM((D,), _BF16),
        pltpu.VMEM((2 * NB, 8, _CB), _F32),
        pltpu.VMEM((2 * NB, 8, _CB), _F32),
        pltpu.VMEM((NC * SU, _LANES), _F32),
        pltpu.VMEM((NC * SU, _LANES), _F32),
        pltpu.VMEM((2, NPOW * SU + 5, N), _F32),
        pltpu.VMEM((2, NPOW * SU + 5, N), _F32),
        pltpu.VMEM((6, 2, _CB, N), _F32),
        pltpu.VMEM((2 * NB, L, _CB), _BF16),
        pltpu.VMEM((LA, Dm), _F32),
        pltpu.VMEM((LA, H * Dh), _F32),
        pltpu.VMEM((LA, Dm), _F32),
        pltpu.VMEM((S, Dm), _BF16),
        pltpu.SemaphoreType.DMA((9,)),
        pltpu.SemaphoreType.DMA((2 * NB,)),
        pltpu.SemaphoreType.DMA((3 * NB,)),
        pltpu.SemaphoreType.DMA((Dm // _LANES,)),
        pltpu.SemaphoreType.DMA((XR,)),
        pltpu.SemaphoreType.DMA(()),
        pltpu.SemaphoreType.DMA(()),
    ] + [pltpu.VMEM((NC * SG, N), _F32)] * (4 * RING)
    return kernel, scratch


@functools.partial(jax.jit, static_argnames=("A_seg_len",))
def pallas_concat_heads__memory_aug_recurrent_mem_tr__ssm_conv_s4__prompt_kernel(
    A_x: jax.Array,
    A_mem0: jax.Array,
    A_Wq: jax.Array,
    A_Wk: jax.Array,
    A_Wv: jax.Array,
    A_Wo: jax.Array,
    A_seg_len: int,
    B_u: jax.Array,
    B_A_re: jax.Array,
    B_A_im: jax.Array,
    B_B_re: jax.Array,
    B_B_im: jax.Array,
    B_C_re: jax.Array,
    B_C_im: jax.Array,
    B_log_dt: jax.Array,
    B_Dskip: jax.Array,
):
    B, S, Dm = A_x.shape
    H, Dh = A_Wq.shape[1], A_Wq.shape[2]
    M = A_mem0.shape[1]
    seg = int(A_seg_len)
    _, L, D = B_u.shape
    N = B_A_re.shape[1]
    assert B == 1 and S == L and S % seg == 0 and Dh == _LANES and N == _LANES

    kernel, scratch = _make_kernel(S, Dm, H, Dh, M, seg, L, D, N)
    out = pl.pallas_call(
        kernel,
        out_shape=jax.ShapeDtypeStruct((S, Dm + D), _BF16),
        in_specs=[pl.BlockSpec(memory_space=pl.ANY)] * 15,
        out_specs=pl.BlockSpec(memory_space=pl.ANY),
        scratch_shapes=scratch,
        compiler_params=pltpu.CompilerParams(vmem_limit_bytes=120 * 1024 * 1024),
    )(
        A_x.reshape(S, Dm), A_mem0.reshape(M, Dm),
        A_Wq.reshape(Dm * H, Dh), A_Wk.reshape(Dm * H, Dh), A_Wv.reshape(Dm * H, Dh),
        A_Wo.reshape(H * Dh, Dm), B_u.reshape(L, D),
        B_A_re, B_A_im, B_B_re, B_B_im, B_C_re, B_C_im, B_log_dt, B_Dskip,
    )
    return out.reshape(B, S, Dm + D)
```

```python
import functools

import jax
import jax.numpy as jnp
from jax import lax
import jax.experimental.pallas as pl
import jax.experimental.pallas.tpu as pltpu

_NN = (((1,), (0,)), ((), ()))
_NT = (((1,), (1,)), ((), ()))
_LANES = 128
_T = 64
_CB = 128
_F32 = jnp.float32
_BF16 = jnp.bfloat16
_U32 = jnp.uint32


def _cmul(ar, ai, br, bi):
    return ar * br - ai * bi, ar * bi + ai * br


def _csqrt(x, y):
    big = jnp.sqrt(0.5 * (jnp.sqrt(x * x + y * y) + jnp.abs(x)))
    small = jnp.where(big > 0, 0.5 * y / big, 0.0)
    pos = x >= 0
    return jnp.where(pos, big, jnp.abs(small)), jnp.where(pos, small, jnp.where(y < 0, -big, big))


def _make_kernel(S, Dm, H, Dh, M, seg, L, D, N):
    n_seg = S // seg
    LA = M + seg
    scale = Dh ** (-0.5)
    NC = L // _T
    NB = D // (2 * _CB)
    SG = 17
    DC = Dm // NB
    NG = _CB // 8
    SPC = n_seg // NC
    NP = 4
    XR = 4
    LAG = 24
    SU = _CB + 1
    SW = Dm // 2 + 1
    NPOW = 11
    HP = H // 2

    def kernel(x_hbm, mem0_hbm, wq_hbm, wk_hbm, wv_hbm, wo_hbm, u_hbm,
               are_hbm, aim_hbm, bre_hbm, bim_hbm, cre_hbm, cim_hbm, ldt_hbm, dsk_hbm,
               out_hbm,
               x_v, mem0_v, wraw_v, wf_v, wo_v, u_v, par_v, ldt_v, dsk_v, dt_v, dk_v,
               ut_v, yt_v, ya_v, pr_v, pi_v, aux_v, ob_v,
               h_v, o_v, acc_v, oa_v,
               sem_par, sem_u, sem_w, sem_wo, sem_x, sem_oa, sem_ob, sem_y, *st_v):
        par_hbm = (are_hbm, aim_hbm, bre_hbm, bim_hbm, cre_hbm, cim_hbm)
        par_cp = [pltpu.make_async_copy(par_hbm[i], par_v.at[i], sem_par.at[i]) for i in range(6)]
        par_cp.append(pltpu.make_async_copy(ldt_hbm, ldt_v, sem_par.at[6]))
        par_cp.append(pltpu.make_async_copy(dsk_hbm, dsk_v, sem_par.at[7]))
        mem_cp = pltpu.make_async_copy(mem0_hbm, mem0_v, sem_par.at[8])
        w_hbm = (wq_hbm, wk_hbm, wv_hbm)

        def u_cp(cb):
            return pltpu.make_async_copy(
                u_hbm.at[:, pl.ds(pl.multiple_of(cb * _CB, _CB), _CB)], u_v.at[cb], sem_u.at[cb])

        def w_cp(t, cb):
            rows = pl.ds(pl.multiple_of(cb * (DC * H), DC * H), DC * H)
            return pltpu.make_async_copy(w_hbm[t].at[rows], wraw_v.at[t, rows], sem_w.at[t * NB + cb])

        def wo_cp(j):
            return pltpu.make_async_copy(
                wo_hbm.at[:, pl.ds(pl.multiple_of(j * _LANES, _LANES), _LANES)], wo_v.at[j], sem_wo.at[j])

        def y_cp(sb):
            return pltpu.make_async_copy(yt_v, ya_v.at[sb], sem_y)

        def x_cp(s):
            src = pl.ds(pl.multiple_of(jnp.minimum(s, n_seg - 1) * seg, seg), seg)
            return pltpu.make_async_copy(x_hbm.at[src], x_v.at[s % XR], sem_x.at[s % XR])

        for cp in par_cp:
            cp.start()
        u_cp(0).start()
        u_cp(1).start()
        for cp in par_cp:
            cp.wait()
        mem_cp.start()
        for s in range(XR - 1):
            x_cp(s).start()

        dt_all = jnp.exp(ldt_v[...].astype(_F32)).astype(_BF16).astype(_F32).reshape(1, D)
        dk_all = dsk_v[...].astype(_F32).reshape(1, D)
        for cb in range(2 * NB):
            dt_v[cb] = jnp.broadcast_to(dt_all[:, cb * _CB:(cb + 1) * _CB], (8, _CB))
            dk_v[cb] = jnp.broadcast_to(dk_all[:, cb * _CB:(cb + 1) * _CB], (8, _CB))

        flip8 = 7 - lax.broadcasted_iota(jnp.int32, (8, _LANES), 0)
        lane8 = lax.broadcasted_iota(jnp.int32, (8, _LANES), 1)
        sub8 = lax.broadcasted_iota(jnp.int32, (8, _LANES), 0)
        lo_c = lax.broadcasted_iota(jnp.int32, (NC, _LANES), 1) < _T
        first_c = lax.broadcasted_iota(jnp.int32, (NC, _LANES), 0) == 0
        raw32 = wraw_v.bitcast(_U32)
        s_buf = [(st_v[4 * i], st_v[4 * i + 1]) for i in range(NG)]
        z_buf = [(st_v[4 * i + 2], st_v[4 * i + 3]) for i in range(NG)]

        def discretise(sb, g):
            hf = g // (_CB // 16)
            g16 = (g % (_CB // 16)) * 16
            r = pl.ds(pl.multiple_of(g16, 16), 16)
            rg = pl.ds(pl.multiple_of(sb * 2 * _CB + g * 16, 16), 16)
            dt = aux_v[0, hf, r, :]
            a = dt * par_v[0, rg, :].astype(_F32)
            b = dt * par_v[1, rg, :].astype(_F32)
            mag = jnp.exp(a)
            l1 = (mag * jnp.cos(b), mag * jnp.sin(b))
            w = _cmul(par_v[4, rg, :].astype(_F32), par_v[5, rg, :].astype(_F32),
                      dt * par_v[2, rg, :].astype(_F32), dt * par_v[3, rg, :].astype(_F32))
            l2 = _cmul(*l1, *l1)
            l4 = _cmul(*l2, *l2)
            l8 = _cmul(*l4, *l4)
            l16 = _cmul(*l8, *l8)
            l32 = _cmul(*l16, *l16)
            l64 = _cmul(*l32, *l32)
            pw = [_csqrt(*_cmul(*w, *l1))]
            pw.append(_cmul(*pw[0], *l1))
            pw += [_cmul(*q, *l2) for q in pw]
            pw += [_cmul(*q, *l4) for q in pw]
            pw += [l8, l16, l32]
            for j in range(NPOW):
                pr_v[hf, pl.ds(j * SU + g16, 16), :] = pw[j][0]
                pi_v[hf, pl.ds(j * SU + g16, 16), :] = pw[j][1]
            aux_v[1, hf, r, :] = l64[0]
            aux_v[2, hf, r, :] = l64[1]
            aux_v[3, hf, r, :] = jnp.broadcast_to(jnp.sum(w[0], axis=-1, keepdims=True), (16, N))
            aux_v[4, hf, r, :] = pw[0][0]
            aux_v[5, hf, r, :] = -pw[0][1]

        def load_u(sb, ck):
            rows = pl.ds(pl.multiple_of(ck * _T, _T), _T)
            fl = []
            for q in range(2):
                tile = u_v[2 * sb + q, rows, :].astype(_F32)
                fl += [jnp.take_along_axis(tile[_T - 8 * (i + 1):_T - 8 * i], flip8, axis=0)
                       for i in range(_T // 8)]
            ut_v[pl.ds(ck * SU, _CB), :] = jnp.concatenate(fl, axis=0).T

        def repack(j0, n):
            for t in range(3):
                src = raw32.at[t, pl.ds(pl.multiple_of(j0 * H, n * H), n * H), :]
                for j in range(n):
                    for half in range(HP // 8):
                        a = src[pl.ds(j * H + half * 8, 8), :]
                        b = src[pl.ds(j * H + HP + half * 8, 8), :]
                        even = (a & _U32(0xFFFF)) | (b << 16)
                        odd = (a >> 16) | (b & _U32(0xFFFF0000))
                        wf_v[t, pl.ds(j0 + (half * 8 * SW + j), 8, stride=SW), :] = even
                        wf_v[t, pl.ds(j0 + ((HP + half * 8) * SW + j), 8, stride=SW), :] = odd

        def states(p):
            vr, vi = [], []
            for hf in range(2):
                ar = [pr_v[hf, pl.ds(p, 8, stride=SU), :]]
                ai = [pi_v[hf, pl.ds(p, 8, stride=SU), :]]
                for lvl in range(3):
                    mr = jnp.broadcast_to(pr_v[hf, pl.ds((8 + lvl) * SU + p, 1), :], (8, N))
                    mi = jnp.broadcast_to(pi_v[hf, pl.ds((8 + lvl) * SU + p, 1), :], (8, N))
                    for i in range(len(ar)):
                        nr, ni = _cmul(ar[i], ai[i], mr, mi)
                        ar.append(nr)
                        ai.append(ni)
                vr += ar
                vi += ai
            v = jnp.concatenate(
                [jnp.concatenate(vr, axis=0), jnp.concatenate(vi, axis=0)], axis=1).astype(_BF16)
            uf = ut_v[pl.ds(p, NC, stride=SU), :]
            lhs = jnp.concatenate([jnp.where(lo_c, uf, 0.0), jnp.where(lo_c, 0.0, uf)], axis=0)
            st = lax.dot_general(lhs, v, _NN, preferred_element_type=_F32)
            sr, si = s_buf[p // 8]
            for hf in range(2):
                rows = pl.ds(hf * 8 + p % 8, NC, stride=SG)
                sr[rows, :] = st[hf * NC:(hf + 1) * NC, :N]
                si[rows, :] = st[hf * NC:(hf + 1) * NC, N:]
            return v

        def scan(g):
            sr, si = s_buf[g]
            zr, zi = z_buf[g]
            cat = lambda i: jnp.concatenate([aux_v[i, hf, g * 8:(g + 1) * 8, :] for hf in range(2)], axis=0)
            lr, li = cat(1), cat(2)
            zr[0:16, :] = cat(4)
            zi[0:16, :] = cat(5)
            for c in range(1, NC):
                s_r = sr[pl.ds((c - 1) * SG, 16), :]
                s_i = si[pl.ds((c - 1) * SG, 16), :]
                if c == 1:
                    xr, xi = s_r, -s_i
                else:
                    xr, xi = (xr * lr + s_r) + xi * li, (xi * lr - s_i) - xr * li
                zr[pl.ds(c * SG, 16), :] = xr
                zi[pl.ds(c * SG, 16), :] = xi

        def inter(p, v):
            z = [jnp.concatenate([zb[pl.ds(hf * 8 + p % 8, NC, stride=SG), :] for hf in range(2)], axis=0)
                 for zb in z_buf[p // 8]]
            y = lax.dot_general(jnp.concatenate(z, axis=1), v, _NT, preferred_element_type=_F32)
            return jnp.where(lo_c, y[:NC], y[NC:])

        def intra(p, y):
            kk = jnp.broadcast_to(y[0:1, :], (8, _LANES))
            g1 = pltpu.roll(kk, 1, 1, stride=1, stride_axis=0)
            g1 = jnp.where((lane8 & (_T - 1)) > sub8, g1, 0.0)
            g1 = jnp.take_along_axis(g1, flip8, axis=0)
            g0 = jnp.where((lane8 & (_T - 1)) >= 8, pltpu.roll(g1, 8, 1), 0.0)
            top = pltpu.bitcast(jnp.concatenate([g0, g1], axis=0).astype(_BF16), _U32)
            gs = [(i, pltpu.roll(top, 16 * i, 1) if i else top) for i in range(_T // 16 - 1, -1, -1)]
            hs = [jnp.where((lane8 >= 16 * i) & (lane8 < _T), gv, _U32(0)) for i, gv in gs]
            hs += [jnp.where(lane8 >= _T + 16 * i, gv, _U32(0)) for i, gv in gs]
            hk = pltpu.bitcast(jnp.concatenate(hs, axis=0), _BF16)
            rows = pl.ds(p, NC, stride=SU)
            yd = lax.dot_general(ut_v[rows, :], hk, _NN, preferred_element_type=_F32)
            yt_v[rows, :] = jnp.where(first_c, 0.0, y) + yd

        def block(sb, carry):
            @pl.when(sb > 0)
            def _():
                for t in range(3):
                    w_cp(t, sb - 1).wait()

            for t in range(3):
                w_cp(t, sb).start()

            @pl.when(sb < NB - 1)
            def _():
                u_cp(2 * sb + 2).start()
                u_cp(2 * sb + 3).start()

            for hf in range(2):
                aux_v[0, hf] = jnp.broadcast_to(dt_v[2 * sb + hf][0:1, :], (_CB, _CB)).T
            u_cp(2 * sb).wait()
            u_cp(2 * sb + 1).wait()

            def prepare(i, c, with_repack):
                for k in range(2 * _CB // 16 // NP):
                    discretise(sb, i * (2 * _CB // 16 // NP) + k)
                for k in range(NC // NP):
                    load_u(sb, i * (NC // NP) + k)
                if with_repack:
                    repack((sb - 1) * (DC // 2) + i * (DC // 2 // NP), DC // 2 // NP)
                return c

            @pl.when(sb == 0)
            def _():
                lax.fori_loop(0, NP, functools.partial(prepare, with_repack=False), 0)

            @pl.when(sb > 0)
            def _():
                lax.fori_loop(0, NP, functools.partial(prepare, with_repack=True), 0)
                y_cp(sb - 1).wait()

            for hf in range(2):
                dk_v[2 * sb + hf] = dk_v[2 * sb + hf] + aux_v[3, hf].T[0:8]

            vs, ys = {}, {}
            for p in range(_CB + LAG):
                if p < _CB:
                    vs[p] = states(p)
                    if p % 8 == 7:
                        scan(p // 8)
                if p == _CB // 2:
                    wo_cp(2 * sb).start()
                    wo_cp(2 * sb + 1).start()
                if p >= LAG:
                    ys[p - LAG] = inter(p - LAG, vs.pop(p - LAG))
            for p in range(_CB):
                intra(p, ys.pop(p))
            y_cp(sb).start()
            return carry
        lax.fori_loop(0, NB, block, 0)
        for t in range(3):
            w_cp(t, NB - 1).wait()

        def last_repack(i, c):
            repack((NB - 1) * (DC // 2) + i * (DC // 2 // NP), DC // 2 // NP)
            return c
        lax.fori_loop(0, NP, last_repack, 0)

        mem_cp.wait()
        y_cp(NB - 1).wait()
        for j in range(Dm // _LANES):
            wo_cp(j).wait()
        h_v[0:M, :] = mem0_v[...].astype(_F32)
        row = lax.broadcasted_iota(jnp.int32, (LA, LA), 0)
        col = lax.broadcasted_iota(jnp.int32, (LA, LA), 1)
        mask = (row < M) | (row >= col)
        wo32 = wo_v.bitcast(_U32)

        def step(s, carry):
            rows = pl.ds(pl.multiple_of(s * seg, seg), seg)
            x_cp(s).wait()
            h_v[M:LA, :] = x_v[s % XR].astype(_F32)
            x_cp(s + XR - 1).start()

            def proj(hd):
                h = h_v[...]
                r0 = ((hd % 2) * HP + hd // 2) * SW
                return [lax.dot_general(h, pltpu.bitcast(wf_v[t, pl.ds(r0, Dm // 2), :], _BF16), _NN,
                                        preferred_element_type=_F32) for t in range(3)]

            def probs(q, k):
                sc = lax.dot_general(q, k, _NT, preferred_element_type=_F32) * scale
                sc = jnp.where(mask, sc, -1e9)
                p = jnp.exp(sc - jnp.max(sc, axis=-1, keepdims=True))
                return p / jnp.sum(p, axis=-1, keepdims=True)

            qkv, pr = {}, {}
            done = [0, 0]

            def do_q():
                pr[done[0]] = probs(*qkv[done[0]][:2])
                done[0] += 1

            def do_v():
                hd = done[1]
                o_v[:, hd * Dh:(hd + 1) * Dh] = lax.dot_general(
                    pr[hd], qkv[hd][2], _NN, preferred_element_type=_F32)
                done[1] += 1

            for hd in range(H):
                qkv[hd] = proj(hd)
                if done[0] <= hd - 1:
                    do_q()
                if done[1] <= hd - 3:
                    do_v()
            n1 = H - H // 4
            o = o_v[:, 0:n1 * Dh]
            for j in range(Dm // _LANES):
                w = pltpu.bitcast(wo32[j, 0:n1 * Dh // 2, :], _BF16)
                acc_v[:, j * _LANES:(j + 1) * _LANES] = lax.dot_general(o, w, _NN, preferred_element_type=_F32)
                if done[0] < H:
                    do_q()
                elif done[1] < H and j >= 2:
                    do_v()
            while done[1] < H:
                do_v()
            o = o_v[:, n1 * Dh:]
            for j in range(Dm // _LANES):
                cols = slice(j * _LANES, (j + 1) * _LANES)
                w = pltpu.bitcast(wo32[j, n1 * Dh // 2:, :], _BF16)
                res = lax.dot_general(o, w, _NN, preferred_element_type=_F32) + acc_v[:, cols]
                h_v[0:M, cols] = res[0:M]
                oa_v[rows, cols] = res[M:].astype(_BF16)
            pltpu.make_async_copy(oa_v.at[rows], out_hbm.at[rows, pl.ds(0, Dm)], sem_oa).start()

            ck = s // SPC
            trows = pl.ds(pl.multiple_of(ck * _T, _T), _T)
            c0 = pl.multiple_of((s % SPC) * (D // SPC), D // SPC)
            dst = ob_v.at[trows, pl.ds(c0, D // SPC)]
            for i in range(NB // SPC):
                sb = (s % SPC) * (NB // SPC) + i
                y = ya_v[sb, pl.ds(ck * SU, _CB), :].T
                for q in range(2):
                    skip = u_v[2 * sb + q, trows, :].astype(_F32) * dk_v[2 * sb + q][0:1, :]
                    dst[:, (2 * i + q) * _CB:(2 * i + q + 1) * _CB] = (y[q * _T:(q + 1) * _T] + skip).astype(_BF16)
            pltpu.make_async_copy(dst, out_hbm.at[trows, pl.ds(Dm + c0, D // SPC)], sem_ob).start()
            return carry
        lax.fori_loop(0, n_seg, step, 0)

        for s in range(n_seg, n_seg + XR - 1):
            x_cp(s).wait()
        pltpu.make_async_copy(oa_v, out_hbm.at[:, pl.ds(0, Dm)], sem_oa).wait()
        pltpu.make_async_copy(ob_v, out_hbm.at[:, pl.ds(Dm, D)], sem_ob).wait()

    scratch = [
        pltpu.VMEM((XR, seg, Dm), _BF16),
        pltpu.VMEM((M, Dm), _BF16),
        pltpu.VMEM((3, Dm * H, Dh), _BF16),
        pltpu.VMEM((3, H * SW, Dh), _U32),
        pltpu.VMEM((Dm // _LANES, H * Dh, _LANES), _BF16),
        pltpu.VMEM((2 * NB, L, _CB), _BF16),
        pltpu.VMEM((6, D, N), _BF16),
        pltpu.VMEM((D,), _BF16),
        pltpu.VMEM((D,), _BF16),
        pltpu.VMEM((2 * NB, 8, _CB), _F32),
        pltpu.VMEM((2 * NB, 8, _CB), _F32),
        pltpu.VMEM((NC * SU, _LANES), _F32),
        pltpu.VMEM((NC * SU, _LANES), _F32),
        pltpu.VMEM((NB, NC * SU, _LANES), _F32),
        pltpu.VMEM((2, NPOW * SU + 5, N), _F32),
        pltpu.VMEM((2, NPOW * SU + 5, N), _F32),
        pltpu.VMEM((6, 2, _CB, N), _F32),
        pltpu.VMEM((L, D), _BF16),
        pltpu.VMEM((LA, Dm), _F32),
        pltpu.VMEM((LA, H * Dh), _F32),
        pltpu.VMEM((LA, Dm), _F32),
        pltpu.VMEM((S, Dm), _BF16),
        pltpu.SemaphoreType.DMA((9,)),
        pltpu.SemaphoreType.DMA((2 * NB,)),
        pltpu.SemaphoreType.DMA((3 * NB,)),
        pltpu.SemaphoreType.DMA((Dm // _LANES,)),
        pltpu.SemaphoreType.DMA((XR,)),
        pltpu.SemaphoreType.DMA(()),
        pltpu.SemaphoreType.DMA(()),
        pltpu.SemaphoreType.DMA(()),
    ] + [pltpu.VMEM((NC * SG, N), _F32)] * (4 * NG)
    return kernel, scratch


@functools.partial(jax.jit, static_argnames=("A_seg_len",))
def pallas_concat_heads__memory_aug_recurrent_mem_tr__ssm_conv_s4__prompt_kernel(
    A_x: jax.Array,
    A_mem0: jax.Array,
    A_Wq: jax.Array,
    A_Wk: jax.Array,
    A_Wv: jax.Array,
    A_Wo: jax.Array,
    A_seg_len: int,
    B_u: jax.Array,
    B_A_re: jax.Array,
    B_A_im: jax.Array,
    B_B_re: jax.Array,
    B_B_im: jax.Array,
    B_C_re: jax.Array,
    B_C_im: jax.Array,
    B_log_dt: jax.Array,
    B_Dskip: jax.Array,
):
    B, S, Dm = A_x.shape
    H, Dh = A_Wq.shape[1], A_Wq.shape[2]
    M = A_mem0.shape[1]
    seg = int(A_seg_len)
    _, L, D = B_u.shape
    N = B_A_re.shape[1]
    assert B == 1 and S == L and S % seg == 0 and Dh == _LANES and N == _LANES

    kernel, scratch = _make_kernel(S, Dm, H, Dh, M, seg, L, D, N)
    out = pl.pallas_call(
        kernel,
        out_shape=jax.ShapeDtypeStruct((S, Dm + D), _BF16),
        in_specs=[pl.BlockSpec(memory_space=pl.ANY)] * 15,
        out_specs=pl.BlockSpec(memory_space=pl.ANY),
        scratch_shapes=scratch,
        compiler_params=pltpu.CompilerParams(vmem_limit_bytes=120 * 1024 * 1024),
    )(
        A_x.reshape(S, Dm), A_mem0.reshape(M, Dm),
        A_Wq.reshape(Dm * H, Dh), A_Wk.reshape(Dm * H, Dh), A_Wv.reshape(Dm * H, Dh),
        A_Wo.reshape(H * Dh, Dm), B_u.reshape(L, D),
        B_A_re, B_A_im, B_B_re, B_B_im, B_C_re, B_C_im, B_log_dt, B_Dskip,
    )
    return out.reshape(B, S, Dm + D)
```

```python
import functools

import jax
import jax.numpy as jnp
from jax import lax
import jax.experimental.pallas as pl
import jax.experimental.pallas.tpu as pltpu

_NN = (((1,), (0,)), ((), ()))
_NT = (((1,), (1,)), ((), ()))
_LANES = 128
_T = 64
_CB = 128
_F32 = jnp.float32
_BF16 = jnp.bfloat16
_U32 = jnp.uint32


def _cmul(ar, ai, br, bi):
    return ar * br - ai * bi, ar * bi + ai * br


def _csqrt(x, y):
    big = jnp.sqrt(0.5 * (jnp.sqrt(x * x + y * y) + jnp.abs(x)))
    small = jnp.where(big > 0, 0.5 * y / big, 0.0)
    pos = x >= 0
    return jnp.where(pos, big, jnp.abs(small)), jnp.where(pos, small, jnp.where(y < 0, -big, big))


def _make_kernel(S, Dm, H, Dh, M, seg, L, D, N):
    LA = M + seg
    scale = Dh ** (-0.5)
    NC = L // _T
    NB = D // (2 * _CB)
    SG = 17
    DC = Dm // NB
    NG = _CB // 8
    NP = 4
    XR = 3
    LAG = 24
    SU = _CB + 1
    SW = Dm // 2 + 1
    NPOW = 11
    HP = H // 2

    def kernel(x_hbm, mem0_hbm, wq_hbm, wk_hbm, wv_hbm, wo_hbm, u_hbm,
               are_hbm, aim_hbm, bre_hbm, bim_hbm, cre_hbm, cim_hbm, ldt_hbm, dsk_hbm,
               out_hbm,
               x_v, mem0_v, wraw_v, wf_v, wo_v, u_v, par_v, ldt_v, dsk_v, dt_v, dk_v,
               ut_v, yt_v, ya_v, pr_v, pi_v, aux_v,
               h_v, o_v, acc_v, out_v,
               sem_par, sem_u, sem_w, sem_wo, sem_x, sem_out, sem_y, *st_v):
        par_hbm = (are_hbm, aim_hbm, bre_hbm, bim_hbm, cre_hbm, cim_hbm)
        head, rest = pl.ds(0, 2 * _CB), pl.ds(2 * _CB, D - 2 * _CB)
        par_head = [pltpu.make_async_copy(par_hbm[i].at[head], par_v.at[i, head], sem_par.at[i]) for i in range(6)]
        par_head.append(pltpu.make_async_copy(ldt_hbm, ldt_v, sem_par.at[6]))
        par_head.append(pltpu.make_async_copy(dsk_hbm, dsk_v, sem_par.at[7]))
        par_rest = [pltpu.make_async_copy(par_hbm[i].at[rest], par_v.at[i, rest], sem_par.at[8 + i]) for i in range(6)]
        mem_cp = pltpu.make_async_copy(mem0_hbm, mem0_v, sem_par.at[14])
        w_hbm = (wq_hbm, wk_hbm, wv_hbm)

        def u_cp(cb):
            return pltpu.make_async_copy(
                u_hbm.at[:, pl.ds(pl.multiple_of(cb * _CB, _CB), _CB)], u_v.at[cb], sem_u.at[cb])

        def w_cp(t, cb):
            rows = pl.ds(pl.multiple_of(cb * (DC * H), DC * H), DC * H)
            return pltpu.make_async_copy(w_hbm[t].at[rows], wraw_v.at[t, rows], sem_w.at[t * NB + cb])

        def wo_cp(j):
            return pltpu.make_async_copy(
                wo_hbm.at[:, pl.ds(pl.multiple_of(j * _LANES, _LANES), _LANES)], wo_v.at[j], sem_wo.at[j])

        def y_cp(sb):
            return pltpu.make_async_copy(yt_v, ya_v.at[sb], sem_y)

        def x_cp(i):
            src = pl.ds(pl.multiple_of(jnp.minimum(i, NC - 1) * _T, _T), _T)
            return pltpu.make_async_copy(x_hbm.at[src], x_v.at[i % XR], sem_x.at[i % XR])

        for cp in par_head:
            cp.start()
        u_cp(0).start()
        u_cp(1).start()
        for cp in par_head:
            cp.wait()
        for cp in par_rest:
            cp.start()
        mem_cp.start()
        for i in range(XR - 1):
            x_cp(i).start()

        dt_all = jnp.exp(ldt_v[...].astype(_F32)).astype(_BF16).astype(_F32).reshape(1, D)
        dk_all = dsk_v[...].astype(_F32).reshape(1, D)
        for cb in range(2 * NB):
            dt_v[cb] = jnp.broadcast_to(dt_all[:, cb * _CB:(cb + 1) * _CB], (8, _CB))
            dk_v[cb] = jnp.broadcast_to(dk_all[:, cb * _CB:(cb + 1) * _CB], (8, _CB))

        flip8 = 7 - lax.broadcasted_iota(jnp.int32, (8, _LANES), 0)
        lane8 = lax.broadcasted_iota(jnp.int32, (8, _LANES), 1)
        sub8 = lax.broadcasted_iota(jnp.int32, (8, _LANES), 0)
        lo_c = lax.broadcasted_iota(jnp.int32, (NC, _LANES), 1) < _T
        first_c = lax.broadcasted_iota(jnp.int32, (NC, _LANES), 0) == 0
        raw32 = wraw_v.bitcast(_U32)
        s_buf = [(st_v[4 * i], st_v[4 * i + 1]) for i in range(NG)]
        z_buf = [(st_v[4 * i + 2], st_v[4 * i + 3]) for i in range(NG)]

        def discretise(sb, g):
            hf = g // (_CB // 16)
            g16 = (g % (_CB // 16)) * 16
            r = pl.ds(pl.multiple_of(g16, 16), 16)
            rg = pl.ds(pl.multiple_of(sb * 2 * _CB + g * 16, 16), 16)
            dt = aux_v[0, hf, r, :]
            a = dt * par_v[0, rg, :].astype(_F32)
            b = dt * par_v[1, rg, :].astype(_F32)
            mag = jnp.exp(a)
            l1 = (mag * jnp.cos(b), mag * jnp.sin(b))
            w = _cmul(par_v[4, rg, :].astype(_F32), par_v[5, rg, :].astype(_F32),
                      dt * par_v[2, rg, :].astype(_F32), dt * par_v[3, rg, :].astype(_F32))
            l2 = _cmul(*l1, *l1)
            l4 = _cmul(*l2, *l2)
            l8 = _cmul(*l4, *l4)
            l16 = _cmul(*l8, *l8)
            l32 = _cmul(*l16, *l16)
            l64 = _cmul(*l32, *l32)
            pw = [_csqrt(*_cmul(*w, *l1))]
            pw.append(_cmul(*pw[0], *l1))
            pw += [_cmul(*q, *l2) for q in pw]
            pw += [_cmul(*q, *l4) for q in pw]
            pw += [l8, l16, l32]
            for j in range(NPOW):
                pr_v[hf, pl.ds(j * SU + g16, 16), :] = pw[j][0]
                pi_v[hf, pl.ds(j * SU + g16, 16), :] = pw[j][1]
            aux_v[1, hf, r, :] = l64[0]
            aux_v[2, hf, r, :] = l64[1]
            aux_v[3, hf, r, :] = jnp.broadcast_to(jnp.sum(w[0], axis=-1, keepdims=True), (16, N))
            aux_v[4, hf, r, :] = pw[0][0]
            aux_v[5, hf, r, :] = -pw[0][1]

        def load_u(sb, ck):
            rows = pl.ds(pl.multiple_of(ck * _T, _T), _T)
            fl = []
            for q in range(2):
                tile = u_v[2 * sb + q, rows, :].astype(_F32)
                fl += [jnp.take_along_axis(tile[_T - 8 * (i + 1):_T - 8 * i], flip8, axis=0)
                       for i in range(_T // 8)]
            ut_v[pl.ds(ck * SU, _CB), :] = jnp.concatenate(fl, axis=0).T

        def repack(j0, n):
            for t in range(3):
                src = raw32.at[t, pl.ds(pl.multiple_of(j0 * H, n * H), n * H), :]
                for j in range(n):
                    for half in range(HP // 8):
                        a = src[pl.ds(j * H + half * 8, 8), :]
                        b = src[pl.ds(j * H + HP + half * 8, 8), :]
                        even = (a & _U32(0xFFFF)) | (b << 16)
                        odd = (a >> 16) | (b & _U32(0xFFFF0000))
                        wf_v[t, pl.ds(j0 + (half * 8 * SW + j), 8, stride=SW), :] = even
                        wf_v[t, pl.ds(j0 + ((HP + half * 8) * SW + j), 8, stride=SW), :] = odd

        def states(p):
            vr, vi = [], []
            for hf in range(2):
                ar = [pr_v[hf, pl.ds(p, 8, stride=SU), :]]
                ai = [pi_v[hf, pl.ds(p, 8, stride=SU), :]]
                for lvl in range(3):
                    mr = jnp.broadcast_to(pr_v[hf, pl.ds((8 + lvl) * SU + p, 1), :], (8, N))
                    mi = jnp.broadcast_to(pi_v[hf, pl.ds((8 + lvl) * SU + p, 1), :], (8, N))
                    for i in range(len(ar)):
                        nr, ni = _cmul(ar[i], ai[i], mr, mi)
                        ar.append(nr)
                        ai.append(ni)
                vr += ar
                vi += ai
            v = jnp.concatenate(
                [jnp.concatenate(vr, axis=0), jnp.concatenate(vi, axis=0)], axis=1).astype(_BF16)
            uf = ut_v[pl.ds(p, NC, stride=SU), :]
            lhs = jnp.concatenate([jnp.where(lo_c, uf, 0.0), jnp.where(lo_c, 0.0, uf)], axis=0)
            st = lax.dot_general(lhs, v, _NN, preferred_element_type=_F32)
            sr, si = s_buf[p // 8]
            for hf in range(2):
                rows = pl.ds(hf * 8 + p % 8, NC, stride=SG)
                sr[rows, :] = st[hf * NC:(hf + 1) * NC, :N]
                si[rows, :] = st[hf * NC:(hf + 1) * NC, N:]
            return v

        def scan(g):
            sr, si = s_buf[g]
            zr, zi = z_buf[g]
            cat = lambda i: jnp.concatenate([aux_v[i, hf, g * 8:(g + 1) * 8, :] for hf in range(2)], axis=0)
            lr, li = cat(1), cat(2)
            zr[0:16, :] = cat(4)
            zi[0:16, :] = cat(5)
            for c in range(1, NC):
                s_r = sr[pl.ds((c - 1) * SG, 16), :]
                s_i = si[pl.ds((c - 1) * SG, 16), :]
                if c == 1:
                    xr, xi = s_r, -s_i
                else:
                    xr, xi = (xr * lr + s_r) + xi * li, (xi * lr - s_i) - xr * li
                zr[pl.ds(c * SG, 16), :] = xr
                zi[pl.ds(c * SG, 16), :] = xi

        def inter(p, v):
            z = [jnp.concatenate([zb[pl.ds(hf * 8 + p % 8, NC, stride=SG), :] for hf in range(2)], axis=0)
                 for zb in z_buf[p // 8]]
            y = lax.dot_general(jnp.concatenate(z, axis=1), v, _NT, preferred_element_type=_F32)
            return jnp.where(lo_c, y[:NC], y[NC:])

        def intra(p, y):
            kk = jnp.broadcast_to(y[0:1, :], (8, _LANES))
            g1 = pltpu.roll(kk, 1, 1, stride=1, stride_axis=0)
            g1 = jnp.where((lane8 & (_T - 1)) > sub8, g1, 0.0)
            g1 = jnp.take_along_axis(g1, flip8, axis=0)
            g0 = jnp.where((lane8 & (_T - 1)) >= 8, pltpu.roll(g1, 8, 1), 0.0)
            top = pltpu.bitcast(jnp.concatenate([g0, g1], axis=0).astype(_BF16), _U32)
            gs = [(i, pltpu.roll(top, 16 * i, 1) if i else top) for i in range(_T // 16 - 1, -1, -1)]
            hs = [jnp.where((lane8 >= 16 * i) & (lane8 < _T), gv, _U32(0)) for i, gv in gs]
            hs += [jnp.where(lane8 >= _T + 16 * i, gv, _U32(0)) for i, gv in gs]
            hk = pltpu.bitcast(jnp.concatenate(hs, axis=0), _BF16)
            rows = pl.ds(p, NC, stride=SU)
            yd = lax.dot_general(ut_v[rows, :], hk, _NN, preferred_element_type=_F32)
            yt_v[rows, :] = jnp.where(first_c, 0.0, y) + yd

        def block(sb, carry):
            @pl.when(sb > 0)
            def _():
                for t in range(3):
                    w_cp(t, sb - 1).wait()

            for t in range(3):
                w_cp(t, sb).start()

            @pl.when(sb < NB - 1)
            def _():
                u_cp(2 * sb + 2).start()
                u_cp(2 * sb + 3).start()

            @pl.when(sb == NB - 1)
            def _():
                wo_cp(NB).start()

            for hf in range(2):
                aux_v[0, hf] = jnp.broadcast_to(dt_v[2 * sb + hf][0:1, :], (_CB, _CB)).T

            def prepare(i, c, parts):
                if "modes" in parts:
                    for k in range(2 * _CB // 16 // NP):
                        discretise(sb, i * (2 * _CB // 16 // NP) + k)
                if "u" in parts:
                    for k in range(NC // NP):
                        load_u(sb, i * (NC // NP) + k)
                if "weights" in parts:
                    repack((sb - 1) * (DC // 2) + i * (DC // 2 // NP), DC // 2 // NP)
                return c

            @pl.when(sb == 0)
            def _():
                lax.fori_loop(0, NP, functools.partial(prepare, parts=("modes",)), 0)
                u_cp(0).wait()
                u_cp(1).wait()
                lax.fori_loop(0, NP, functools.partial(prepare, parts=("u",)), 0)
                for cp in par_rest:
                    cp.wait()

            @pl.when(sb > 0)
            def _():
                u_cp(2 * sb).wait()
                u_cp(2 * sb + 1).wait()
                lax.fori_loop(0, NP, functools.partial(prepare, parts=("modes", "u", "weights")), 0)
                y_cp(sb - 1).wait()

            for hf in range(2):
                dk_v[2 * sb + hf] = dk_v[2 * sb + hf] + aux_v[3, hf].T[0:8]

            vs, ys = {}, {}
            for p in range(_CB + LAG):
                if p < _CB:
                    vs[p] = states(p)
                    if p % 8 == 7:
                        scan(p // 8)
                if p == _CB // 2:
                    wo_cp(sb).start()
                if p >= LAG:
                    ys[p - LAG] = inter(p - LAG, vs.pop(p - LAG))
            for p in range(_CB):
                intra(p, ys.pop(p))
            y_cp(sb).start()
            return carry
        lax.fori_loop(0, NB, block, 0)
        for t in range(3):
            w_cp(t, NB - 1).wait()
        for j in range(NB + 1, Dm // _LANES):
            wo_cp(j).start()

        def last_repack(i, c):
            repack((NB - 1) * (DC // 2) + i * (DC // 2 // NP), DC // 2 // NP)
            return c
        lax.fori_loop(0, NP, last_repack, 0)

        mem_cp.wait()
        y_cp(NB - 1).wait()
        h_v[0:M, :] = mem0_v[...].astype(_F32)
        row = lax.broadcasted_iota(jnp.int32, (LA, LA), 0)
        col = lax.broadcasted_iota(jnp.int32, (LA, LA), 1)
        mask = (row < M) | (row >= col)
        wo32 = wo_v.bitcast(_U32)

        def segment(xs, dst, wait_wo):
            h_v[M:LA, :] = xs.astype(_F32)

            def proj(hd):
                h = h_v[...]
                r0 = ((hd % 2) * HP + hd // 2) * SW
                return [lax.dot_general(h, pltpu.bitcast(wf_v[t, pl.ds(r0, Dm // 2), :], _BF16), _NN,
                                        preferred_element_type=_F32) for t in range(3)]

            qkv, prob = {}, {}

            def scores(hd):
                q, k, _ = qkv[hd]
                sc = lax.dot_general(q, k, _NT, preferred_element_type=_F32) * scale
                sc = jnp.where(mask, sc, -1e9)
                p = jnp.exp(sc - jnp.max(sc, axis=-1, keepdims=True))
                prob[hd] = p / jnp.sum(p, axis=-1, keepdims=True)

            def values(hd):
                o_v[:, hd * Dh:(hd + 1) * Dh] = lax.dot_general(
                    prob[hd], qkv[hd][2], _NN, preferred_element_type=_F32)

            for hd in range(H):
                qkv[hd] = proj(hd)
                if hd >= 1:
                    scores(hd - 1)
                if hd >= 3:
                    values(hd - 3)
            if wait_wo:
                for j in range(Dm // _LANES):
                    wo_cp(j).wait()
            n1 = H - H // 4
            late = [(scores, H - 1), None, (values, H - 3), (values, H - 2), (values, H - 1)]
            o = o_v[:, 0:n1 * Dh]
            for j in range(Dm // _LANES):
                w = pltpu.bitcast(wo32[j, 0:n1 * Dh // 2, :], _BF16)
                acc_v[:, j * _LANES:(j + 1) * _LANES] = lax.dot_general(o, w, _NN, preferred_element_type=_F32)
                if j < len(late) and late[j] is not None:
                    late[j][0](late[j][1])
            o = o_v[:, n1 * Dh:]
            for j in range(Dm // _LANES):
                cols = slice(j * _LANES, (j + 1) * _LANES)
                w = pltpu.bitcast(wo32[j, n1 * Dh // 2:, :], _BF16)
                res = lax.dot_general(o, w, _NN, preferred_element_type=_F32) + acc_v[:, cols]
                h_v[0:M, cols] = res[0:M]
                dst[:, cols] = res[M:].astype(_BF16)

        def chunk(i, carry, wait_wo=False):
            rows = pl.ds(pl.multiple_of(i * _T, _T), _T)
            dst = out_v.at[rows]
            x_cp(i).wait()
            x_cp(i + XR - 1).start()
            for k in range(_T // seg):
                segment(x_v[i % XR, k * seg:(k + 1) * seg, :], dst.at[pl.ds(k * seg, seg)], wait_wo and k == 0)
            for sb in range(NB):
                y = ya_v[sb, pl.ds(i * SU, _CB), :].T
                for q in range(2):
                    cb = 2 * sb + q
                    skip = u_v[cb, rows, :].astype(_F32) * dk_v[cb][0:1, :]
                    dst[:, Dm + cb * _CB:Dm + (cb + 1) * _CB] = (y[q * _T:(q + 1) * _T] + skip).astype(_BF16)
            pltpu.make_async_copy(dst, out_hbm.at[rows], sem_out).start()
            return carry

        chunk(0, 0, wait_wo=True)
        lax.fori_loop(1, NC, chunk, 0)

        for i in range(NC, NC + XR - 1):
            x_cp(i).wait()
        pltpu.make_async_copy(out_v, out_hbm, sem_out).wait()

    scratch = [
        pltpu.VMEM((XR, _T, Dm), _BF16),
        pltpu.VMEM((M, Dm), _BF16),
        pltpu.VMEM((3, Dm * H, Dh), _BF16),
        pltpu.VMEM((3, H * SW, Dh), _U32),
        pltpu.VMEM((Dm // _LANES, H * Dh, _LANES), _BF16),
        pltpu.VMEM((2 * NB, L, _CB), _BF16),
        pltpu.VMEM((6, D, N), _BF16),
        pltpu.VMEM((D,), _BF16),
        pltpu.VMEM((D,), _BF16),
        pltpu.VMEM((2 * NB, 8, _CB), _F32),
        pltpu.VMEM((2 * NB, 8, _CB), _F32),
        pltpu.VMEM((NC * SU, _LANES), _F32),
        pltpu.VMEM((NC * SU, _LANES), _F32),
        pltpu.VMEM((NB, NC * SU, _LANES), _F32),
        pltpu.VMEM((2, NPOW * SU + 5, N), _F32),
        pltpu.VMEM((2, NPOW * SU + 5, N), _F32),
        pltpu.VMEM((6, 2, _CB, N), _F32),
        pltpu.VMEM((LA, Dm), _F32),
        pltpu.VMEM((LA, H * Dh), _F32),
        pltpu.VMEM((LA, Dm), _F32),
        pltpu.VMEM((S, Dm + D), _BF16),
        pltpu.SemaphoreType.DMA((15,)),
        pltpu.SemaphoreType.DMA((2 * NB,)),
        pltpu.SemaphoreType.DMA((3 * NB,)),
        pltpu.SemaphoreType.DMA((Dm // _LANES,)),
        pltpu.SemaphoreType.DMA((XR,)),
        pltpu.SemaphoreType.DMA(()),
        pltpu.SemaphoreType.DMA(()),
    ] + [pltpu.VMEM((NC * SG, N), _F32)] * (4 * NG)
    return kernel, scratch


@functools.partial(jax.jit, static_argnames=("A_seg_len",))
def pallas_concat_heads__memory_aug_recurrent_mem_tr__ssm_conv_s4__prompt_kernel(
    A_x: jax.Array,
    A_mem0: jax.Array,
    A_Wq: jax.Array,
    A_Wk: jax.Array,
    A_Wv: jax.Array,
    A_Wo: jax.Array,
    A_seg_len: int,
    B_u: jax.Array,
    B_A_re: jax.Array,
    B_A_im: jax.Array,
    B_B_re: jax.Array,
    B_B_im: jax.Array,
    B_C_re: jax.Array,
    B_C_im: jax.Array,
    B_log_dt: jax.Array,
    B_Dskip: jax.Array,
):
    B, S, Dm = A_x.shape
    H, Dh = A_Wq.shape[1], A_Wq.shape[2]
    M = A_mem0.shape[1]
    seg = int(A_seg_len)
    _, L, D = B_u.shape
    N = B_A_re.shape[1]
    assert B == 1 and S == L and S % seg == 0 and Dh == _LANES and N == _LANES

    kernel, scratch = _make_kernel(S, Dm, H, Dh, M, seg, L, D, N)
    out = pl.pallas_call(
        kernel,
        out_shape=jax.ShapeDtypeStruct((S, Dm + D), _BF16),
        in_specs=[pl.BlockSpec(memory_space=pl.ANY)] * 15,
        out_specs=pl.BlockSpec(memory_space=pl.ANY),
        scratch_shapes=scratch,
        compiler_params=pltpu.CompilerParams(vmem_limit_bytes=120 * 1024 * 1024),
    )(
        A_x.reshape(S, Dm), A_mem0.reshape(M, Dm),
        A_Wq.reshape(Dm * H, Dh), A_Wk.reshape(Dm * H, Dh), A_Wv.reshape(Dm * H, Dh),
        A_Wo.reshape(H * Dh, Dm), B_u.reshape(L, D),
        B_A_re, B_A_im, B_B_re, B_B_im, B_C_re, B_C_im, B_log_dt, B_Dskip,
    )
    return out.reshape(B, S, Dm + D)
```

```python
import functools

import jax
import jax.numpy as jnp
from jax import lax
import jax.experimental.pallas as pl
import jax.experimental.pallas.tpu as pltpu

_NN = (((1,), (0,)), ((), ()))
_NT = (((1,), (1,)), ((), ()))
_LANES = 128
_T = 64
_CB = 128
_F32 = jnp.float32
_BF16 = jnp.bfloat16
_U32 = jnp.uint32


def _cmul(ar, ai, br, bi):
    return ar * br - ai * bi, ar * bi + ai * br


def _csqrt(x, y):
    big = jnp.sqrt(0.5 * (jnp.sqrt(x * x + y * y) + jnp.abs(x)))
    small = jnp.where(big > 0, 0.5 * y / big, 0.0)
    pos = x >= 0
    return jnp.where(pos, big, jnp.abs(small)), jnp.where(pos, small, jnp.where(y < 0, -big, big))


def _make_kernel(S, Dm, H, Dh, M, seg, L, D, N):
    LA = M + seg
    scale = Dh ** (-0.5)
    NC = L // _T
    NB = D // (2 * _CB)
    SG = 17
    DC = Dm // NB
    NG = _CB // 8
    NP = 4
    XR = 4
    SPC = _T // seg
    LAG = 24
    SU = _CB + 1
    SW = Dm // 2 + 1
    NPOW = 11
    HP = H // 2

    def kernel(x_hbm, mem0_hbm, wq_hbm, wk_hbm, wv_hbm, wo_hbm, u_hbm,
               are_hbm, aim_hbm, bre_hbm, bim_hbm, cre_hbm, cim_hbm, ldt_hbm, dsk_hbm,
               out_hbm,
               x_v, mem0_v, wraw_v, wf_v, wo_v, u_v, par_v, ldt_v, dsk_v, dt_v, dk_v,
               ut_v, yt_v, ya_v, pr_v, pi_v, aux_v,
               o_v, acc_v, out_v,
               sem_par, sem_u, sem_w, sem_wo, sem_x, sem_out, sem_y, *bufs):
        h_v, st_v = bufs[:SPC], bufs[SPC:]
        par_hbm = (are_hbm, aim_hbm, bre_hbm, bim_hbm, cre_hbm, cim_hbm)
        head, rest = pl.ds(0, 2 * _CB), pl.ds(2 * _CB, D - 2 * _CB)
        par_head = [pltpu.make_async_copy(par_hbm[i].at[head], par_v.at[i, head], sem_par.at[i]) for i in range(6)]
        par_head.append(pltpu.make_async_copy(ldt_hbm, ldt_v, sem_par.at[6]))
        par_head.append(pltpu.make_async_copy(dsk_hbm, dsk_v, sem_par.at[7]))
        par_rest = [pltpu.make_async_copy(par_hbm[i].at[rest], par_v.at[i, rest], sem_par.at[8 + i]) for i in range(6)]
        mem_cp = pltpu.make_async_copy(mem0_hbm, mem0_v, sem_par.at[14])
        w_hbm = (wq_hbm, wk_hbm, wv_hbm)

        def u_cp(cb):
            return pltpu.make_async_copy(
                u_hbm.at[:, pl.ds(pl.multiple_of(cb * _CB, _CB), _CB)], u_v.at[cb], sem_u.at[cb])

        def w_cp(t, cb):
            rows = pl.ds(pl.multiple_of(cb * (DC * H), DC * H), DC * H)
            return pltpu.make_async_copy(w_hbm[t].at[rows], wraw_v.at[t, rows], sem_w.at[t * NB + cb])

        def wo_cp(j):
            return pltpu.make_async_copy(
                wo_hbm.at[:, pl.ds(pl.multiple_of(j * _LANES, _LANES), _LANES)], wo_v.at[j], sem_wo.at[j])

        def y_cp(sb):
            return pltpu.make_async_copy(yt_v, ya_v.at[sb], sem_y)

        def x_cp(i):
            src = pl.ds(pl.multiple_of(jnp.minimum(i, NC - 1) * _T, _T), _T)
            return pltpu.make_async_copy(x_hbm.at[src], x_v.at[i % XR], sem_x.at[i % XR])

        for cp in par_head:
            cp.start()
        u_cp(0).start()
        u_cp(1).start()
        for cp in par_head:
            cp.wait()
        for cp in par_rest:
            cp.start()
        mem_cp.start()
        for i in range(XR - 1):
            x_cp(i).start()

        dt_all = jnp.exp(ldt_v[...].astype(_F32)).astype(_BF16).astype(_F32).reshape(1, D)
        dk_all = dsk_v[...].astype(_F32).reshape(1, D)
        for cb in range(2 * NB):
            dt_v[cb] = jnp.broadcast_to(dt_all[:, cb * _CB:(cb + 1) * _CB], (8, _CB))
            dk_v[cb] = jnp.broadcast_to(dk_all[:, cb * _CB:(cb + 1) * _CB], (8, _CB))

        flip8 = 7 - lax.broadcasted_iota(jnp.int32, (8, _LANES), 0)
        lane8 = lax.broadcasted_iota(jnp.int32, (8, _LANES), 1)
        sub8 = lax.broadcasted_iota(jnp.int32, (8, _LANES), 0)
        lo_c = lax.broadcasted_iota(jnp.int32, (NC, _LANES), 1) < _T
        first_c = lax.broadcasted_iota(jnp.int32, (NC, _LANES), 0) == 0
        raw32 = wraw_v.bitcast(_U32)
        s_buf = [(st_v[4 * i], st_v[4 * i + 1]) for i in range(NG)]
        z_buf = [(st_v[4 * i + 2], st_v[4 * i + 3]) for i in range(NG)]

        def discretise(sb, g):
            hf = g // (_CB // 16)
            g16 = (g % (_CB // 16)) * 16
            r = pl.ds(pl.multiple_of(g16, 16), 16)
            rg = pl.ds(pl.multiple_of(sb * 2 * _CB + g * 16, 16), 16)
            dt = aux_v[0, hf, r, :]
            a = dt * par_v[0, rg, :].astype(_F32)
            b = dt * par_v[1, rg, :].astype(_F32)
            mag = jnp.exp(a)
            l1 = (mag * jnp.cos(b), mag * jnp.sin(b))
            w = _cmul(par_v[4, rg, :].astype(_F32), par_v[5, rg, :].astype(_F32),
                      dt * par_v[2, rg, :].astype(_F32), dt * par_v[3, rg, :].astype(_F32))
            l2 = _cmul(*l1, *l1)
            l4 = _cmul(*l2, *l2)
            l8 = _cmul(*l4, *l4)
            l16 = _cmul(*l8, *l8)
            l32 = _cmul(*l16, *l16)
            l64 = _cmul(*l32, *l32)
            pw = [_csqrt(*_cmul(*w, *l1))]
            pw.append(_cmul(*pw[0], *l1))
            pw += [_cmul(*q, *l2) for q in pw]
            pw += [_cmul(*q, *l4) for q in pw]
            pw += [l8, l16, l32]
            for j in range(NPOW):
                pr_v[hf, pl.ds(j * SU + g16, 16), :] = pw[j][0]
                pi_v[hf, pl.ds(j * SU + g16, 16), :] = pw[j][1]
            aux_v[1, hf, r, :] = l64[0]
            aux_v[2, hf, r, :] = l64[1]
            aux_v[3, hf, r, :] = jnp.broadcast_to(jnp.sum(w[0], axis=-1, keepdims=True), (16, N))
            aux_v[4, hf, r, :] = pw[0][0]
            aux_v[5, hf, r, :] = -pw[0][1]

        def load_u(sb, ck):
            rows = pl.ds(pl.multiple_of(ck * _T, _T), _T)
            fl = []
            for q in range(2):
                tile = u_v[2 * sb + q, rows, :].astype(_F32)
                fl += [jnp.take_along_axis(tile[_T - 8 * (i + 1):_T - 8 * i], flip8, axis=0)
                       for i in range(_T // 8)]
            ut_v[pl.ds(ck * SU, _CB), :] = jnp.concatenate(fl, axis=0).T

        def repack(j0, n):
            for t in range(3):
                src = raw32.at[t, pl.ds(pl.multiple_of(j0 * H, n * H), n * H), :]
                for j in range(n):
                    for half in range(HP // 8):
                        a = src[pl.ds(j * H + half * 8, 8), :]
                        b = src[pl.ds(j * H + HP + half * 8, 8), :]
                        even = (a & _U32(0xFFFF)) | (b << 16)
                        odd = (a >> 16) | (b & _U32(0xFFFF0000))
                        wf_v[t, pl.ds(j0 + (half * 8 * SW + j), 8, stride=SW), :] = even
                        wf_v[t, pl.ds(j0 + ((HP + half * 8) * SW + j), 8, stride=SW), :] = odd

        def states(p):
            vr, vi = [], []
            for hf in range(2):
                ar = [pr_v[hf, pl.ds(p, 8, stride=SU), :]]
                ai = [pi_v[hf, pl.ds(p, 8, stride=SU), :]]
                for lvl in range(3):
                    mr = jnp.broadcast_to(pr_v[hf, pl.ds((8 + lvl) * SU + p, 1), :], (8, N))
                    mi = jnp.broadcast_to(pi_v[hf, pl.ds((8 + lvl) * SU + p, 1), :], (8, N))
                    for i in range(len(ar)):
                        nr, ni = _cmul(ar[i], ai[i], mr, mi)
                        ar.append(nr)
                        ai.append(ni)
                vr += ar
                vi += ai
            v = jnp.concatenate(
                [jnp.concatenate(vr, axis=0), jnp.concatenate(vi, axis=0)], axis=1).astype(_BF16)
            uf = ut_v[pl.ds(p, NC, stride=SU), :]
            lhs = jnp.concatenate([jnp.where(lo_c, uf, 0.0), jnp.where(lo_c, 0.0, uf)], axis=0)
            st = lax.dot_general(lhs, v, _NN, preferred_element_type=_F32)
            sr, si = s_buf[p // 8]
            for hf in range(2):
                rows = pl.ds(hf * 8 + p % 8, NC, stride=SG)
                sr[rows, :] = st[hf * NC:(hf + 1) * NC, :N]
                si[rows, :] = st[hf * NC:(hf + 1) * NC, N:]
            return v

        def scan(g):
            sr, si = s_buf[g]
            zr, zi = z_buf[g]
            cat = lambda i: jnp.concatenate([aux_v[i, hf, g * 8:(g + 1) * 8, :] for hf in range(2)], axis=0)
            lr, li = cat(1), cat(2)
            zr[0:16, :] = cat(4)
            zi[0:16, :] = cat(5)
            for c in range(1, NC):
                s_r = sr[pl.ds((c - 1) * SG, 16), :]
                s_i = si[pl.ds((c - 1) * SG, 16), :]
                if c == 1:
                    xr, xi = s_r, -s_i
                else:
                    xr, xi = (xr * lr + s_r) + xi * li, (xi * lr - s_i) - xr * li
                zr[pl.ds(c * SG, 16), :] = xr
                zi[pl.ds(c * SG, 16), :] = xi

        def inter(p, v):
            z = [jnp.concatenate([zb[pl.ds(hf * 8 + p % 8, NC, stride=SG), :] for hf in range(2)], axis=0)
                 for zb in z_buf[p // 8]]
            y = lax.dot_general(jnp.concatenate(z, axis=1), v, _NT, preferred_element_type=_F32)
            return jnp.where(lo_c, y[:NC], y[NC:])

        def intra(p, y):
            kk = jnp.broadcast_to(y[0:1, :], (8, _LANES))
            g1 = pltpu.roll(kk, 1, 1, stride=1, stride_axis=0)
            g1 = jnp.where((lane8 & (_T - 1)) > sub8, g1, 0.0)
            g1 = jnp.take_along_axis(g1, flip8, axis=0)
            g0 = jnp.where((lane8 & (_T - 1)) >= 8, pltpu.roll(g1, 8, 1), 0.0)
            top = pltpu.bitcast(jnp.concatenate([g0, g1], axis=0).astype(_BF16), _U32)
            gs = [(i, pltpu.roll(top, 16 * i, 1) if i else top) for i in range(_T // 16 - 1, -1, -1)]
            hs = [jnp.where((lane8 >= 16 * i) & (lane8 < _T), gv, _U32(0)) for i, gv in gs]
            hs += [jnp.where(lane8 >= _T + 16 * i, gv, _U32(0)) for i, gv in gs]
            hk = pltpu.bitcast(jnp.concatenate(hs, axis=0), _BF16)
            rows = pl.ds(p, NC, stride=SU)
            yd = lax.dot_general(ut_v[rows, :], hk, _NN, preferred_element_type=_F32)
            yt_v[rows, :] = jnp.where(first_c, 0.0, y) + yd

        def block(sb, carry):
            @pl.when(sb > 0)
            def _():
                for t in range(3):
                    w_cp(t, sb - 1).wait()

            for t in range(3):
                w_cp(t, sb).start()

            @pl.when(sb < NB - 1)
            def _():
                u_cp(2 * sb + 2).start()
                u_cp(2 * sb + 3).start()

            @pl.when(sb == NB - 1)
            def _():
                wo_cp(NB).start()

            for hf in range(2):
                aux_v[0, hf] = jnp.broadcast_to(dt_v[2 * sb + hf][0:1, :], (_CB, _CB)).T

            def prepare(i, c, parts):
                if "modes" in parts:
                    for k in range(2 * _CB // 16 // NP):
                        discretise(sb, i * (2 * _CB // 16 // NP) + k)
                if "u" in parts:
                    for k in range(NC // NP):
                        load_u(sb, i * (NC // NP) + k)
                if "weights" in parts:
                    repack((sb - 1) * (DC // 2) + i * (DC // 2 // NP), DC // 2 // NP)
                return c

            @pl.when(sb == 0)
            def _():
                lax.fori_loop(0, NP, functools.partial(prepare, parts=("modes",)), 0)
                u_cp(0).wait()
                u_cp(1).wait()
                lax.fori_loop(0, NP, functools.partial(prepare, parts=("u",)), 0)
                for cp in par_rest:
                    cp.wait()

            @pl.when(sb > 0)
            def _():
                u_cp(2 * sb).wait()
                u_cp(2 * sb + 1).wait()
                lax.fori_loop(0, NP, functools.partial(prepare, parts=("modes", "u", "weights")), 0)
                y_cp(sb - 1).wait()

            for hf in range(2):
                dk_v[2 * sb + hf] = dk_v[2 * sb + hf] + aux_v[3, hf].T[0:8]

            vs, ys = {}, {}
            for p in range(_CB + LAG):
                if p < _CB:
                    vs[p] = states(p)
                    if p % 8 == 7:
                        scan(p // 8)
                if p == _CB // 2:
                    wo_cp(sb).start()
                if p >= LAG:
                    ys[p - LAG] = inter(p - LAG, vs.pop(p - LAG))
            for p in range(_CB):
                intra(p, ys.pop(p))
            y_cp(sb).start()
            return carry
        lax.fori_loop(0, NB, block, 0)
        for t in range(3):
            w_cp(t, NB - 1).wait()
        for j in range(NB + 1, Dm // _LANES):
            wo_cp(j).start()

        def last_repack(i, c):
            repack((NB - 1) * (DC // 2) + i * (DC // 2 // NP), DC // 2 // NP)
            return c
        lax.fori_loop(0, NP, last_repack, 0)

        mem_cp.wait()
        y_cp(NB - 1).wait()
        x_cp(0).wait()
        h_v[0][0:M, :] = mem0_v[...].astype(_F32)
        h_v[0][M:LA, :] = x_v[0, 0:seg, :].astype(_F32)
        row = lax.broadcasted_iota(jnp.int32, (LA, LA), 0)
        col = lax.broadcasted_iota(jnp.int32, (LA, LA), 1)
        mask = (row < M) | (row >= col)
        wo32 = wo_v.bitcast(_U32)

        def segment(h_in, h_out, dst, side_work, wait_wo):
            def proj(hd):
                h = h_in[...]
                r0 = ((hd % 2) * HP + hd // 2) * SW
                return [lax.dot_general(h, pltpu.bitcast(wf_v[t, pl.ds(r0, Dm // 2), :], _BF16), _NN,
                                        preferred_element_type=_F32) for t in range(3)]

            qkv, prob = {}, {}

            def scores(hd):
                q, k, _ = qkv[hd]
                sc = lax.dot_general(q, k, _NT, preferred_element_type=_F32) * scale
                sc = jnp.where(mask, sc, -1e9)
                p = jnp.exp(sc - jnp.max(sc, axis=-1, keepdims=True))
                prob[hd] = p / jnp.sum(p, axis=-1, keepdims=True)

            def values(hd):
                o_v[:, hd * Dh:(hd + 1) * Dh] = lax.dot_general(
                    prob[hd], qkv[hd][2], _NN, preferred_element_type=_F32)

            for hd in range(H):
                qkv[hd] = proj(hd)
                if hd >= 1:
                    scores(hd - 1)
                if hd >= 3:
                    values(hd - 3)
                if hd in side_work:
                    side_work[hd]()
            if wait_wo:
                for j in range(Dm // _LANES):
                    wo_cp(j).wait()
            n1 = H - H // 4
            late = [(scores, H - 1), None, (values, H - 3), (values, H - 2), (values, H - 1)]
            o = o_v[:, 0:n1 * Dh]
            for j in range(Dm // _LANES):
                w = pltpu.bitcast(wo32[j, 0:n1 * Dh // 2, :], _BF16)
                acc_v[:, j * _LANES:(j + 1) * _LANES] = lax.dot_general(o, w, _NN, preferred_element_type=_F32)
                if j < len(late) and late[j] is not None:
                    late[j][0](late[j][1])
            o = o_v[:, n1 * Dh:]
            for j in range(Dm // _LANES):
                cols = slice(j * _LANES, (j + 1) * _LANES)
                w = pltpu.bitcast(wo32[j, n1 * Dh // 2:, :], _BF16)
                res = lax.dot_general(o, w, _NN, preferred_element_type=_F32) + acc_v[:, cols]
                h_out[0:M, cols] = res[0:M]
                dst[:, cols] = res[M:].astype(_BF16)

        def out_cp(i):
            rows = pl.ds(pl.multiple_of(i * _T, _T), _T)
            return pltpu.make_async_copy(out_v.at[rows], out_hbm.at[rows], sem_out)

        def chunk(i, carry, first=False):
            rows = pl.ds(pl.multiple_of(i * _T, _T), _T)
            dst = out_v.at[rows]
            x_cp(i + 1).wait()

            def s4_epilogue(sb):
                y = ya_v[sb, pl.ds(i * SU, _CB), :].T
                for q in range(2):
                    cb = 2 * sb + q
                    skip = u_v[cb, rows, :].astype(_F32) * dk_v[cb][0:1, :]
                    dst[:, Dm + cb * _CB:Dm + (cb + 1) * _CB] = (y[q * _T:(q + 1) * _T] + skip).astype(_BF16)

            def next_rows(k):
                if k < SPC:
                    h_v[k][M:LA, :] = x_v[i % XR, k * seg:(k + 1) * seg, :].astype(_F32)
                else:
                    h_v[0][M:LA, :] = x_v[(i + 1) % XR, 0:seg, :].astype(_F32)

            def traffic():
                x_cp(i + XR - 1).start()
                if not first:
                    out_cp(i - 1).start()

            for k in range(SPC):
                side = {H // 2: functools.partial(next_rows, k + 1)}
                if k == 0:
                    side[2] = traffic
                    for sb in range(NB):
                        side[4 + 2 * sb] = functools.partial(s4_epilogue, sb)
                segment(h_v[k], h_v[(k + 1) % SPC], dst.at[pl.ds(k * seg, seg)], side, first and k == 0)
            return carry

        chunk(0, 0, first=True)
        lax.fori_loop(1, NC, chunk, 0)
        out_cp(NC - 1).start()

        for i in range(NC + 1, NC + XR - 1):
            x_cp(i).wait()
        pltpu.make_async_copy(out_v, out_hbm, sem_out).wait()

    scratch = [
        pltpu.VMEM((XR, _T, Dm), _BF16),
        pltpu.VMEM((M, Dm), _BF16),
        pltpu.VMEM((3, Dm * H, Dh), _BF16),
        pltpu.VMEM((3, H * SW, Dh), _U32),
        pltpu.VMEM((Dm // _LANES, H * Dh, _LANES), _BF16),
        pltpu.VMEM((2 * NB, L, _CB), _BF16),
        pltpu.VMEM((6, D, N), _BF16),
        pltpu.VMEM((D,), _BF16),
        pltpu.VMEM((D,), _BF16),
        pltpu.VMEM((2 * NB, 8, _CB), _F32),
        pltpu.VMEM((2 * NB, 8, _CB), _F32),
        pltpu.VMEM((NC * SU, _LANES), _F32),
        pltpu.VMEM((NC * SU, _LANES), _F32),
        pltpu.VMEM((NB, NC * SU, _LANES), _F32),
        pltpu.VMEM((2, NPOW * SU + 5, N), _F32),
        pltpu.VMEM((2, NPOW * SU + 5, N), _F32),
        pltpu.VMEM((6, 2, _CB, N), _F32),
        pltpu.VMEM((LA, H * Dh), _F32),
        pltpu.VMEM((LA, Dm), _F32),
        pltpu.VMEM((S, Dm + D), _BF16),
        pltpu.SemaphoreType.DMA((15,)),
        pltpu.SemaphoreType.DMA((2 * NB,)),
        pltpu.SemaphoreType.DMA((3 * NB,)),
        pltpu.SemaphoreType.DMA((Dm // _LANES,)),
        pltpu.SemaphoreType.DMA((XR,)),
        pltpu.SemaphoreType.DMA(()),
        pltpu.SemaphoreType.DMA(()),
    ]
    scratch += [pltpu.VMEM((LA, Dm), _F32)] * SPC
    scratch += [pltpu.VMEM((NC * SG, N), _F32)] * (4 * NG)
    return kernel, scratch


@functools.partial(jax.jit, static_argnames=("A_seg_len",))
def pallas_concat_heads__memory_aug_recurrent_mem_tr__ssm_conv_s4__prompt_kernel(
    A_x: jax.Array,
    A_mem0: jax.Array,
    A_Wq: jax.Array,
    A_Wk: jax.Array,
    A_Wv: jax.Array,
    A_Wo: jax.Array,
    A_seg_len: int,
    B_u: jax.Array,
    B_A_re: jax.Array,
    B_A_im: jax.Array,
    B_B_re: jax.Array,
    B_B_im: jax.Array,
    B_C_re: jax.Array,
    B_C_im: jax.Array,
    B_log_dt: jax.Array,
    B_Dskip: jax.Array,
):
    B, S, Dm = A_x.shape
    H, Dh = A_Wq.shape[1], A_Wq.shape[2]
    M = A_mem0.shape[1]
    seg = int(A_seg_len)
    _, L, D = B_u.shape
    N = B_A_re.shape[1]
    assert B == 1 and S == L and S % seg == 0 and Dh == _LANES and N == _LANES

    kernel, scratch = _make_kernel(S, Dm, H, Dh, M, seg, L, D, N)
    out = pl.pallas_call(
        kernel,
        out_shape=jax.ShapeDtypeStruct((S, Dm + D), _BF16),
        in_specs=[pl.BlockSpec(memory_space=pl.ANY)] * 15,
        out_specs=pl.BlockSpec(memory_space=pl.ANY),
        scratch_shapes=scratch,
        compiler_params=pltpu.CompilerParams(vmem_limit_bytes=120 * 1024 * 1024),
    )(
        A_x.reshape(S, Dm), A_mem0.reshape(M, Dm),
        A_Wq.reshape(Dm * H, Dh), A_Wk.reshape(Dm * H, Dh), A_Wv.reshape(Dm * H, Dh),
        A_Wo.reshape(H * Dh, Dm), B_u.reshape(L, D),
        B_A_re, B_A_im, B_B_re, B_B_im, B_C_re, B_C_im, B_log_dt, B_Dskip,
    )
    return out.reshape(B, S, Dm + D)
```

```python
import functools

import jax
import jax.numpy as jnp
from jax import lax
import jax.experimental.pallas as pl
import jax.experimental.pallas.tpu as pltpu

_NN = (((1,), (0,)), ((), ()))
_NT = (((1,), (1,)), ((), ()))
_LANES = 128
_T = 64
_CB = 128
_F32 = jnp.float32
_BF16 = jnp.bfloat16
_U32 = jnp.uint32


def _cmul(ar, ai, br, bi):
    return ar * br - ai * bi, ar * bi + ai * br


def _csqrt(x, y):
    big = jnp.sqrt(0.5 * (jnp.sqrt(x * x + y * y) + jnp.abs(x)))
    small = jnp.where(big > 0, 0.5 * y / big, 0.0)
    pos = x >= 0
    return jnp.where(pos, big, jnp.abs(small)), jnp.where(pos, small, jnp.where(y < 0, -big, big))


def _make_kernel(S, Dm, H, Dh, M, seg, L, D, N):
    LA = M + seg
    scale = Dh ** (-0.5)
    NC = L // _T
    NB = D // (2 * _CB)
    SG = 17
    DC = Dm // NB
    NG = _CB // 8
    XR = 4
    SPC = _T // seg
    LAG = 24
    SU = _CB + 1
    SW = Dm // 2 + 1
    NPOW = 11
    HP = H // 2
    PRE = 8
    NPRE = 4
    R = NPRE * SPC * PRE

    def head_row(hd):
        return ((hd % 2) * HP + hd // 2) * SW

    def kernel(x_hbm, mem0_hbm, wq_hbm, wk_hbm, wv_hbm, wo_hbm, u_hbm,
               are_hbm, aim_hbm, bre_hbm, bim_hbm, cre_hbm, cim_hbm, ldt_hbm, dsk_hbm,
               out_hbm,
               x_v, xpre_v, xb_v, zpre_v, mem0_v, wraw_v, wo_v, u_v, par_v, ldt_v, dsk_v, dt_v, dk_v,
               ut_v, yt_v, ya_v, pr_v, pi_v, aux_v,
               o_v, acc_v, out_v,
               sem_par, sem_u, sem_w, sem_wo, sem_x, sem_out, sem_y, *bufs):
        h_v, wf_v, st_v = bufs[:SPC], bufs[SPC:SPC + 3], bufs[SPC + 3:]
        par_hbm = (are_hbm, aim_hbm, bre_hbm, bim_hbm, cre_hbm, cim_hbm)
        head, rest = pl.ds(0, 2 * _CB), pl.ds(2 * _CB, D - 2 * _CB)
        par_head = [pltpu.make_async_copy(par_hbm[i].at[head], par_v.at[i, head], sem_par.at[i]) for i in range(6)]
        par_head.append(pltpu.make_async_copy(ldt_hbm, ldt_v, sem_par.at[6]))
        par_head.append(pltpu.make_async_copy(dsk_hbm, dsk_v, sem_par.at[7]))
        par_rest = [pltpu.make_async_copy(par_hbm[i].at[rest], par_v.at[i, rest], sem_par.at[8 + i]) for i in range(6)]
        mem_cp = pltpu.make_async_copy(mem0_hbm, mem0_v, sem_par.at[14])
        w_hbm = (wq_hbm, wk_hbm, wv_hbm)

        def u_cp(cb):
            return pltpu.make_async_copy(
                u_hbm.at[:, pl.ds(pl.multiple_of(cb * _CB, _CB), _CB)], u_v.at[cb], sem_u.at[cb])

        def w_cp(t, cb):
            rows = pl.ds(pl.multiple_of(cb * (DC * H), DC * H), DC * H)
            return pltpu.make_async_copy(w_hbm[t].at[rows], wraw_v.at[t, rows], sem_w.at[t * NB + cb])

        def wo_cp(j):
            return pltpu.make_async_copy(
                wo_hbm.at[:, pl.ds(pl.multiple_of(j * _LANES, _LANES), _LANES)], wo_v.at[j], sem_wo.at[j])

        def y_cp(sb):
            return pltpu.make_async_copy(yt_v, ya_v.at[sb], sem_y)

        def x_cp(i):
            src = pl.ds(jnp.minimum(i, NC - 1) * SPC, SPC)
            return pltpu.make_async_copy(x_hbm.at[src], x_v.at[i % XR], sem_x.at[i % XR])

        xpre_cp = pltpu.make_async_copy(
            x_hbm.at[pl.ds(0, NPRE * SPC), pl.ds(seg - PRE, PRE)], xpre_v, sem_par.at[15])

        for cp in par_head:
            cp.start()
        u_cp(0).start()
        u_cp(1).start()
        zpre_v[...] = jnp.zeros(zpre_v.shape, _F32)
        for cp in par_head:
            cp.wait()
        for cp in par_rest:
            cp.start()
        mem_cp.start()
        xpre_cp.start()
        for i in range(XR - 1):
            x_cp(i).start()

        dt_all = jnp.exp(ldt_v[...].astype(_F32)).astype(_BF16).astype(_F32).reshape(1, D)
        dk_all = dsk_v[...].astype(_F32).reshape(1, D)
        for cb in range(2 * NB):
            dt_v[cb] = jnp.broadcast_to(dt_all[:, cb * _CB:(cb + 1) * _CB], (8, _CB))
            dk_v[cb] = jnp.broadcast_to(dk_all[:, cb * _CB:(cb + 1) * _CB], (8, _CB))

        flip8 = 7 - lax.broadcasted_iota(jnp.int32, (8, _LANES), 0)
        lane8 = lax.broadcasted_iota(jnp.int32, (8, _LANES), 1)
        sub8 = lax.broadcasted_iota(jnp.int32, (8, _LANES), 0)
        lo_c = lax.broadcasted_iota(jnp.int32, (NC, _LANES), 1) < _T
        first_c = lax.broadcasted_iota(jnp.int32, (NC, _LANES), 0) == 0
        raw32 = wraw_v.bitcast(_U32)
        s_buf = [(st_v[4 * i], st_v[4 * i + 1]) for i in range(NG)]
        z_buf = [(st_v[4 * i + 2], st_v[4 * i + 3]) for i in range(NG)]

        def discretise(sb, g):
            hf = g // (_CB // 16)
            g16 = (g % (_CB // 16)) * 16
            r = pl.ds(pl.multiple_of(g16, 16), 16)
            rg = pl.ds(pl.multiple_of(sb * 2 * _CB + g * 16, 16), 16)
            dt = aux_v[0, hf, r, :]
            a = dt * par_v[0, rg, :].astype(_F32)
            b = dt * par_v[1, rg, :].astype(_F32)
            mag = jnp.exp(a)
            l1 = (mag * jnp.cos(b), mag * jnp.sin(b))
            w = _cmul(par_v[4, rg, :].astype(_F32), par_v[5, rg, :].astype(_F32),
                      dt * par_v[2, rg, :].astype(_F32), dt * par_v[3, rg, :].astype(_F32))
            l2 = _cmul(*l1, *l1)
            l4 = _cmul(*l2, *l2)
            l8 = _cmul(*l4, *l4)
            l16 = _cmul(*l8, *l8)
            l32 = _cmul(*l16, *l16)
            l64 = _cmul(*l32, *l32)
            pw = [_csqrt(*_cmul(*w, *l1))]
            pw.append(_cmul(*pw[0], *l1))
            pw += [_cmul(*q, *l2) for q in pw]
            pw += [_cmul(*q, *l4) for q in pw]
            pw += [l8, l16, l32]
            for j in range(NPOW):
                pr_v[hf, pl.ds(j * SU + g16, 16), :] = pw[j][0]
                pi_v[hf, pl.ds(j * SU + g16, 16), :] = pw[j][1]
            aux_v[1, hf, r, :] = l64[0]
            aux_v[2, hf, r, :] = l64[1]
            aux_v[3, hf, r, :] = jnp.broadcast_to(jnp.sum(w[0], axis=-1, keepdims=True), (16, N))
            aux_v[4, hf, r, :] = pw[0][0]
            aux_v[5, hf, r, :] = -pw[0][1]
            return pw[7][0][8:16]

        def load_u(sb, ck):
            rows = pl.ds(pl.multiple_of(ck * _T, _T), _T)
            fl = []
            for q in range(2):
                tile = u_v[2 * sb + q, rows, :].astype(_F32)
                fl += [jnp.take_along_axis(tile[_T - 8 * (i + 1):_T - 8 * i], flip8, axis=0)
                       for i in range(_T // 8)]
            ut = jnp.concatenate(fl, axis=0).T
            ut_v[pl.ds(ck * SU, _CB), :] = ut
            return ut[_CB - 8:]

        def repack(c):
            nj = DC // 2 // 4

            def body(i, carry):
                j0 = c * (DC // 2) + i * nj
                for t in range(3):
                    src = raw32.at[t, pl.ds(pl.multiple_of(j0 * H, nj * H), nj * H), :]
                    for j in range(nj):
                        for half in range(HP // 8):
                            a = src[pl.ds(j * H + half * 8, 8), :]
                            b = src[pl.ds(j * H + HP + half * 8, 8), :]
                            wf_v[t][pl.ds(j0 + (half * 8 * SW + j), 8, stride=SW), :] = (a & _U32(0xFFFF)) | (b << 16)
                            wf_v[t][pl.ds(j0 + ((HP + half * 8) * SW + j), 8, stride=SW), :] = (
                                (a >> 16) | (b & _U32(0xFFFF0000)))
                return carry
            lax.fori_loop(0, 4, body, 0)

        def project_ahead(c, par):
            lhs = xb_v[c]
            r0 = par * (HP * SW) + c * (DC // 2)
            for t in range(3):
                for k in range(HP):
                    w = wf_v[t][pl.ds(r0 + k * SW, DC // 2), :]
                    zpre_v[par, t * HP + k] += lax.dot_general(
                        lhs, pltpu.bitcast(w, _BF16), _NN, preferred_element_type=_F32)

        def states(p):
            vr, vi = [], []
            for hf in range(2):
                ar = [pr_v[hf, pl.ds(p, 8, stride=SU), :]]
                ai = [pi_v[hf, pl.ds(p, 8, stride=SU), :]]
                for lvl in range(3):
                    mr = jnp.broadcast_to(pr_v[hf, pl.ds((8 + lvl) * SU + p, 1), :], (8, N))
                    mi = jnp.broadcast_to(pi_v[hf, pl.ds((8 + lvl) * SU + p, 1), :], (8, N))
                    for i in range(len(ar)):
                        nr, ni = _cmul(ar[i], ai[i], mr, mi)
                        ar.append(nr)
                        ai.append(ni)
                vr += ar
                vi += ai
            v = jnp.concatenate(
                [jnp.concatenate(vr, axis=0), jnp.concatenate(vi, axis=0)], axis=1).astype(_BF16)
            uf = ut_v[pl.ds(p, NC, stride=SU), :]
            lhs = jnp.concatenate([jnp.where(lo_c, uf, 0.0), jnp.where(lo_c, 0.0, uf)], axis=0)
            st = lax.dot_general(lhs, v, _NN, preferred_element_type=_F32)
            sr, si = s_buf[p // 8]
            for hf in range(2):
                rows = pl.ds(hf * 8 + p % 8, NC, stride=SG)
                sr[rows, :] = st[hf * NC:(hf + 1) * NC, :N]
                si[rows, :] = st[hf * NC:(hf + 1) * NC, N:]
            return v

        def scan(g):
            sr, si = s_buf[g]
            zr, zi = z_buf[g]
            cat = lambda i: jnp.concatenate([aux_v[i, hf, g * 8:(g + 1) * 8, :] for hf in range(2)], axis=0)
            lr, li = cat(1), cat(2)
            zr[0:16, :] = cat(4)
            zi[0:16, :] = cat(5)
            for c in range(1, NC):
                s_r = sr[pl.ds((c - 1) * SG, 16), :]
                s_i = si[pl.ds((c - 1) * SG, 16), :]
                if c == 1:
                    xr, xi = s_r, -s_i
                else:
                    xr, xi = (xr * lr + s_r) + xi * li, (xi * lr - s_i) - xr * li
                zr[pl.ds(c * SG, 16), :] = xr
                zi[pl.ds(c * SG, 16), :] = xi

        def inter(p, v):
            z = [jnp.concatenate([zb[pl.ds(hf * 8 + p % 8, NC, stride=SG), :] for hf in range(2)], axis=0)
                 for zb in z_buf[p // 8]]
            y = lax.dot_general(jnp.concatenate(z, axis=1), v, _NT, preferred_element_type=_F32)
            return jnp.where(lo_c, y[:NC], y[NC:])

        def intra(p, y):
            kk = jnp.broadcast_to(y[0:1, :], (8, _LANES))
            g1 = pltpu.roll(kk, 1, 1, stride=1, stride_axis=0)
            g1 = jnp.where((lane8 & (_T - 1)) > sub8, g1, 0.0)
            g1 = jnp.take_along_axis(g1, flip8, axis=0)
            g0 = jnp.where((lane8 & (_T - 1)) >= 8, pltpu.roll(g1, 8, 1), 0.0)
            top = pltpu.bitcast(jnp.concatenate([g0, g1], axis=0).astype(_BF16), _U32)
            gs = [(i, pltpu.roll(top, 16 * i, 1) if i else top) for i in range(_T // 16 - 1, -1, -1)]
            hs = [jnp.where((lane8 >= 16 * i) & (lane8 < _T), gv, _U32(0)) for i, gv in gs]
            hs += [jnp.where(lane8 >= _T + 16 * i, gv, _U32(0)) for i, gv in gs]
            hk = pltpu.bitcast(jnp.concatenate(hs, axis=0), _BF16)
            rows = pl.ds(p, NC, stride=SU)
            yd = lax.dot_general(ut_v[rows, :], hk, _NN, preferred_element_type=_F32)
            yt_v[rows, :] = jnp.where(first_c, 0.0, y) + yd

        def block(sb, carry):
            @pl.when(sb > 0)
            def _():
                for t in range(3):
                    w_cp(t, sb - 1).wait()

            for t in range(3):
                w_cp(t, sb).start()

            @pl.when(sb < NB - 1)
            def _():
                u_cp(2 * sb + 2).start()
                u_cp(2 * sb + 3).start()

            for hf in range(2):
                aux_v[0, hf] = jnp.broadcast_to(dt_v[2 * sb + hf][0:1, :], (_CB, _CB)).T

            @pl.when(sb == 0)
            def _():
                def modes(i, c):
                    for k in range(4):
                        discretise(0, i * 4 + k)
                    return c
                lax.fori_loop(0, 2 * _CB // 64, modes, 0)
                u_cp(0).wait()
                u_cp(1).wait()

                def chunks(i, c):
                    for k in range(8):
                        load_u(0, i * 8 + k)
                    return c
                lax.fori_loop(0, NC // 8, chunks, 0)
                for cp in par_rest:
                    cp.wait()
                xpre_cp.wait()
                xpre = xpre_v[...].astype(_F32).reshape(R, Dm)
                for c in range(NB):
                    xb_v[c] = xpre[:, c * DC:(c + 1) * DC]

            @pl.when(sb > 0)
            def _():
                repack(sb - 1)
                u_cp(2 * sb).wait()
                u_cp(2 * sb + 1).wait()

                def prepare(i, c):
                    for k in range(_CB // 16):
                        discretise(sb, i * (_CB // 16) + k)
                    for k in range(NC // 2):
                        load_u(sb, i * (NC // 2) + k)
                    project_ahead(sb - 1, i)
                    return c
                lax.fori_loop(0, 2, prepare, 0)
                y_cp(sb - 1).wait()

            for hf in range(2):
                dk_v[2 * sb + hf] = dk_v[2 * sb + hf] + aux_v[3, hf].T[0:8]

            vs, ys = {}, {}
            for p in range(_CB + LAG):
                if p < _CB:
                    vs[p] = states(p)
                    if p % 8 == 7:
                        scan(p // 8)
                if p == _CB // 2:
                    wo_cp(2 * sb).start()
                    wo_cp(2 * sb + 1).start()
                if p >= LAG:
                    ys[p - LAG] = inter(p - LAG, vs.pop(p - LAG))
            for p in range(_CB):
                intra(p, ys.pop(p))
            y_cp(sb).start()
            return carry
        lax.fori_loop(0, NB, block, 0)
        for t in range(3):
            w_cp(t, NB - 1).wait()
        repack(NB - 1)
        lax.fori_loop(0, 2, lambda i, c: project_ahead(NB - 1, i), None)

        mem_cp.wait()
        y_cp(NB - 1).wait()
        x_cp(0).wait()
        h_v[0][0:M, :] = mem0_v[...].astype(_F32)
        h_v[0][M:LA, :] = x_v[0, 0].astype(_F32)
        row = lax.broadcasted_iota(jnp.int32, (LA, LA), 0)
        col = lax.broadcasted_iota(jnp.int32, (LA, LA), 1)
        mask = (row < M) | (row >= col)
        wo32 = wo_v.bitcast(_U32)

        def segment(h_in, h_out, dst, side_work, pre_rows):
            def proj(hd):
                h = h_in[...] if pre_rows is None else h_in[0:LA - PRE, :]
                out = [lax.dot_general(h, pltpu.bitcast(wf_v[t][pl.ds(head_row(hd), Dm // 2), :], _BF16), _NN,
                                       preferred_element_type=_F32) for t in range(3)]
                if pre_rows is not None:
                    out = [jnp.concatenate([out[t], zpre_v[hd % 2, t * HP + hd // 2, pre_rows, :]], axis=0) for t in range(3)]
                return out

            qkv, prob = {}, {}

            def scores(hd):
                q, k, _ = qkv[hd]
                sc = lax.dot_general(q, k, _NT, preferred_element_type=_F32) * scale
                sc = jnp.where(mask, sc, -1e9)
                p = jnp.exp(sc - jnp.max(sc, axis=-1, keepdims=True))
                prob[hd] = p / jnp.sum(p, axis=-1, keepdims=True)

            def values(hd):
                o_v[:, hd * Dh:(hd + 1) * Dh] = lax.dot_general(
                    prob[hd], qkv[hd][2], _NN, preferred_element_type=_F32)

            for hd in range(H):
                qkv[hd] = proj(hd)
                if hd >= 1:
                    scores(hd - 1)
                if hd >= 3:
                    values(hd - 3)
                if hd in side_work:
                    side_work[hd]()
            n1 = H - H // 4
            late = [(scores, H - 1), None, (values, H - 3), (values, H - 2), (values, H - 1)]
            o = o_v[:, 0:n1 * Dh]
            for j in range(Dm // _LANES):
                w = pltpu.bitcast(wo32[j, 0:n1 * Dh // 2, :], _BF16)
                acc_v[:, j * _LANES:(j + 1) * _LANES] = lax.dot_general(o, w, _NN, preferred_element_type=_F32)
                if j < len(late) and late[j] is not None:
                    late[j][0](late[j][1])
            o = o_v[:, n1 * Dh:]
            for j in range(Dm // _LANES):
                cols = slice(j * _LANES, (j + 1) * _LANES)
                w = pltpu.bitcast(wo32[j, n1 * Dh // 2:, :], _BF16)
                res = lax.dot_general(o, w, _NN, preferred_element_type=_F32) + acc_v[:, cols]
                h_out[0:M, cols] = res[0:M]
                dst[:, cols] = res[M:].astype(_BF16)

        def out_cp(i):
            rows = pl.ds(pl.multiple_of(i * _T, _T), _T)
            return pltpu.make_async_copy(out_v.at[rows], out_hbm.at[rows], sem_out)

        def chunk(i, carry, ahead):
            rows = pl.ds(pl.multiple_of(i * _T, _T), _T)
            dst = out_v.at[rows]
            x_cp(i + 1).wait()

            def s4_epilogue(sb):
                y = ya_v[sb, pl.ds(i * SU, _CB), :].T
                for q in range(2):
                    cb = 2 * sb + q
                    skip = u_v[cb, rows, :].astype(_F32) * dk_v[cb][0:1, :]
                    dst[:, Dm + cb * _CB:Dm + (cb + 1) * _CB] = (y[q * _T:(q + 1) * _T] + skip).astype(_BF16)

            def next_rows(k):
                if k < SPC:
                    h_v[k][M:LA, :] = x_v[i % XR, k].astype(_F32)
                else:
                    h_v[0][M:LA, :] = x_v[(i + 1) % XR, 0].astype(_F32)

            def traffic():
                x_cp(i + XR - 1).start()

            for k in range(SPC):
                side = {H // 2: functools.partial(next_rows, k + 1)}
                if k == 0:
                    side[2] = traffic
                    for sb in range(NB):
                        side[4 + 2 * sb] = functools.partial(s4_epilogue, sb)
                pre_rows = pl.ds(pl.multiple_of((i * SPC + k) * PRE, PRE), PRE) if ahead else None
                segment(h_v[k], h_v[(k + 1) % SPC], dst.at[pl.ds(k * seg, seg)], side, pre_rows)
            out_cp(i).start()
            return carry

        for j in range(Dm // _LANES):
            wo_cp(j).wait()
        lax.fori_loop(0, NPRE, functools.partial(chunk, ahead=True), 0)
        lax.fori_loop(NPRE, NC, functools.partial(chunk, ahead=False), 0)

        for i in range(NC + 1, NC + XR - 1):
            x_cp(i).wait()
        pltpu.make_async_copy(out_v, out_hbm, sem_out).wait()

    scratch = [
        pltpu.VMEM((XR, SPC, seg, Dm), _BF16),
        pltpu.VMEM((NPRE * SPC, PRE, Dm), _BF16),
        pltpu.VMEM((NB, R, DC), _F32),
        pltpu.VMEM((2, 3 * HP, R, Dh), _F32),
        pltpu.VMEM((M, Dm), _BF16),
        pltpu.VMEM((3, Dm * H, Dh), _BF16),
        pltpu.VMEM((Dm // _LANES, H * Dh, _LANES), _BF16),
        pltpu.VMEM((2 * NB, L, _CB), _BF16),
        pltpu.VMEM((6, D, N), _BF16),
        pltpu.VMEM((D,), _BF16),
        pltpu.VMEM((D,), _BF16),
        pltpu.VMEM((2 * NB, 8, _CB), _F32),
        pltpu.VMEM((2 * NB, 8, _CB), _F32),
        pltpu.VMEM((NC * SU, _LANES), _F32),
        pltpu.VMEM((NC * SU, _LANES), _F32),
        pltpu.VMEM((NB, NC * SU, _LANES), _F32),
        pltpu.VMEM((2, NPOW * SU + 5, N), _F32),
        pltpu.VMEM((2, NPOW * SU + 5, N), _F32),
        pltpu.VMEM((6, 2, _CB, N), _F32),
        pltpu.VMEM((LA, H * Dh), _F32),
        pltpu.VMEM((LA, Dm), _F32),
        pltpu.VMEM((S, Dm + D), _BF16),
        pltpu.SemaphoreType.DMA((16,)),
        pltpu.SemaphoreType.DMA((2 * NB,)),
        pltpu.SemaphoreType.DMA((3 * NB,)),
        pltpu.SemaphoreType.DMA((Dm // _LANES,)),
        pltpu.SemaphoreType.DMA((XR,)),
        pltpu.SemaphoreType.DMA(()),
        pltpu.SemaphoreType.DMA(()),
    ]
    scratch += [pltpu.VMEM((LA, Dm), _F32)] * SPC
    scratch += [pltpu.VMEM((H * SW, Dh), _U32)] * 3
    scratch += [pltpu.VMEM((NC * SG, N), _F32)] * (4 * NG)
    return kernel, scratch


@functools.partial(jax.jit, static_argnames=("A_seg_len",))
def pallas_concat_heads__memory_aug_recurrent_mem_tr__ssm_conv_s4__prompt_kernel(
    A_x: jax.Array,
    A_mem0: jax.Array,
    A_Wq: jax.Array,
    A_Wk: jax.Array,
    A_Wv: jax.Array,
    A_Wo: jax.Array,
    A_seg_len: int,
    B_u: jax.Array,
    B_A_re: jax.Array,
    B_A_im: jax.Array,
    B_B_re: jax.Array,
    B_B_im: jax.Array,
    B_C_re: jax.Array,
    B_C_im: jax.Array,
    B_log_dt: jax.Array,
    B_Dskip: jax.Array,
):
    B, S, Dm = A_x.shape
    H, Dh = A_Wq.shape[1], A_Wq.shape[2]
    M = A_mem0.shape[1]
    seg = int(A_seg_len)
    _, L, D = B_u.shape
    N = B_A_re.shape[1]
    assert B == 1 and S == L and S % seg == 0 and Dh == _LANES and N == _LANES

    kernel, scratch = _make_kernel(S, Dm, H, Dh, M, seg, L, D, N)
    out = pl.pallas_call(
        kernel,
        out_shape=jax.ShapeDtypeStruct((S, Dm + D), _BF16),
        in_specs=[pl.BlockSpec(memory_space=pl.ANY)] * 15,
        out_specs=pl.BlockSpec(memory_space=pl.ANY),
        scratch_shapes=scratch,
        compiler_params=pltpu.CompilerParams(vmem_limit_bytes=120 * 1024 * 1024),
    )(
        A_x.reshape(S // seg, seg, Dm), A_mem0.reshape(M, Dm),
        A_Wq.reshape(Dm * H, Dh), A_Wk.reshape(Dm * H, Dh), A_Wv.reshape(Dm * H, Dh),
        A_Wo.reshape(H * Dh, Dm), B_u.reshape(L, D),
        B_A_re, B_A_im, B_B_re, B_B_im, B_C_re, B_C_im, B_log_dt, B_Dskip,
    )
    return out.reshape(B, S, Dm + D)
```

```python
import functools

import jax
import jax.numpy as jnp
from jax import lax
import jax.experimental.pallas as pl
import jax.experimental.pallas.tpu as pltpu

_NN = (((1,), (0,)), ((), ()))
_NT = (((1,), (1,)), ((), ()))
_LANES = 128
_T = 64
_CB = 128
_F32 = jnp.float32
_BF16 = jnp.bfloat16
_U32 = jnp.uint32


def _cmul(ar, ai, br, bi):
    return ar * br - ai * bi, ar * bi + ai * br


def _csqrt(x, y):
    big = jnp.sqrt(0.5 * (jnp.sqrt(x * x + y * y) + jnp.abs(x)))
    small = jnp.where(big > 0, 0.5 * y / big, 0.0)
    pos = x >= 0
    return jnp.where(pos, big, jnp.abs(small)), jnp.where(pos, small, jnp.where(y < 0, -big, big))


def _make_kernel(S, Dm, H, Dh, M, seg, L, D, N):
    LA = M + seg
    scale = Dh ** (-0.5)
    NC = L // _T
    NB = D // (2 * _CB)
    SG = 17
    DC = Dm // NB
    NG = _CB // 8
    XR = 4
    SPC = _T // seg
    EARLY = 1
    SU = _CB + 1
    SW = Dm // 2 + 1
    NPOW = 11
    HP = H // 2
    PRE = 8
    NPRE = 4
    R = NPRE * SPC * PRE

    def head_row(hd):
        return ((hd % 2) * HP + hd // 2) * SW

    def kernel(x_hbm, mem0_hbm, wq_hbm, wk_hbm, wv_hbm, wo_hbm, u_hbm,
               are_hbm, aim_hbm, bre_hbm, bim_hbm, cre_hbm, cim_hbm, ldt_hbm, dsk_hbm,
               out_hbm,
               x_v, xpre_v, xb_v, zpre_v, mem0_v, wraw_v, wo_v, u_v, par_v, ldt_v, dsk_v, dt_v, dk_v,
               ut_v, yt_v, ya_v, pr_v, pi_v, aux_v,
               o_v, acc_v, out_v,
               sem_par, sem_u, sem_w, sem_wo, sem_x, sem_out, sem_y, *bufs):
        h_v, wf_v, st_v = bufs[:SPC], bufs[SPC:SPC + 3], bufs[SPC + 3:]
        par_hbm = (are_hbm, aim_hbm, bre_hbm, bim_hbm, cre_hbm, cim_hbm)
        head, rest = pl.ds(0, 2 * _CB), pl.ds(2 * _CB, D - 2 * _CB)
        par_head = [pltpu.make_async_copy(par_hbm[i].at[head], par_v.at[i, head], sem_par.at[i]) for i in range(6)]
        par_head.append(pltpu.make_async_copy(ldt_hbm, ldt_v, sem_par.at[6]))
        par_head.append(pltpu.make_async_copy(dsk_hbm, dsk_v, sem_par.at[7]))
        par_rest = [pltpu.make_async_copy(par_hbm[i].at[rest], par_v.at[i, rest], sem_par.at[8 + i]) for i in range(6)]
        mem_cp = pltpu.make_async_copy(mem0_hbm, mem0_v, sem_par.at[14])
        w_hbm = (wq_hbm, wk_hbm, wv_hbm)

        def u_cp(cb):
            return pltpu.make_async_copy(
                u_hbm.at[:, pl.ds(pl.multiple_of(cb * _CB, _CB), _CB)], u_v.at[cb], sem_u.at[cb])

        def w_cp(t, cb):
            rows = pl.ds(pl.multiple_of(cb * (DC * H), DC * H), DC * H)
            return pltpu.make_async_copy(w_hbm[t].at[rows], wraw_v.at[t, rows], sem_w.at[t * NB + cb])

        def wo_cp(j):
            return pltpu.make_async_copy(
                wo_hbm.at[:, pl.ds(pl.multiple_of(j * _LANES, _LANES), _LANES)], wo_v.at[j], sem_wo.at[j])

        def y_cp(sb):
            return pltpu.make_async_copy(yt_v, ya_v.at[sb], sem_y)

        def x_cp(i):
            src = pl.ds(jnp.minimum(i, NC - 1) * SPC, SPC)
            return pltpu.make_async_copy(x_hbm.at[src], x_v.at[i % XR], sem_x.at[i % XR])

        xpre_cp = pltpu.make_async_copy(
            x_hbm.at[pl.ds(0, NPRE * SPC), pl.ds(seg - PRE, PRE)], xpre_v, sem_par.at[15])

        for cp in par_head:
            cp.start()
        u_cp(0).start()
        u_cp(1).start()
        zpre_v[...] = jnp.zeros(zpre_v.shape, _F32)
        for cp in par_head:
            cp.wait()
        for cp in par_rest:
            cp.start()
        mem_cp.start()
        xpre_cp.start()
        for i in range(XR - 1):
            x_cp(i).start()

        dt_all = jnp.exp(ldt_v[...].astype(_F32)).astype(_BF16).astype(_F32).reshape(1, D)
        dk_all = dsk_v[...].astype(_F32).reshape(1, D)
        for cb in range(2 * NB):
            dt_v[cb] = jnp.broadcast_to(dt_all[:, cb * _CB:(cb + 1) * _CB], (8, _CB))
            dk_v[cb] = jnp.broadcast_to(dk_all[:, cb * _CB:(cb + 1) * _CB], (8, _CB))

        flip8 = 7 - lax.broadcasted_iota(jnp.int32, (8, _LANES), 0)
        lane8 = lax.broadcasted_iota(jnp.int32, (8, _LANES), 1)
        sub8 = lax.broadcasted_iota(jnp.int32, (8, _LANES), 0)
        lo_c = lax.broadcasted_iota(jnp.int32, (NC, _LANES), 1) < _T
        first_c = lax.broadcasted_iota(jnp.int32, (NC, _LANES), 0) == 0
        raw32 = wraw_v.bitcast(_U32)
        s_buf = [(st_v[4 * i], st_v[4 * i + 1]) for i in range(NG)]
        z_buf = [(st_v[4 * i + 2], st_v[4 * i + 3]) for i in range(NG)]

        def discretise(sb, g):
            hf = g // (_CB // 16)
            g16 = (g % (_CB // 16)) * 16
            r = pl.ds(pl.multiple_of(g16, 16), 16)
            rg = pl.ds(pl.multiple_of(sb * 2 * _CB + g * 16, 16), 16)
            dt = aux_v[0, hf, r, :]
            a = dt * par_v[0, rg, :].astype(_F32)
            b = dt * par_v[1, rg, :].astype(_F32)
            mag = jnp.exp(a)
            l1 = (mag * jnp.cos(b), mag * jnp.sin(b))
            w = _cmul(par_v[4, rg, :].astype(_F32), par_v[5, rg, :].astype(_F32),
                      dt * par_v[2, rg, :].astype(_F32), dt * par_v[3, rg, :].astype(_F32))
            l2 = _cmul(*l1, *l1)
            l4 = _cmul(*l2, *l2)
            l8 = _cmul(*l4, *l4)
            l16 = _cmul(*l8, *l8)
            l32 = _cmul(*l16, *l16)
            l64 = _cmul(*l32, *l32)
            pw = [_csqrt(*_cmul(*w, *l1))]
            pw.append(_cmul(*pw[0], *l1))
            pw += [_cmul(*q, *l2) for q in pw]
            pw += [_cmul(*q, *l4) for q in pw]
            pw += [l8, l16, l32]
            for j in range(NPOW):
                pr_v[hf, pl.ds(j * SU + g16, 16), :] = pw[j][0]
                pi_v[hf, pl.ds(j * SU + g16, 16), :] = pw[j][1]
            aux_v[1, hf, r, :] = l64[0]
            aux_v[2, hf, r, :] = l64[1]
            aux_v[3, hf, r, :] = jnp.broadcast_to(jnp.sum(w[0], axis=-1, keepdims=True), (16, N))
            aux_v[4, hf, r, :] = pw[0][0]
            aux_v[5, hf, r, :] = -pw[0][1]
            return pw[7][0][8:16]

        def load_u(sb, ck):
            rows = pl.ds(pl.multiple_of(ck * _T, _T), _T)
            fl = []
            for q in range(2):
                tile = u_v[2 * sb + q, rows, :].astype(_F32)
                fl += [jnp.take_along_axis(tile[_T - 8 * (i + 1):_T - 8 * i], flip8, axis=0)
                       for i in range(_T // 8)]
            ut = jnp.concatenate(fl, axis=0).T
            ut_v[pl.ds(ck * SU, _CB), :] = ut
            return ut[_CB - 8:]

        def repack(c):
            nj = DC // 2 // 4

            def body(i, carry):
                j0 = c * (DC // 2) + i * nj
                for t in range(3):
                    src = raw32.at[t, pl.ds(pl.multiple_of(j0 * H, nj * H), nj * H), :]
                    for j in range(nj):
                        for half in range(HP // 8):
                            a = src[pl.ds(j * H + half * 8, 8), :]
                            b = src[pl.ds(j * H + HP + half * 8, 8), :]
                            wf_v[t][pl.ds(j0 + (half * 8 * SW + j), 8, stride=SW), :] = (a & _U32(0xFFFF)) | (b << 16)
                            wf_v[t][pl.ds(j0 + ((HP + half * 8) * SW + j), 8, stride=SW), :] = (
                                (a >> 16) | (b & _U32(0xFFFF0000)))
                return carry
            lax.fori_loop(0, 4, body, 0)

        def project_ahead(c, par):
            lhs = xb_v[c]
            r0 = par * (HP * SW) + c * (DC // 2)
            for t in range(3):
                for k in range(HP):
                    w = wf_v[t][pl.ds(r0 + k * SW, DC // 2), :]
                    zpre_v[par, t * HP + k] += lax.dot_general(
                        lhs, pltpu.bitcast(w, _BF16), _NN, preferred_element_type=_F32)

        def states(p):
            vr, vi = [], []
            for hf in range(2):
                ar = [pr_v[hf, pl.ds(p, 8, stride=SU), :]]
                ai = [pi_v[hf, pl.ds(p, 8, stride=SU), :]]
                for lvl in range(3):
                    mr = jnp.broadcast_to(pr_v[hf, pl.ds((8 + lvl) * SU + p, 1), :], (8, N))
                    mi = jnp.broadcast_to(pi_v[hf, pl.ds((8 + lvl) * SU + p, 1), :], (8, N))
                    for i in range(len(ar)):
                        nr, ni = _cmul(ar[i], ai[i], mr, mi)
                        ar.append(nr)
                        ai.append(ni)
                vr += ar
                vi += ai
            v = jnp.concatenate(
                [jnp.concatenate(vr, axis=0), jnp.concatenate(vi, axis=0)], axis=1).astype(_BF16)
            uf = ut_v[pl.ds(p, NC, stride=SU), :]
            lhs = jnp.concatenate([jnp.where(lo_c, uf, 0.0), jnp.where(lo_c, 0.0, uf)], axis=0)
            st = lax.dot_general(lhs, v, _NN, preferred_element_type=_F32)
            sr, si = s_buf[p // 8]
            for hf in range(2):
                rows = pl.ds(hf * 8 + p % 8, NC, stride=SG)
                sr[rows, :] = st[hf * NC:(hf + 1) * NC, :N]
                si[rows, :] = st[hf * NC:(hf + 1) * NC, N:]
            return v

        def scan(g):
            sr, si = s_buf[g]
            zr, zi = z_buf[g]
            cat = lambda i: jnp.concatenate([aux_v[i, hf, g * 8:(g + 1) * 8, :] for hf in range(2)], axis=0)
            lr, li = cat(1), cat(2)
            zr[0:16, :] = cat(4)
            zi[0:16, :] = cat(5)
            for c in range(1, NC):
                s_r = sr[pl.ds((c - 1) * SG, 16), :]
                s_i = si[pl.ds((c - 1) * SG, 16), :]
                if c == 1:
                    xr, xi = s_r, -s_i
                else:
                    xr, xi = (xr * lr + s_r) + xi * li, (xi * lr - s_i) - xr * li
                zr[pl.ds(c * SG, 16), :] = xr
                zi[pl.ds(c * SG, 16), :] = xi

        def inter(p, v):
            z = [jnp.concatenate([zb[pl.ds(hf * 8 + p % 8, NC, stride=SG), :] for hf in range(2)], axis=0)
                 for zb in z_buf[p // 8]]
            y = lax.dot_general(jnp.concatenate(z, axis=1), v, _NT, preferred_element_type=_F32)
            return jnp.where(lo_c, y[:NC], y[NC:])

        def intra(p, y):
            kk = jnp.broadcast_to(y[0:1, :], (8, _LANES))
            g1 = pltpu.roll(kk, 1, 1, stride=1, stride_axis=0)
            g1 = jnp.where((lane8 & (_T - 1)) > sub8, g1, 0.0)
            g1 = jnp.take_along_axis(g1, flip8, axis=0)
            g0 = jnp.where((lane8 & (_T - 1)) >= 8, pltpu.roll(g1, 8, 1), 0.0)
            top = pltpu.bitcast(jnp.concatenate([g0, g1], axis=0).astype(_BF16), _U32)
            gs = [(i, pltpu.roll(top, 16 * i, 1) if i else top) for i in range(_T // 16 - 1, -1, -1)]
            hs = [jnp.where((lane8 >= 16 * i) & (lane8 < _T), gv, _U32(0)) for i, gv in gs]
            hs += [jnp.where(lane8 >= _T + 16 * i, gv, _U32(0)) for i, gv in gs]
            hk = pltpu.bitcast(jnp.concatenate(hs, axis=0), _BF16)
            rows = pl.ds(p, NC, stride=SU)
            yd = lax.dot_general(ut_v[rows, :], hk, _NN, preferred_element_type=_F32)
            yt_v[rows, :] = jnp.where(first_c, 0.0, y) + yd

        def block(sb, carry):
            @pl.when(sb > 0)
            def _():
                for t in range(3):
                    w_cp(t, sb - 1).wait()

            for t in range(3):
                w_cp(t, sb).start()

            @pl.when(sb < NB - 1)
            def _():
                u_cp(2 * sb + 2).start()
                u_cp(2 * sb + 3).start()

            for hf in range(2):
                aux_v[0, hf] = jnp.broadcast_to(dt_v[2 * sb + hf][0:1, :], (_CB, _CB)).T

            @pl.when(sb == 0)
            def _():
                def modes(i, c):
                    for k in range(4):
                        discretise(0, i * 4 + k)
                    return c
                lax.fori_loop(0, 2 * _CB // 64, modes, 0)
                u_cp(0).wait()
                u_cp(1).wait()

                def chunks(i, c):
                    for k in range(8):
                        load_u(0, i * 8 + k)
                    return c
                lax.fori_loop(0, NC // 8, chunks, 0)
                for cp in par_rest:
                    cp.wait()
                xpre_cp.wait()
                xpre = xpre_v[...].astype(_F32).reshape(R, Dm)
                for c in range(NB):
                    xb_v[c] = xpre[:, c * DC:(c + 1) * DC]

            @pl.when(sb > 0)
            def _():
                repack(sb - 1)
                u_cp(2 * sb).wait()
                u_cp(2 * sb + 1).wait()

                def prepare(i, c):
                    for k in range(_CB // 16):
                        discretise(sb, i * (_CB // 16) + k)
                    for k in range(NC // 2):
                        load_u(sb, i * (NC // 2) + k)
                    project_ahead(sb - 1, i)
                    return c
                lax.fori_loop(0, 2, prepare, 0)

            for hf in range(2):
                dk_v[2 * sb + hf] = dk_v[2 * sb + hf] + aux_v[3, hf].T[0:8]

            vs, ys = {}, {}
            for p in range(_CB):
                vs[p] = states(p)
                if p % 8 == 7 and p // 8 < EARLY:
                    scan(p // 8)
            wo_cp(2 * sb).start()
            wo_cp(2 * sb + 1).start()

            @pl.when(sb > 0)
            def _():
                y_cp(sb - 1).wait()

            for g in range(NG):
                if g + EARLY < NG:
                    scan(g + EARLY)
                for p in range(g * 8, (g + 1) * 8):
                    ys[p] = inter(p, vs.pop(p))
            for p in range(_CB):
                intra(p, ys.pop(p))
            y_cp(sb).start()
            return carry
        lax.fori_loop(0, NB, block, 0)
        for t in range(3):
            w_cp(t, NB - 1).wait()
        repack(NB - 1)
        lax.fori_loop(0, 2, lambda i, c: project_ahead(NB - 1, i), None)

        mem_cp.wait()
        y_cp(NB - 1).wait()
        x_cp(0).wait()
        h_v[0][0:M, :] = mem0_v[...].astype(_F32)
        h_v[0][M:LA, :] = x_v[0, 0].astype(_F32)
        row = lax.broadcasted_iota(jnp.int32, (LA, LA), 0)
        col = lax.broadcasted_iota(jnp.int32, (LA, LA), 1)
        mask = (row < M) | (row >= col)
        wo32 = wo_v.bitcast(_U32)

        def segment(h_in, h_out, dst, side_work, pre_rows):
            def proj(hd):
                h = h_in[...] if pre_rows is None else h_in[0:LA - PRE, :]
                out = [lax.dot_general(h, pltpu.bitcast(wf_v[t][pl.ds(head_row(hd), Dm // 2), :], _BF16), _NN,
                                       preferred_element_type=_F32) for t in range(3)]
                if pre_rows is not None:
                    out = [jnp.concatenate([out[t], zpre_v[hd % 2, t * HP + hd // 2, pre_rows, :]], axis=0) for t in range(3)]
                return out

            qkv, prob = {}, {}

            def scores(hd):
                q, k, _ = qkv[hd]
                sc = lax.dot_general(q, k, _NT, preferred_element_type=_F32) * scale
                sc = jnp.where(mask, sc, -1e9)
                p = jnp.exp(sc - jnp.max(sc, axis=-1, keepdims=True))
                prob[hd] = p / jnp.sum(p, axis=-1, keepdims=True)

            def values(hd):
                o_v[:, hd * Dh:(hd + 1) * Dh] = lax.dot_general(
                    prob[hd], qkv[hd][2], _NN, preferred_element_type=_F32)

            for hd in range(H):
                qkv[hd] = proj(hd)
                if hd >= 1:
                    scores(hd - 1)
                if hd >= 3:
                    values(hd - 3)
                if hd in side_work:
                    side_work[hd]()
            n1 = H - H // 4
            late = [(scores, H - 1), None, (values, H - 3), (values, H - 2), (values, H - 1)]
            o = o_v[:, 0:n1 * Dh]
            for j in range(Dm // _LANES):
                w = pltpu.bitcast(wo32[j, 0:n1 * Dh // 2, :], _BF16)
                acc_v[:, j * _LANES:(j + 1) * _LANES] = lax.dot_general(o, w, _NN, preferred_element_type=_F32)
                if j < len(late) and late[j] is not None:
                    late[j][0](late[j][1])
            o = o_v[:, n1 * Dh:]
            for j in range(Dm // _LANES):
                cols = slice(j * _LANES, (j + 1) * _LANES)
                w = pltpu.bitcast(wo32[j, n1 * Dh // 2:, :], _BF16)
                res = lax.dot_general(o, w, _NN, preferred_element_type=_F32) + acc_v[:, cols]
                h_out[0:M, cols] = res[0:M]
                dst[:, cols] = res[M:].astype(_BF16)

        def out_cp(i):
            rows = pl.ds(pl.multiple_of(i * _T, _T), _T)
            return pltpu.make_async_copy(out_v.at[rows], out_hbm.at[rows], sem_out)

        def chunk(i, carry, ahead):
            rows = pl.ds(pl.multiple_of(i * _T, _T), _T)
            dst = out_v.at[rows]
            x_cp(i + 1).wait()

            def s4_epilogue(sb):
                y = ya_v[sb, pl.ds(i * SU, _CB), :].T
                for q in range(2):
                    cb = 2 * sb + q
                    skip = u_v[cb, rows, :].astype(_F32) * dk_v[cb][0:1, :]
                    dst[:, Dm + cb * _CB:Dm + (cb + 1) * _CB] = (y[q * _T:(q + 1) * _T] + skip).astype(_BF16)

            def next_rows(k):
                if k < SPC:
                    h_v[k][M:LA, :] = x_v[i % XR, k].astype(_F32)
                else:
                    h_v[0][M:LA, :] = x_v[(i + 1) % XR, 0].astype(_F32)

            def traffic():
                x_cp(i + XR - 1).start()

            for k in range(SPC):
                side = {H // 2: functools.partial(next_rows, k + 1)}
                if k == 0:
                    side[2] = traffic
                    for sb in range(NB):
                        side[4 + 2 * sb] = functools.partial(s4_epilogue, sb)
                pre_rows = pl.ds(pl.multiple_of((i * SPC + k) * PRE, PRE), PRE) if ahead else None
                segment(h_v[k], h_v[(k + 1) % SPC], dst.at[pl.ds(k * seg, seg)], side, pre_rows)
            out_cp(i).start()
            return carry

        for j in range(Dm // _LANES):
            wo_cp(j).wait()
        lax.fori_loop(0, NPRE, functools.partial(chunk, ahead=True), 0)
        lax.fori_loop(NPRE, NC, functools.partial(chunk, ahead=False), 0)

        for i in range(NC + 1, NC + XR - 1):
            x_cp(i).wait()
        pltpu.make_async_copy(out_v, out_hbm, sem_out).wait()

    scratch = [
        pltpu.VMEM((XR, SPC, seg, Dm), _BF16),
        pltpu.VMEM((NPRE * SPC, PRE, Dm), _BF16),
        pltpu.VMEM((NB, R, DC), _F32),
        pltpu.VMEM((2, 3 * HP, R, Dh), _F32),
        pltpu.VMEM((M, Dm), _BF16),
        pltpu.VMEM((3, Dm * H, Dh), _BF16),
        pltpu.VMEM((Dm // _LANES, H * Dh, _LANES), _BF16),
        pltpu.VMEM((2 * NB, L, _CB), _BF16),
        pltpu.VMEM((6, D, N), _BF16),
        pltpu.VMEM((D,), _BF16),
        pltpu.VMEM((D,), _BF16),
        pltpu.VMEM((2 * NB, 8, _CB), _F32),
        pltpu.VMEM((2 * NB, 8, _CB), _F32),
        pltpu.VMEM((NC * SU, _LANES), _F32),
        pltpu.VMEM((NC * SU, _LANES), _F32),
        pltpu.VMEM((NB, NC * SU, _LANES), _F32),
        pltpu.VMEM((2, NPOW * SU + 5, N), _F32),
        pltpu.VMEM((2, NPOW * SU + 5, N), _F32),
        pltpu.VMEM((6, 2, _CB, N), _F32),
        pltpu.VMEM((LA, H * Dh), _F32),
        pltpu.VMEM((LA, Dm), _F32),
        pltpu.VMEM((S, Dm + D), _BF16),
        pltpu.SemaphoreType.DMA((16,)),
        pltpu.SemaphoreType.DMA((2 * NB,)),
        pltpu.SemaphoreType.DMA((3 * NB,)),
        pltpu.SemaphoreType.DMA((Dm // _LANES,)),
        pltpu.SemaphoreType.DMA((XR,)),
        pltpu.SemaphoreType.DMA(()),
        pltpu.SemaphoreType.DMA(()),
    ]
    scratch += [pltpu.VMEM((LA, Dm), _F32)] * SPC
    scratch += [pltpu.VMEM((H * SW, Dh), _U32)] * 3
    scratch += [pltpu.VMEM((NC * SG, N), _F32)] * (4 * NG)
    return kernel, scratch


@functools.partial(jax.jit, static_argnames=("A_seg_len",))
def pallas_concat_heads__memory_aug_recurrent_mem_tr__ssm_conv_s4__prompt_kernel(
    A_x: jax.Array,
    A_mem0: jax.Array,
    A_Wq: jax.Array,
    A_Wk: jax.Array,
    A_Wv: jax.Array,
    A_Wo: jax.Array,
    A_seg_len: int,
    B_u: jax.Array,
    B_A_re: jax.Array,
    B_A_im: jax.Array,
    B_B_re: jax.Array,
    B_B_im: jax.Array,
    B_C_re: jax.Array,
    B_C_im: jax.Array,
    B_log_dt: jax.Array,
    B_Dskip: jax.Array,
):
    B, S, Dm = A_x.shape
    H, Dh = A_Wq.shape[1], A_Wq.shape[2]
    M = A_mem0.shape[1]
    seg = int(A_seg_len)
    _, L, D = B_u.shape
    N = B_A_re.shape[1]
    assert B == 1 and S == L and S % seg == 0 and Dh == _LANES and N == _LANES

    kernel, scratch = _make_kernel(S, Dm, H, Dh, M, seg, L, D, N)
    out = pl.pallas_call(
        kernel,
        out_shape=jax.ShapeDtypeStruct((S, Dm + D), _BF16),
        in_specs=[pl.BlockSpec(memory_space=pl.ANY)] * 15,
        out_specs=pl.BlockSpec(memory_space=pl.ANY),
        scratch_shapes=scratch,
        compiler_params=pltpu.CompilerParams(vmem_limit_bytes=120 * 1024 * 1024),
    )(
        A_x.reshape(S // seg, seg, Dm), A_mem0.reshape(M, Dm),
        A_Wq.reshape(Dm * H, Dh), A_Wk.reshape(Dm * H, Dh), A_Wv.reshape(Dm * H, Dh),
        A_Wo.reshape(H * Dh, Dm), B_u.reshape(L, D),
        B_A_re, B_A_im, B_B_re, B_B_im, B_C_re, B_C_im, B_log_dt, B_Dskip,
    )
    return out.reshape(B, S, Dm + D)
```

```python
import functools

import jax
import jax.numpy as jnp
from jax import lax
import jax.experimental.pallas as pl
import jax.experimental.pallas.tpu as pltpu

_NN = (((1,), (0,)), ((), ()))
_NT = (((1,), (1,)), ((), ()))
_LANES = 128
_T = 64
_CB = 128
_F32 = jnp.float32
_BF16 = jnp.bfloat16
_U32 = jnp.uint32


def _cmul(ar, ai, br, bi):
    return ar * br - ai * bi, ar * bi + ai * br


def _csqrt(x, y):
    big = jnp.sqrt(0.5 * (jnp.sqrt(x * x + y * y) + jnp.abs(x)))
    small = jnp.where(big > 0, 0.5 * y / big, 0.0)
    pos = x >= 0
    return jnp.where(pos, big, jnp.abs(small)), jnp.where(pos, small, jnp.where(y < 0, -big, big))


def _make_kernel(S, Dm, H, Dh, M, seg, L, D, N):
    LA = M + seg
    scale = Dh ** (-0.5)
    NC = L // _T
    NB = D // (2 * _CB)
    SG = 17
    DC = Dm // NB
    NG = _CB // 8
    XR = 4
    SPC = _T // seg
    EARLY = 1
    SU = _CB + 1
    SW = Dm // 2 + 1
    NPOW = 11
    HP = H // 2
    WR = H * Dh // (2 * NB)
    PRE = 8
    NPRE = 4
    R = NPRE * SPC * PRE

    def head_row(hd):
        return ((hd % 2) * HP + hd // 2) * SW

    def kernel(x_hbm, mem0_hbm, wq_hbm, wk_hbm, wv_hbm, wo_hbm, u_hbm,
               are_hbm, aim_hbm, bre_hbm, bim_hbm, cre_hbm, cim_hbm, ldt_hbm, dsk_hbm,
               out_hbm,
               x_v, xpre_v, xb_v, zpre_v, mem0_v, wraw_v, wo_v, u_v, par_v, ldt_v, dsk_v, dt_v, dk_v,
               ut_v, yt_v, ya_v, pr_v, pi_v, aux_v,
               o_v, acc_v, out_v,
               sem_par, sem_u, sem_w, sem_wo, sem_x, sem_out, sem_y, *bufs):
        h_v, wf_v, st_v = bufs[:SPC], bufs[SPC:SPC + 3], bufs[SPC + 3:]
        par_hbm = (are_hbm, aim_hbm, bre_hbm, bim_hbm, cre_hbm, cim_hbm)
        vec_cp = [pltpu.make_async_copy(ldt_hbm, ldt_v, sem_par.at[6]),
                  pltpu.make_async_copy(dsk_hbm, dsk_v, sem_par.at[7])]
        mem_cp = pltpu.make_async_copy(mem0_hbm, mem0_v, sem_par.at[8])

        def par_cp(sb):
            rows = pl.ds(pl.multiple_of(sb * 2 * _CB, 2 * _CB), 2 * _CB)
            return [pltpu.make_async_copy(par_hbm[i].at[rows], par_v.at[i, rows], sem_par.at[i]) for i in range(6)]

        w_hbm = (wq_hbm, wk_hbm, wv_hbm)

        def u_cp(cb):
            return pltpu.make_async_copy(
                u_hbm.at[:, pl.ds(pl.multiple_of(cb * _CB, _CB), _CB)], u_v.at[cb], sem_u.at[cb])

        def w_cp(t, cb):
            rows = pl.ds(pl.multiple_of(cb * (DC * H), DC * H), DC * H)
            return pltpu.make_async_copy(w_hbm[t].at[rows], wraw_v.at[t, rows], sem_w.at[t * NB + cb])

        def wo_start(r):
            rows = pl.ds(r * WR if isinstance(r, int) else pl.multiple_of(r * WR, WR), WR)
            for j in range(Dm // _LANES):
                pltpu.make_async_copy(wo_hbm.at[rows, pl.ds(j * _LANES, _LANES)], wo_v.at[j, rows], sem_wo).start()

        def y_cp(sb):
            return pltpu.make_async_copy(yt_v, ya_v.at[sb], sem_y)

        def x_cp(i):
            src = pl.ds(jnp.minimum(i, NC - 1) * SPC, SPC)
            return pltpu.make_async_copy(x_hbm.at[src], x_v.at[i % XR], sem_x.at[i % XR])

        xpre_cp = pltpu.make_async_copy(
            x_hbm.at[pl.ds(0, NPRE * SPC), pl.ds(seg - PRE, PRE)], xpre_v, sem_par.at[9])

        for cp in par_cp(0) + vec_cp:
            cp.start()
        u_cp(0).start()
        u_cp(1).start()
        zpre_v[...] = jnp.zeros(zpre_v.shape, _F32)
        for cp in par_cp(0) + vec_cp:
            cp.wait()
        xpre_cp.start()

        dt_all = jnp.exp(ldt_v[...].astype(_F32)).astype(_BF16).astype(_F32).reshape(1, D)
        dk_all = dsk_v[...].astype(_F32).reshape(1, D)
        for cb in range(2 * NB):
            dt_v[cb] = jnp.broadcast_to(dt_all[:, cb * _CB:(cb + 1) * _CB], (8, _CB))
            dk_v[cb] = jnp.broadcast_to(dk_all[:, cb * _CB:(cb + 1) * _CB], (8, _CB))

        flip8 = 7 - lax.broadcasted_iota(jnp.int32, (8, _LANES), 0)
        lane8 = lax.broadcasted_iota(jnp.int32, (8, _LANES), 1)
        sub8 = lax.broadcasted_iota(jnp.int32, (8, _LANES), 0)
        lo_c = lax.broadcasted_iota(jnp.int32, (NC, _LANES), 1) < _T
        first_c = lax.broadcasted_iota(jnp.int32, (NC, _LANES), 0) == 0
        raw32 = wraw_v.bitcast(_U32)
        s_buf = [(st_v[4 * i], st_v[4 * i + 1]) for i in range(NG)]
        z_buf = [(st_v[4 * i + 2], st_v[4 * i + 3]) for i in range(NG)]

        def discretise(sb, g):
            hf = g // (_CB // 16)
            g16 = (g % (_CB // 16)) * 16
            r = pl.ds(pl.multiple_of(g16, 16), 16)
            rg = pl.ds(pl.multiple_of(sb * 2 * _CB + g * 16, 16), 16)
            dt = aux_v[0, hf, r, :]
            a = dt * par_v[0, rg, :].astype(_F32)
            b = dt * par_v[1, rg, :].astype(_F32)
            mag = jnp.exp(a)
            l1 = (mag * jnp.cos(b), mag * jnp.sin(b))
            w = _cmul(par_v[4, rg, :].astype(_F32), par_v[5, rg, :].astype(_F32),
                      dt * par_v[2, rg, :].astype(_F32), dt * par_v[3, rg, :].astype(_F32))
            l2 = _cmul(*l1, *l1)
            l4 = _cmul(*l2, *l2)
            l8 = _cmul(*l4, *l4)
            l16 = _cmul(*l8, *l8)
            l32 = _cmul(*l16, *l16)
            l64 = _cmul(*l32, *l32)
            pw = [_csqrt(*_cmul(*w, *l1))]
            pw.append(_cmul(*pw[0], *l1))
            pw += [_cmul(*q, *l2) for q in pw]
            pw += [_cmul(*q, *l4) for q in pw]
            pw += [l8, l16, l32]
            for j in range(NPOW):
                pr_v[hf, pl.ds(j * SU + g16, 16), :] = pw[j][0]
                pi_v[hf, pl.ds(j * SU + g16, 16), :] = pw[j][1]
            aux_v[1, hf, r, :] = l64[0]
            aux_v[2, hf, r, :] = l64[1]
            aux_v[3, hf, r, :] = jnp.broadcast_to(jnp.sum(w[0], axis=-1, keepdims=True), (16, N))
            aux_v[4, hf, r, :] = pw[0][0]
            aux_v[5, hf, r, :] = -pw[0][1]
            return pw[7][0][8:16]

        def load_u(sb, ck):
            rows = pl.ds(pl.multiple_of(ck * _T, _T), _T)
            fl = []
            for q in range(2):
                tile = u_v[2 * sb + q, rows, :].astype(_F32)
                fl += [jnp.take_along_axis(tile[_T - 8 * (i + 1):_T - 8 * i], flip8, axis=0)
                       for i in range(_T // 8)]
            ut = jnp.concatenate(fl, axis=0).T
            ut_v[pl.ds(ck * SU, _CB), :] = ut
            return ut[_CB - 8:]

        def repack(c):
            nj = DC // 2 // 4

            def body(i, carry):
                j0 = c * (DC // 2) + i * nj
                for t in range(3):
                    src = raw32.at[t, pl.ds(pl.multiple_of(j0 * H, nj * H), nj * H), :]
                    for j in range(nj):
                        for half in range(HP // 8):
                            a = src[pl.ds(j * H + half * 8, 8), :]
                            b = src[pl.ds(j * H + HP + half * 8, 8), :]
                            wf_v[t][pl.ds(j0 + (half * 8 * SW + j), 8, stride=SW), :] = (a & _U32(0xFFFF)) | (b << 16)
                            wf_v[t][pl.ds(j0 + ((HP + half * 8) * SW + j), 8, stride=SW), :] = (
                                (a >> 16) | (b & _U32(0xFFFF0000)))
                return carry
            lax.fori_loop(0, 4, body, 0)

        def project_ahead(c, par):
            lhs = xb_v[c]
            r0 = par * (HP * SW) + c * (DC // 2)
            for t in range(3):
                for k in range(HP):
                    w = wf_v[t][pl.ds(r0 + k * SW, DC // 2), :]
                    zpre_v[par, t * HP + k] += lax.dot_general(
                        lhs, pltpu.bitcast(w, _BF16), _NN, preferred_element_type=_F32)

        def states(p):
            vr, vi = [], []
            for hf in range(2):
                ar = [pr_v[hf, pl.ds(p, 8, stride=SU), :]]
                ai = [pi_v[hf, pl.ds(p, 8, stride=SU), :]]
                for lvl in range(3):
                    mr = jnp.broadcast_to(pr_v[hf, pl.ds((8 + lvl) * SU + p, 1), :], (8, N))
                    mi = jnp.broadcast_to(pi_v[hf, pl.ds((8 + lvl) * SU + p, 1), :], (8, N))
                    for i in range(len(ar)):
                        nr, ni = _cmul(ar[i], ai[i], mr, mi)
                        ar.append(nr)
                        ai.append(ni)
                vr += ar
                vi += ai
            v = jnp.concatenate(
                [jnp.concatenate(vr, axis=0), jnp.concatenate(vi, axis=0)], axis=1).astype(_BF16)
            uf = ut_v[pl.ds(p, NC, stride=SU), :]
            lhs = jnp.concatenate([jnp.where(lo_c, uf, 0.0), jnp.where(lo_c, 0.0, uf)], axis=0)
            st = lax.dot_general(lhs, v, _NN, preferred_element_type=_F32)
            sr, si = s_buf[p // 8]
            for hf in range(2):
                rows = pl.ds(hf * 8 + p % 8, NC, stride=SG)
                sr[rows, :] = st[hf * NC:(hf + 1) * NC, :N]
                si[rows, :] = st[hf * NC:(hf + 1) * NC, N:]
            return v

        def scan(g):
            sr, si = s_buf[g]
            zr, zi = z_buf[g]
            cat = lambda i: jnp.concatenate([aux_v[i, hf, g * 8:(g + 1) * 8, :] for hf in range(2)], axis=0)
            lr, li = cat(1), cat(2)
            zr[0:16, :] = cat(4)
            zi[0:16, :] = cat(5)
            for c in range(1, NC):
                s_r = sr[pl.ds((c - 1) * SG, 16), :]
                s_i = si[pl.ds((c - 1) * SG, 16), :]
                if c == 1:
                    xr, xi = s_r, -s_i
                else:
                    xr, xi = (xr * lr + s_r) + xi * li, (xi * lr - s_i) - xr * li
                zr[pl.ds(c * SG, 16), :] = xr
                zi[pl.ds(c * SG, 16), :] = xi

        def inter(p, v):
            z = [jnp.concatenate([zb[pl.ds(hf * 8 + p % 8, NC, stride=SG), :] for hf in range(2)], axis=0)
                 for zb in z_buf[p // 8]]
            y = lax.dot_general(jnp.concatenate(z, axis=1), v, _NT, preferred_element_type=_F32)
            return jnp.where(lo_c, y[:NC], y[NC:])

        def intra(p, y):
            kk = jnp.broadcast_to(y[0:1, :], (8, _LANES))
            g1 = pltpu.roll(kk, 1, 1, stride=1, stride_axis=0)
            g1 = jnp.where((lane8 & (_T - 1)) > sub8, g1, 0.0)
            g1 = jnp.take_along_axis(g1, flip8, axis=0)
            g0 = jnp.where((lane8 & (_T - 1)) >= 8, pltpu.roll(g1, 8, 1), 0.0)
            top = pltpu.bitcast(jnp.concatenate([g0, g1], axis=0).astype(_BF16), _U32)
            gs = [(i, pltpu.roll(top, 16 * i, 1) if i else top) for i in range(_T // 16 - 1, -1, -1)]
            hs = [jnp.where((lane8 >= 16 * i) & (lane8 < _T), gv, _U32(0)) for i, gv in gs]
            hs += [jnp.where(lane8 >= _T + 16 * i, gv, _U32(0)) for i, gv in gs]
            hk = pltpu.bitcast(jnp.concatenate(hs, axis=0), _BF16)
            rows = pl.ds(p, NC, stride=SU)
            yd = lax.dot_general(ut_v[rows, :], hk, _NN, preferred_element_type=_F32)
            yt_v[rows, :] = jnp.where(first_c, 0.0, y) + yd

        def block(sb, carry):
            @pl.when(sb > 0)
            def _():
                for t in range(3):
                    w_cp(t, sb - 1).wait()

            for t in range(3):
                w_cp(t, sb).start()

            @pl.when(sb < NB - 1)
            def _():
                for cp in par_cp(sb + 1) + [u_cp(2 * sb + 2), u_cp(2 * sb + 3)]:
                    cp.start()

            @pl.when(sb == NB - 1)
            def _():
                for cp in [mem_cp] + [x_cp(i) for i in range(XR - 1)]:
                    cp.start()

            for hf in range(2):
                aux_v[0, hf] = jnp.broadcast_to(dt_v[2 * sb + hf][0:1, :], (_CB, _CB)).T

            @pl.when(sb == 0)
            def _():
                def modes(i, c, with_u):
                    for k in range(4):
                        discretise(0, i * 4 + k)
                    for k in range(NC // 2 if with_u else 0):
                        load_u(0, (i - 2) * (NC // 2) + k)
                    return c
                lax.fori_loop(0, 2, functools.partial(modes, with_u=False), 0)
                u_cp(0).wait()
                u_cp(1).wait()
                lax.fori_loop(2, 4, functools.partial(modes, with_u=True), 0)
                xpre_cp.wait()
                xpre = xpre_v[...].astype(_F32).reshape(R, Dm)
                for c in range(NB):
                    xb_v[c] = xpre[:, c * DC:(c + 1) * DC]

            @pl.when(sb > 0)
            def _():
                repack(sb - 1)
                for cp in par_cp(sb) + [u_cp(2 * sb), u_cp(2 * sb + 1)]:
                    cp.wait()

                def prepare(i, c):
                    for k in range(_CB // 16):
                        discretise(sb, i * (_CB // 16) + k)
                    for k in range(NC // 2):
                        load_u(sb, i * (NC // 2) + k)
                    project_ahead(sb - 1, i)
                    return c
                lax.fori_loop(0, 2, prepare, 0)

            for hf in range(2):
                dk_v[2 * sb + hf] = dk_v[2 * sb + hf] + aux_v[3, hf].T[0:8]

            vs, ys = {}, {}
            for p in range(_CB):
                vs[p] = states(p)
                if p % 8 == 7 and p // 8 < EARLY:
                    scan(p // 8)

            @pl.when(sb > 0)
            def _():
                y_cp(sb - 1).wait()
                wo_start(2 * sb - 1)

            wo_start(2 * sb)

            @pl.when(sb == NB - 1)
            def _():
                wo_start(2 * NB - 1)

            for g in range(NG):
                if g + EARLY < NG:
                    scan(g + EARLY)
                for p in range(g * 8, (g + 1) * 8):
                    ys[p] = inter(p, vs.pop(p))
            for p in range(_CB):
                intra(p, ys.pop(p))
            y_cp(sb).start()
            return carry
        lax.fori_loop(0, NB, block, 0)
        for t in range(3):
            w_cp(t, NB - 1).wait()
        repack(NB - 1)
        lax.fori_loop(0, 2, lambda i, c: project_ahead(NB - 1, i), None)

        mem_cp.wait()
        y_cp(NB - 1).wait()
        x_cp(0).wait()
        h_v[0][0:M, :] = mem0_v[...].astype(_F32)
        h_v[0][M:LA, :] = x_v[0, 0].astype(_F32)
        row = lax.broadcasted_iota(jnp.int32, (LA, LA), 0)
        col = lax.broadcasted_iota(jnp.int32, (LA, LA), 1)
        mask = (row < M) | (row >= col)
        wo32 = wo_v.bitcast(_U32)

        def segment(h_in, h_out, dst, side_work, pre_rows):
            def proj(hd):
                h = h_in[...] if pre_rows is None else h_in[0:LA - PRE, :]
                out = [lax.dot_general(h, pltpu.bitcast(wf_v[t][pl.ds(head_row(hd), Dm // 2), :], _BF16), _NN,
                                       preferred_element_type=_F32) for t in range(3)]
                if pre_rows is not None:
                    out = [jnp.concatenate([out[t], zpre_v[hd % 2, t * HP + hd // 2, pre_rows, :]], axis=0) for t in range(3)]
                return out

            qkv, prob = {}, {}

            def scores(hd):
                q, k, _ = qkv[hd]
                sc = lax.dot_general(q, k, _NT, preferred_element_type=_F32) * scale
                sc = jnp.where(mask, sc, -1e9)
                p = jnp.exp(sc - jnp.max(sc, axis=-1, keepdims=True))
                prob[hd] = p / jnp.sum(p, axis=-1, keepdims=True)

            def values(hd):
                o_v[:, hd * Dh:(hd + 1) * Dh] = lax.dot_general(
                    prob[hd], qkv[hd][2], _NN, preferred_element_type=_F32)

            for hd in range(H):
                qkv[hd] = proj(hd)
                if hd >= 1:
                    scores(hd - 1)
                if hd >= 3:
                    values(hd - 3)
                if hd in side_work:
                    side_work[hd]()
            n1 = H - H // 4
            late = [(scores, H - 1), None, (values, H - 3), (values, H - 2), (values, H - 1)]
            o = o_v[:, 0:n1 * Dh]
            for j in range(Dm // _LANES):
                w = pltpu.bitcast(wo32[j, 0:n1 * Dh // 2, :], _BF16)
                acc_v[:, j * _LANES:(j + 1) * _LANES] = lax.dot_general(o, w, _NN, preferred_element_type=_F32)
                if j < len(late) and late[j] is not None:
                    late[j][0](late[j][1])
            o = o_v[:, n1 * Dh:]
            for j in range(Dm // _LANES):
                cols = slice(j * _LANES, (j + 1) * _LANES)
                w = pltpu.bitcast(wo32[j, n1 * Dh // 2:, :], _BF16)
                res = lax.dot_general(o, w, _NN, preferred_element_type=_F32) + acc_v[:, cols]
                h_out[0:M, cols] = res[0:M]
                dst[:, cols] = res[M:].astype(_BF16)

        def out_cp(i):
            rows = pl.ds(pl.multiple_of(i * _T, _T), _T)
            return pltpu.make_async_copy(out_v.at[rows], out_hbm.at[rows], sem_out)

        def chunk(i, carry, ahead):
            rows = pl.ds(pl.multiple_of(i * _T, _T), _T)
            dst = out_v.at[rows]
            x_cp(i + 1).wait()

            def s4_epilogue(sb):
                y = ya_v[sb, pl.ds(i * SU, _CB), :].T
                for q in range(2):
                    cb = 2 * sb + q
                    skip = u_v[cb, rows, :].astype(_F32) * dk_v[cb][0:1, :]
                    dst[:, Dm + cb * _CB:Dm + (cb + 1) * _CB] = (y[q * _T:(q + 1) * _T] + skip).astype(_BF16)

            def next_rows(k):
                if k < SPC:
                    h_v[k][M:LA, :] = x_v[i % XR, k].astype(_F32)
                else:
                    h_v[0][M:LA, :] = x_v[(i + 1) % XR, 0].astype(_F32)

            def traffic():
                x_cp(i + XR - 1).start()

            for k in range(SPC):
                side = {H // 2: functools.partial(next_rows, k + 1)}
                if k == 0:
                    side[2] = traffic
                    for sb in range(NB):
                        side[4 + 2 * sb] = functools.partial(s4_epilogue, sb)
                pre_rows = pl.ds(pl.multiple_of((i * SPC + k) * PRE, PRE), PRE) if ahead else None
                segment(h_v[k], h_v[(k + 1) % SPC], dst.at[pl.ds(k * seg, seg)], side, pre_rows)
            out_cp(i).start()
            return carry

        pltpu.make_async_copy(wo_v, wo_v, sem_wo).wait()
        lax.fori_loop(0, NPRE, functools.partial(chunk, ahead=True), 0)
        lax.fori_loop(NPRE, NC, functools.partial(chunk, ahead=False), 0)

        for i in range(NC + 1, NC + XR - 1):
            x_cp(i).wait()
        pltpu.make_async_copy(out_v, out_hbm, sem_out).wait()

    scratch = [
        pltpu.VMEM((XR, SPC, seg, Dm), _BF16),
        pltpu.VMEM((NPRE * SPC, PRE, Dm), _BF16),
        pltpu.VMEM((NB, R, DC), _F32),
        pltpu.VMEM((2, 3 * HP, R, Dh), _F32),
        pltpu.VMEM((M, Dm), _BF16),
        pltpu.VMEM((3, Dm * H, Dh), _BF16),
        pltpu.VMEM((Dm // _LANES, H * Dh, _LANES), _BF16),
        pltpu.VMEM((2 * NB, L, _CB), _BF16),
        pltpu.VMEM((6, D, N), _BF16),
        pltpu.VMEM((D,), _BF16),
        pltpu.VMEM((D,), _BF16),
        pltpu.VMEM((2 * NB, 8, _CB), _F32),
        pltpu.VMEM((2 * NB, 8, _CB), _F32),
        pltpu.VMEM((NC * SU, _LANES), _F32),
        pltpu.VMEM((NC * SU, _LANES), _F32),
        pltpu.VMEM((NB, NC * SU, _LANES), _F32),
        pltpu.VMEM((2, NPOW * SU + 5, N), _F32),
        pltpu.VMEM((2, NPOW * SU + 5, N), _F32),
        pltpu.VMEM((6, 2, _CB, N), _F32),
        pltpu.VMEM((LA, H * Dh), _F32),
        pltpu.VMEM((LA, Dm), _F32),
        pltpu.VMEM((S, Dm + D), _BF16),
        pltpu.SemaphoreType.DMA((10,)),
        pltpu.SemaphoreType.DMA((2 * NB,)),
        pltpu.SemaphoreType.DMA((3 * NB,)),
        pltpu.SemaphoreType.DMA(()),
        pltpu.SemaphoreType.DMA((XR,)),
        pltpu.SemaphoreType.DMA(()),
        pltpu.SemaphoreType.DMA(()),
    ]
    scratch += [pltpu.VMEM((LA, Dm), _F32)] * SPC
    scratch += [pltpu.VMEM((H * SW, Dh), _U32)] * 3
    scratch += [pltpu.VMEM((NC * SG, N), _F32)] * (4 * NG)
    return kernel, scratch


@functools.partial(jax.jit, static_argnames=("A_seg_len",))
def pallas_concat_heads__memory_aug_recurrent_mem_tr__ssm_conv_s4__prompt_kernel(
    A_x: jax.Array,
    A_mem0: jax.Array,
    A_Wq: jax.Array,
    A_Wk: jax.Array,
    A_Wv: jax.Array,
    A_Wo: jax.Array,
    A_seg_len: int,
    B_u: jax.Array,
    B_A_re: jax.Array,
    B_A_im: jax.Array,
    B_B_re: jax.Array,
    B_B_im: jax.Array,
    B_C_re: jax.Array,
    B_C_im: jax.Array,
    B_log_dt: jax.Array,
    B_Dskip: jax.Array,
):
    B, S, Dm = A_x.shape
    H, Dh = A_Wq.shape[1], A_Wq.shape[2]
    M = A_mem0.shape[1]
    seg = int(A_seg_len)
    _, L, D = B_u.shape
    N = B_A_re.shape[1]
    assert B == 1 and S == L and S % seg == 0 and Dh == _LANES and N == _LANES

    kernel, scratch = _make_kernel(S, Dm, H, Dh, M, seg, L, D, N)
    out = pl.pallas_call(
        kernel,
        out_shape=jax.ShapeDtypeStruct((S, Dm + D), _BF16),
        in_specs=[pl.BlockSpec(memory_space=pl.ANY)] * 15,
        out_specs=pl.BlockSpec(memory_space=pl.ANY),
        scratch_shapes=scratch,
        compiler_params=pltpu.CompilerParams(vmem_limit_bytes=120 * 1024 * 1024),
    )(
        A_x.reshape(S // seg, seg, Dm), A_mem0.reshape(M, Dm),
        A_Wq.reshape(Dm * H, Dh), A_Wk.reshape(Dm * H, Dh), A_Wv.reshape(Dm * H, Dh),
        A_Wo.reshape(H * Dh, Dm), B_u.reshape(L, D),
        B_A_re, B_A_im, B_B_re, B_B_im, B_C_re, B_C_im, B_log_dt, B_Dskip,
    )
    return out.reshape(B, S, Dm + D)
```

```python
import functools

import jax
import jax.numpy as jnp
from jax import lax
import jax.experimental.pallas as pl
import jax.experimental.pallas.tpu as pltpu

_NN = (((1,), (0,)), ((), ()))
_NT = (((1,), (1,)), ((), ()))
_LANES = 128
_T = 64
_CB = 128
_F32 = jnp.float32
_BF16 = jnp.bfloat16
_U32 = jnp.uint32


def _cmul(ar, ai, br, bi):
    return ar * br - ai * bi, ar * bi + ai * br


def _csqrt(x, y):
    big = jnp.sqrt(0.5 * (jnp.sqrt(x * x + y * y) + jnp.abs(x)))
    small = jnp.where(big > 0, 0.5 * y / big, 0.0)
    pos = x >= 0
    return jnp.where(pos, big, jnp.abs(small)), jnp.where(pos, small, jnp.where(y < 0, -big, big))


def _make_kernel(S, Dm, H, Dh, M, seg, L, D, N):
    LA = M + seg
    scale = Dh ** (-0.5)
    NC = L // _T
    NB = D // (2 * _CB)
    SG = 17
    DC = Dm // NB
    NG = _CB // 8
    XR = 4
    SPC = _T // seg
    EARLY = 1
    SU = _CB + 1
    SW = Dm // 2 + 1
    NPOW = 11
    HP = H // 2
    WR = H * Dh // (2 * NB)
    PRE = 8
    NPRE = 5
    R = NPRE * SPC * PRE

    def head_row(hd):
        return ((hd % 2) * HP + hd // 2) * SW

    def kernel(x_hbm, mem0_hbm, wq_hbm, wk_hbm, wv_hbm, wo_hbm, u_hbm,
               are_hbm, aim_hbm, bre_hbm, bim_hbm, cre_hbm, cim_hbm, ldt_hbm, dsk_hbm,
               out_hbm,
               x_v, xpre_v, xb_v, zpre_v, mem0_v, wraw_v, wo_v, u_v, par_v, ldt_v, dsk_v, dt_v, dk_v,
               ut_v, yt_v, ya_v, pr_v, pi_v, aux_v,
               o_v, acc_v, out_v,
               sem_par, sem_misc, sem_u, sem_w, sem_wo, sem_x, sem_out, sem_y, *bufs):
        h_v, wf_v, st_v = bufs[:SPC], bufs[SPC:SPC + 3], bufs[SPC + 3:]
        par_hbm = (are_hbm, aim_hbm, bre_hbm, bim_hbm, cre_hbm, cim_hbm)
        vec_cp = [pltpu.make_async_copy(ldt_hbm, ldt_v, sem_misc.at[0]),
                  pltpu.make_async_copy(dsk_hbm, dsk_v, sem_misc.at[1])]
        mem_cp = pltpu.make_async_copy(mem0_hbm, mem0_v, sem_misc.at[2])

        def par_cp(sb):
            rows = pl.ds(pl.multiple_of(sb * 2 * _CB, 2 * _CB), 2 * _CB)
            return [pltpu.make_async_copy(par_hbm[i].at[rows], par_v.at[i, rows], sem_par.at[sb * 6 + i])
                    for i in range(6)]

        w_hbm = (wq_hbm, wk_hbm, wv_hbm)

        def u_cp(cb):
            return pltpu.make_async_copy(
                u_hbm.at[:, pl.ds(pl.multiple_of(cb * _CB, _CB), _CB)], u_v.at[cb], sem_u.at[cb])

        def w_cp(t, cb):
            rows = pl.ds(pl.multiple_of(cb * (DC * H), DC * H), DC * H)
            return pltpu.make_async_copy(w_hbm[t].at[rows], wraw_v.at[t, rows], sem_w.at[t * NB + cb])

        def wo_start(r):
            rows = pl.ds(r * WR if isinstance(r, int) else pl.multiple_of(r * WR, WR), WR)
            for j in range(Dm // _LANES):
                pltpu.make_async_copy(wo_hbm.at[rows, pl.ds(j * _LANES, _LANES)], wo_v.at[j, rows], sem_wo).start()

        def y_cp(sb):
            return pltpu.make_async_copy(yt_v, ya_v.at[sb], sem_y)

        def x_cp(i):
            src = pl.ds(jnp.minimum(i, NC - 1) * SPC, SPC)
            return pltpu.make_async_copy(x_hbm.at[src], x_v.at[i % XR], sem_x.at[i % XR])

        xpre_cp = pltpu.make_async_copy(
            x_hbm.at[pl.ds(0, NPRE * SPC), pl.ds(seg - PRE, PRE)], xpre_v, sem_misc.at[3])

        for cp in par_cp(0) + vec_cp:
            cp.start()
        u_cp(0).start()
        u_cp(1).start()
        zpre_v[...] = jnp.zeros(zpre_v.shape, _F32)
        for cp in par_cp(0) + vec_cp:
            cp.wait()
        xpre_cp.start()

        dt_all = jnp.exp(ldt_v[...].astype(_F32)).astype(_BF16).astype(_F32).reshape(1, D)
        dk_all = dsk_v[...].astype(_F32).reshape(1, D)
        for cb in range(2 * NB):
            dt_v[cb] = jnp.broadcast_to(dt_all[:, cb * _CB:(cb + 1) * _CB], (8, _CB))
            dk_v[cb] = jnp.broadcast_to(dk_all[:, cb * _CB:(cb + 1) * _CB], (8, _CB))

        flip8 = 7 - lax.broadcasted_iota(jnp.int32, (8, _LANES), 0)
        lane8 = lax.broadcasted_iota(jnp.int32, (8, _LANES), 1)
        sub8 = lax.broadcasted_iota(jnp.int32, (8, _LANES), 0)
        lo_c = lax.broadcasted_iota(jnp.int32, (NC, _LANES), 1) < _T
        first_c = lax.broadcasted_iota(jnp.int32, (NC, _LANES), 0) == 0
        raw32 = wraw_v.bitcast(_U32)
        s_buf = [(st_v[4 * i], st_v[4 * i + 1]) for i in range(NG)]
        z_buf = [(st_v[4 * i + 2], st_v[4 * i + 3]) for i in range(NG)]

        def discretise(sb, g):
            hf = g // (_CB // 16)
            g16 = (g % (_CB // 16)) * 16
            r = pl.ds(pl.multiple_of(g16, 16), 16)
            rg = pl.ds(pl.multiple_of(sb * 2 * _CB + g * 16, 16), 16)
            dt = aux_v[0, hf, r, :]
            a = dt * par_v[0, rg, :].astype(_F32)
            b = dt * par_v[1, rg, :].astype(_F32)
            mag = jnp.exp(a)
            l1 = (mag * jnp.cos(b), mag * jnp.sin(b))
            w = _cmul(par_v[4, rg, :].astype(_F32), par_v[5, rg, :].astype(_F32),
                      dt * par_v[2, rg, :].astype(_F32), dt * par_v[3, rg, :].astype(_F32))
            l2 = _cmul(*l1, *l1)
            l4 = _cmul(*l2, *l2)
            l8 = _cmul(*l4, *l4)
            l16 = _cmul(*l8, *l8)
            l32 = _cmul(*l16, *l16)
            l64 = _cmul(*l32, *l32)
            pw = [_csqrt(*_cmul(*w, *l1))]
            pw.append(_cmul(*pw[0], *l1))
            pw += [_cmul(*q, *l2) for q in pw]
            pw += [_cmul(*q, *l4) for q in pw]
            pw += [l8, l16, l32]
            for j in range(NPOW):
                pr_v[hf, pl.ds(j * SU + g16, 16), :] = pw[j][0]
                pi_v[hf, pl.ds(j * SU + g16, 16), :] = pw[j][1]
            aux_v[1, hf, r, :] = l64[0]
            aux_v[2, hf, r, :] = l64[1]
            aux_v[3, hf, r, :] = jnp.broadcast_to(jnp.sum(w[0], axis=-1, keepdims=True), (16, N))
            aux_v[4, hf, r, :] = pw[0][0]
            aux_v[5, hf, r, :] = -pw[0][1]
            return pw[7][0][8:16]

        def load_u(sb, ck):
            rows = pl.ds(pl.multiple_of(ck * _T, _T), _T)
            fl = []
            for q in range(2):
                tile = u_v[2 * sb + q, rows, :].astype(_F32)
                fl += [jnp.take_along_axis(tile[_T - 8 * (i + 1):_T - 8 * i], flip8, axis=0)
                       for i in range(_T // 8)]
            ut = jnp.concatenate(fl, axis=0).T
            ut_v[pl.ds(ck * SU, _CB), :] = ut
            return ut[_CB - 8:]

        def repack(c):
            nj = DC // 2 // 4

            def body(i, carry):
                j0 = c * (DC // 2) + i * nj
                for t in range(3):
                    src = raw32.at[t, pl.ds(pl.multiple_of(j0 * H, nj * H), nj * H), :]
                    for j in range(nj):
                        for half in range(HP // 8):
                            a = src[pl.ds(j * H + half * 8, 8), :]
                            b = src[pl.ds(j * H + HP + half * 8, 8), :]
                            wf_v[t][pl.ds(j0 + (half * 8 * SW + j), 8, stride=SW), :] = (a & _U32(0xFFFF)) | (b << 16)
                            wf_v[t][pl.ds(j0 + ((HP + half * 8) * SW + j), 8, stride=SW), :] = (
                                (a >> 16) | (b & _U32(0xFFFF0000)))
                return carry
            lax.fori_loop(0, 4, body, 0)

        def project_ahead(c, par):
            lhs = xb_v[c]
            r0 = par * (HP * SW) + c * (DC // 2)
            for t in range(3):
                for k in range(HP):
                    w = wf_v[t][pl.ds(r0 + k * SW, DC // 2), :]
                    zpre_v[par, t * HP + k] += lax.dot_general(
                        lhs, pltpu.bitcast(w, _BF16), _NN, preferred_element_type=_F32)

        def states(p):
            vr, vi = [], []
            for hf in range(2):
                ar = [pr_v[hf, pl.ds(p, 8, stride=SU), :]]
                ai = [pi_v[hf, pl.ds(p, 8, stride=SU), :]]
                for lvl in range(3):
                    mr = jnp.broadcast_to(pr_v[hf, pl.ds((8 + lvl) * SU + p, 1), :], (8, N))
                    mi = jnp.broadcast_to(pi_v[hf, pl.ds((8 + lvl) * SU + p, 1), :], (8, N))
                    for i in range(len(ar)):
                        nr, ni = _cmul(ar[i], ai[i], mr, mi)
                        ar.append(nr)
                        ai.append(ni)
                vr += ar
                vi += ai
            v = jnp.concatenate(
                [jnp.concatenate(vr, axis=0), jnp.concatenate(vi, axis=0)], axis=1).astype(_BF16)
            uf = ut_v[pl.ds(p, NC, stride=SU), :]
            lhs = jnp.concatenate([jnp.where(lo_c, uf, 0.0), jnp.where(lo_c, 0.0, uf)], axis=0)
            st = lax.dot_general(lhs, v, _NN, preferred_element_type=_F32)
            sr, si = s_buf[p // 8]
            for hf in range(2):
                rows = pl.ds(hf * 8 + p % 8, NC, stride=SG)
                sr[rows, :] = st[hf * NC:(hf + 1) * NC, :N]
                si[rows, :] = st[hf * NC:(hf + 1) * NC, N:]
            return v

        def scan(g):
            sr, si = s_buf[g]
            zr, zi = z_buf[g]
            cat = lambda i: jnp.concatenate([aux_v[i, hf, g * 8:(g + 1) * 8, :] for hf in range(2)], axis=0)
            lr, li = cat(1), cat(2)
            zr[0:16, :] = cat(4)
            zi[0:16, :] = cat(5)
            for c in range(1, NC):
                s_r = sr[pl.ds((c - 1) * SG, 16), :]
                s_i = si[pl.ds((c - 1) * SG, 16), :]
                if c == 1:
                    xr, xi = s_r, -s_i
                else:
                    xr, xi = (xr * lr + s_r) + xi * li, (xi * lr - s_i) - xr * li
                zr[pl.ds(c * SG, 16), :] = xr
                zi[pl.ds(c * SG, 16), :] = xi

        def inter(p, v):
            z = [jnp.concatenate([zb[pl.ds(hf * 8 + p % 8, NC, stride=SG), :] for hf in range(2)], axis=0)
                 for zb in z_buf[p // 8]]
            y = lax.dot_general(jnp.concatenate(z, axis=1), v, _NT, preferred_element_type=_F32)
            return jnp.where(lo_c, y[:NC], y[NC:])

        def intra(p, y):
            kk = jnp.broadcast_to(y[0:1, :], (8, _LANES))
            g1 = pltpu.roll(kk, 1, 1, stride=1, stride_axis=0)
            g1 = jnp.where((lane8 & (_T - 1)) > sub8, g1, 0.0)
            g1 = jnp.take_along_axis(g1, flip8, axis=0)
            g0 = jnp.where((lane8 & (_T - 1)) >= 8, pltpu.roll(g1, 8, 1), 0.0)
            top = pltpu.bitcast(jnp.concatenate([g0, g1], axis=0).astype(_BF16), _U32)
            gs = [(i, pltpu.roll(top, 16 * i, 1) if i else top) for i in range(_T // 16 - 1, -1, -1)]
            hs = [jnp.where((lane8 >= 16 * i) & (lane8 < _T), gv, _U32(0)) for i, gv in gs]
            hs += [jnp.where(lane8 >= _T + 16 * i, gv, _U32(0)) for i, gv in gs]
            hk = pltpu.bitcast(jnp.concatenate(hs, axis=0), _BF16)
            rows = pl.ds(p, NC, stride=SU)
            yd = lax.dot_general(ut_v[rows, :], hk, _NN, preferred_element_type=_F32)
            yt_v[rows, :] = jnp.where(first_c, 0.0, y) + yd

        def block(sb, carry):
            @pl.when(sb > 0)
            def _():
                for t in range(3):
                    w_cp(t, sb - 1).wait()

            for t in range(3):
                w_cp(t, sb).start()

            @pl.when(sb < NB - 1)
            def _():
                for cp in par_cp(sb + 1) + [u_cp(2 * sb + 2), u_cp(2 * sb + 3)]:
                    cp.start()

            @pl.when(sb == NB - 1)
            def _():
                for cp in [mem_cp] + [x_cp(i) for i in range(XR - 1)]:
                    cp.start()

            for hf in range(2):
                aux_v[0, hf] = jnp.broadcast_to(dt_v[2 * sb + hf][0:1, :], (_CB, _CB)).T

            @pl.when(sb == 0)
            def _():
                def modes(i, c, with_u):
                    for k in range(4):
                        discretise(0, i * 4 + k)
                    for k in range(NC // 2 if with_u else 0):
                        load_u(0, (i - 2) * (NC // 2) + k)
                    return c
                lax.fori_loop(0, 2, functools.partial(modes, with_u=False), 0)
                u_cp(0).wait()
                u_cp(1).wait()
                lax.fori_loop(2, 4, functools.partial(modes, with_u=True), 0)
                xpre_cp.wait()
                xpre = xpre_v[...].astype(_F32).reshape(R, Dm)
                for c in range(NB):
                    xb_v[c] = xpre[:, c * DC:(c + 1) * DC]

            @pl.when(sb > 0)
            def _():
                repack(sb - 1)
                for cp in par_cp(sb) + [u_cp(2 * sb), u_cp(2 * sb + 1)]:
                    cp.wait()

                def prepare(i, c):
                    for k in range(_CB // 16):
                        discretise(sb, i * (_CB // 16) + k)
                    for k in range(NC // 2):
                        load_u(sb, i * (NC // 2) + k)
                    project_ahead(sb - 1, i)
                    return c
                lax.fori_loop(0, 2, prepare, 0)

            for hf in range(2):
                dk_v[2 * sb + hf] = dk_v[2 * sb + hf] + aux_v[3, hf].T[0:8]

            vs, ys = {}, {}
            for p in range(_CB):
                vs[p] = states(p)
                if p % 8 == 7 and p // 8 < EARLY:
                    scan(p // 8)

            @pl.when(sb > 0)
            def _():
                y_cp(sb - 1).wait()
                wo_start(2 * sb - 1)

            wo_start(2 * sb)

            @pl.when(sb == NB - 1)
            def _():
                wo_start(2 * NB - 1)

            for g in range(NG):
                if g + EARLY < NG:
                    scan(g + EARLY)
                for p in range(g * 8, (g + 1) * 8):
                    ys[p] = inter(p, vs.pop(p))
            for p in range(_CB):
                intra(p, ys.pop(p))
            y_cp(sb).start()
            return carry
        lax.fori_loop(0, NB, block, 0)
        for t in range(3):
            w_cp(t, NB - 1).wait()
        repack(NB - 1)
        lax.fori_loop(0, 2, lambda i, c: project_ahead(NB - 1, i), None)

        mem_cp.wait()
        y_cp(NB - 1).wait()
        x_cp(0).wait()
        h_v[0][0:M, :] = mem0_v[...].astype(_F32)
        h_v[0][M:LA, :] = x_v[0, 0].astype(_F32)
        row = lax.broadcasted_iota(jnp.int32, (LA, LA), 0)
        col = lax.broadcasted_iota(jnp.int32, (LA, LA), 1)
        mask = (row < M) | (row >= col)
        wo32 = wo_v.bitcast(_U32)

        def segment(h_in, h_out, dst, side_work, pre_rows):
            def proj(hd):
                h = h_in[...] if pre_rows is None else h_in[0:LA - PRE, :]
                out = [lax.dot_general(h, pltpu.bitcast(wf_v[t][pl.ds(head_row(hd), Dm // 2), :], _BF16), _NN,
                                       preferred_element_type=_F32) for t in range(3)]
                if pre_rows is not None:
                    out = [jnp.concatenate([out[t], zpre_v[hd % 2, t * HP + hd // 2, pre_rows, :]], axis=0) for t in range(3)]
                return out

            qkv, prob = {}, {}

            def scores(hd):
                q, k, _ = qkv[hd]
                sc = lax.dot_general(q, k, _NT, preferred_element_type=_F32) * scale
                sc = jnp.where(mask, sc, -1e9)
                p = jnp.exp(sc - jnp.max(sc, axis=-1, keepdims=True))
                prob[hd] = p / jnp.sum(p, axis=-1, keepdims=True)

            def values(hd):
                o_v[:, hd * Dh:(hd + 1) * Dh] = lax.dot_general(
                    prob[hd], qkv[hd][2], _NN, preferred_element_type=_F32)

            for hd in range(H):
                qkv[hd] = proj(hd)
                if hd >= 1:
                    scores(hd - 1)
                if hd >= 3:
                    values(hd - 3)
                if hd in side_work:
                    side_work[hd]()
            n1 = H - H // 4
            late = [(scores, H - 1), None, (values, H - 3), (values, H - 2), (values, H - 1)]
            o = o_v[:, 0:n1 * Dh]
            for j in range(Dm // _LANES):
                w = pltpu.bitcast(wo32[j, 0:n1 * Dh // 2, :], _BF16)
                acc_v[:, j * _LANES:(j + 1) * _LANES] = lax.dot_general(o, w, _NN, preferred_element_type=_F32)
                if j < len(late) and late[j] is not None:
                    late[j][0](late[j][1])
            o = o_v[:, n1 * Dh:]
            for j in range(Dm // _LANES):
                cols = slice(j * _LANES, (j + 1) * _LANES)
                w = pltpu.bitcast(wo32[j, n1 * Dh // 2:, :], _BF16)
                res = lax.dot_general(o, w, _NN, preferred_element_type=_F32) + acc_v[:, cols]
                h_out[0:M, cols] = res[0:M]
                dst[:, cols] = res[M:].astype(_BF16)

        def out_cp(i):
            rows = pl.ds(pl.multiple_of(i * _T, _T), _T)
            return pltpu.make_async_copy(out_v.at[rows], out_hbm.at[rows], sem_out)

        def chunk(i, carry, ahead):
            rows = pl.ds(pl.multiple_of(i * _T, _T), _T)
            dst = out_v.at[rows]
            x_cp(i + 1).wait()

            def s4_epilogue(sb):
                y = ya_v[sb, pl.ds(i * SU, _CB), :].T
                for q in range(2):
                    cb = 2 * sb + q
                    skip = u_v[cb, rows, :].astype(_F32) * dk_v[cb][0:1, :]
                    dst[:, Dm + cb * _CB:Dm + (cb + 1) * _CB] = (y[q * _T:(q + 1) * _T] + skip).astype(_BF16)

            def next_rows(k):
                if k < SPC:
                    h_v[k][M:LA, :] = x_v[i % XR, k].astype(_F32)
                else:
                    h_v[0][M:LA, :] = x_v[(i + 1) % XR, 0].astype(_F32)

            def traffic():
                x_cp(i + XR - 1).start()

            for k in range(SPC):
                side = {H // 2: functools.partial(next_rows, k + 1)}
                if k == 0:
                    side[2] = traffic
                    for sb in range(NB):
                        side[4 + 2 * sb] = functools.partial(s4_epilogue, sb)
                pre_rows = pl.ds(pl.multiple_of((i * SPC + k) * PRE, PRE), PRE) if ahead else None
                segment(h_v[k], h_v[(k + 1) % SPC], dst.at[pl.ds(k * seg, seg)], side, pre_rows)
            out_cp(i).start()
            return carry

        pltpu.make_async_copy(wo_v, wo_v, sem_wo).wait()
        lax.fori_loop(0, NPRE, functools.partial(chunk, ahead=True), 0)
        lax.fori_loop(NPRE, NC, functools.partial(chunk, ahead=False), 0)

        for i in range(NC + 1, NC + XR - 1):
            x_cp(i).wait()
        pltpu.make_async_copy(out_v, out_hbm, sem_out).wait()

    scratch = [
        pltpu.VMEM((XR, SPC, seg, Dm), _BF16),
        pltpu.VMEM((NPRE * SPC, PRE, Dm), _BF16),
        pltpu.VMEM((NB, R, DC), _F32),
        pltpu.VMEM((2, 3 * HP, R, Dh), _F32),
        pltpu.VMEM((M, Dm), _BF16),
        pltpu.VMEM((3, Dm * H, Dh), _BF16),
        pltpu.VMEM((Dm // _LANES, H * Dh, _LANES), _BF16),
        pltpu.VMEM((2 * NB, L, _CB), _BF16),
        pltpu.VMEM((6, D, N), _BF16),
        pltpu.VMEM((D,), _BF16),
        pltpu.VMEM((D,), _BF16),
        pltpu.VMEM((2 * NB, 8, _CB), _F32),
        pltpu.VMEM((2 * NB, 8, _CB), _F32),
        pltpu.VMEM((NC * SU, _LANES), _F32),
        pltpu.VMEM((NC * SU, _LANES), _F32),
        pltpu.VMEM((NB, NC * SU, _LANES), _F32),
        pltpu.VMEM((2, NPOW * SU + 5, N), _F32),
        pltpu.VMEM((2, NPOW * SU + 5, N), _F32),
        pltpu.VMEM((6, 2, _CB, N), _F32),
        pltpu.VMEM((LA, H * Dh), _F32),
        pltpu.VMEM((LA, Dm), _F32),
        pltpu.VMEM((S, Dm + D), _BF16),
        pltpu.SemaphoreType.DMA((6 * NB,)),
        pltpu.SemaphoreType.DMA((4,)),
        pltpu.SemaphoreType.DMA((2 * NB,)),
        pltpu.SemaphoreType.DMA((3 * NB,)),
        pltpu.SemaphoreType.DMA(()),
        pltpu.SemaphoreType.DMA((XR,)),
        pltpu.SemaphoreType.DMA(()),
        pltpu.SemaphoreType.DMA(()),
    ]
    scratch += [pltpu.VMEM((LA, Dm), _F32)] * SPC
    scratch += [pltpu.VMEM((H * SW, Dh), _U32)] * 3
    scratch += [pltpu.VMEM((NC * SG, N), _F32)] * (4 * NG)
    return kernel, scratch


@functools.partial(jax.jit, static_argnames=("A_seg_len",))
def pallas_concat_heads__memory_aug_recurrent_mem_tr__ssm_conv_s4__prompt_kernel(
    A_x: jax.Array,
    A_mem0: jax.Array,
    A_Wq: jax.Array,
    A_Wk: jax.Array,
    A_Wv: jax.Array,
    A_Wo: jax.Array,
    A_seg_len: int,
    B_u: jax.Array,
    B_A_re: jax.Array,
    B_A_im: jax.Array,
    B_B_re: jax.Array,
    B_B_im: jax.Array,
    B_C_re: jax.Array,
    B_C_im: jax.Array,
    B_log_dt: jax.Array,
    B_Dskip: jax.Array,
):
    B, S, Dm = A_x.shape
    H, Dh = A_Wq.shape[1], A_Wq.shape[2]
    M = A_mem0.shape[1]
    seg = int(A_seg_len)
    _, L, D = B_u.shape
    N = B_A_re.shape[1]
    assert B == 1 and S == L and S % seg == 0 and Dh == _LANES and N == _LANES

    kernel, scratch = _make_kernel(S, Dm, H, Dh, M, seg, L, D, N)
    out = pl.pallas_call(
        kernel,
        out_shape=jax.ShapeDtypeStruct((S, Dm + D), _BF16),
        in_specs=[pl.BlockSpec(memory_space=pl.ANY)] * 15,
        out_specs=pl.BlockSpec(memory_space=pl.ANY),
        scratch_shapes=scratch,
        compiler_params=pltpu.CompilerParams(vmem_limit_bytes=120 * 1024 * 1024),
    )(
        A_x.reshape(S // seg, seg, Dm), A_mem0.reshape(M, Dm),
        A_Wq.reshape(Dm * H, Dh), A_Wk.reshape(Dm * H, Dh), A_Wv.reshape(Dm * H, Dh),
        A_Wo.reshape(H * Dh, Dm), B_u.reshape(L, D),
        B_A_re, B_A_im, B_B_re, B_B_im, B_C_re, B_C_im, B_log_dt, B_Dskip,
    )
    return out.reshape(B, S, Dm + D)
```

```python
import functools

import jax
import jax.numpy as jnp
from jax import lax
import jax.experimental.pallas as pl
import jax.experimental.pallas.tpu as pltpu

_NN = (((1,), (0,)), ((), ()))
_NT = (((1,), (1,)), ((), ()))
_LANES = 128
_T = 64
_CB = 128
_F32 = jnp.float32
_BF16 = jnp.bfloat16
_U32 = jnp.uint32


def _cmul(ar, ai, br, bi):
    return ar * br - ai * bi, ar * bi + ai * br


def _csqrt(x, y):
    big = jnp.sqrt(0.5 * (jnp.sqrt(x * x + y * y) + jnp.abs(x)))
    small = jnp.where(big > 0, 0.5 * y / big, 0.0)
    pos = x >= 0
    return jnp.where(pos, big, jnp.abs(small)), jnp.where(pos, small, jnp.where(y < 0, -big, big))


def _make_kernel(S, Dm, H, Dh, M, seg, L, D, N):
    LA = M + seg
    scale = Dh ** (-0.5)
    NC = L // _T
    NB = D // (2 * _CB)
    SG = 17
    DC = Dm // NB
    NG = _CB // 8
    XR = 4
    SPC = _T // seg
    EARLY = 1
    SU = _CB + 1
    SW = Dm // 2 + 1
    NPOW = 11
    HP = H // 2
    WR = H * Dh // (2 * NB)
    PRE = 8
    NPRE = 5
    R = NPRE * SPC * PRE

    def head_row(hd):
        return ((hd % 2) * HP + hd // 2) * SW

    def kernel(x_hbm, mem0_hbm, wq_hbm, wk_hbm, wv_hbm, wo_hbm, u_hbm,
               are_hbm, aim_hbm, bre_hbm, bim_hbm, cre_hbm, cim_hbm, ldt_hbm, dsk_hbm,
               out_hbm,
               x_v, xpre_v, xb_v, zpre_v, mem0_v, wraw_v, wo_v, u_v, par_v, ldt_v, dsk_v, dt_v, dk_v,
               ut_v, yt_v, ya_v, pr_v, pi_v, aux_v,
               o_v, acc_v, out_v,
               sem_par, sem_misc, sem_u, sem_w, sem_wo, sem_x, sem_out, sem_y, *bufs):
        h_v, wf_v, st_v = bufs[:SPC], bufs[SPC:SPC + 3], bufs[SPC + 3:]
        par_hbm = (are_hbm, aim_hbm, bre_hbm, bim_hbm, cre_hbm, cim_hbm)
        vec_cp = [pltpu.make_async_copy(ldt_hbm, ldt_v, sem_misc.at[0]),
                  pltpu.make_async_copy(dsk_hbm, dsk_v, sem_misc.at[1])]
        mem_cp = pltpu.make_async_copy(mem0_hbm, mem0_v, sem_misc.at[2])

        def par_cp(sb):
            rows = pl.ds(pl.multiple_of(sb * 2 * _CB, 2 * _CB), 2 * _CB)
            return [pltpu.make_async_copy(par_hbm[i].at[rows], par_v.at[i, rows], sem_par.at[sb * 6 + i])
                    for i in range(6)]

        w_hbm = (wq_hbm, wk_hbm, wv_hbm)

        def u_cp(cb):
            return pltpu.make_async_copy(
                u_hbm.at[:, pl.ds(pl.multiple_of(cb * _CB, _CB), _CB)], u_v.at[cb], sem_u.at[cb])

        def w_cp(t, cb):
            rows = pl.ds(pl.multiple_of(cb * (DC * H), DC * H), DC * H)
            return pltpu.make_async_copy(w_hbm[t].at[rows], wraw_v.at[t, rows], sem_w.at[t * NB + cb])

        def wo_start(r):
            rows = pl.ds(r * WR if isinstance(r, int) else pl.multiple_of(r * WR, WR), WR)
            for j in range(Dm // _LANES):
                pltpu.make_async_copy(wo_hbm.at[rows, pl.ds(j * _LANES, _LANES)], wo_v.at[j, rows], sem_wo).start()

        def y_cp(sb):
            return pltpu.make_async_copy(yt_v, ya_v.at[sb], sem_y)

        def x_cp(i):
            src = pl.ds(jnp.minimum(i, NC - 1) * SPC, SPC)
            return pltpu.make_async_copy(x_hbm.at[src], x_v.at[i & (XR - 1)], sem_x.at[i & (XR - 1)])

        xpre_cp = pltpu.make_async_copy(
            x_hbm.at[pl.ds(0, NPRE * SPC), pl.ds(seg - PRE, PRE)], xpre_v, sem_misc.at[3])

        for cp in par_cp(0) + vec_cp:
            cp.start()
        u_cp(0).start()
        u_cp(1).start()
        zpre_v[...] = jnp.zeros(zpre_v.shape, _F32)
        for cp in par_cp(0) + vec_cp:
            cp.wait()
        xpre_cp.start()

        dt_all = jnp.exp(ldt_v[...].astype(_F32)).astype(_BF16).astype(_F32).reshape(1, D)
        dk_all = dsk_v[...].astype(_F32).reshape(1, D)
        for cb in range(2 * NB):
            dt_v[cb] = jnp.broadcast_to(dt_all[:, cb * _CB:(cb + 1) * _CB], (8, _CB))
            dk_v[cb] = jnp.broadcast_to(dk_all[:, cb * _CB:(cb + 1) * _CB], (8, _CB))

        flip8 = 7 - lax.broadcasted_iota(jnp.int32, (8, _LANES), 0)
        lane8 = lax.broadcasted_iota(jnp.int32, (8, _LANES), 1)
        sub8 = lax.broadcasted_iota(jnp.int32, (8, _LANES), 0)
        lo_c = lax.broadcasted_iota(jnp.int32, (NC, _LANES), 1) < _T
        first_c = lax.broadcasted_iota(jnp.int32, (NC, _LANES), 0) == 0
        raw32 = wraw_v.bitcast(_U32)
        s_buf = [(st_v[4 * i], st_v[4 * i + 1]) for i in range(NG)]
        z_buf = [(st_v[4 * i + 2], st_v[4 * i + 3]) for i in range(NG)]

        def discretise(sb, g):
            hf = g // (_CB // 16)
            g16 = (g % (_CB // 16)) * 16
            r = pl.ds(pl.multiple_of(g16, 16), 16)
            rg = pl.ds(pl.multiple_of(sb * 2 * _CB + g * 16, 16), 16)
            dt = aux_v[0, hf, r, :]
            a = dt * par_v[0, rg, :].astype(_F32)
            b = dt * par_v[1, rg, :].astype(_F32)
            mag = jnp.exp(a)
            l1 = (mag * jnp.cos(b), mag * jnp.sin(b))
            w = _cmul(par_v[4, rg, :].astype(_F32), par_v[5, rg, :].astype(_F32),
                      dt * par_v[2, rg, :].astype(_F32), dt * par_v[3, rg, :].astype(_F32))
            l2 = _cmul(*l1, *l1)
            l4 = _cmul(*l2, *l2)
            l8 = _cmul(*l4, *l4)
            l16 = _cmul(*l8, *l8)
            l32 = _cmul(*l16, *l16)
            l64 = _cmul(*l32, *l32)
            pw = [_csqrt(*_cmul(*w, *l1))]
            pw.append(_cmul(*pw[0], *l1))
            pw += [_cmul(*q, *l2) for q in pw]
            pw += [_cmul(*q, *l4) for q in pw]
            pw += [l8, l16, l32]
            for j in range(NPOW):
                pr_v[hf, pl.ds(j * SU + g16, 16), :] = pw[j][0]
                pi_v[hf, pl.ds(j * SU + g16, 16), :] = pw[j][1]
            aux_v[1, hf, r, :] = l64[0]
            aux_v[2, hf, r, :] = l64[1]
            aux_v[3, hf, r, :] = jnp.broadcast_to(jnp.sum(w[0], axis=-1, keepdims=True), (16, N))
            aux_v[4, hf, r, :] = pw[0][0]
            aux_v[5, hf, r, :] = -pw[0][1]
            return pw[7][0][8:16]

        def load_u(sb, ck):
            rows = pl.ds(pl.multiple_of(ck * _T, _T), _T)
            fl = []
            for q in range(2):
                tile = u_v[2 * sb + q, rows, :].astype(_F32)
                fl += [jnp.take_along_axis(tile[_T - 8 * (i + 1):_T - 8 * i], flip8, axis=0)
                       for i in range(_T // 8)]
            ut = jnp.concatenate(fl, axis=0).T
            ut_v[pl.ds(ck * SU, _CB), :] = ut
            return ut[_CB - 8:]

        def repack(c):
            nj = DC // 2 // 4

            def body(i, carry):
                j0 = c * (DC // 2) + i * nj
                for t in range(3):
                    src = raw32.at[t, pl.ds(pl.multiple_of(j0 * H, nj * H), nj * H), :]
                    for j in range(nj):
                        for half in range(HP // 8):
                            a = src[pl.ds(j * H + half * 8, 8), :]
                            b = src[pl.ds(j * H + HP + half * 8, 8), :]
                            wf_v[t][pl.ds(j0 + (half * 8 * SW + j), 8, stride=SW), :] = (a & _U32(0xFFFF)) | (b << 16)
                            wf_v[t][pl.ds(j0 + ((HP + half * 8) * SW + j), 8, stride=SW), :] = (
                                (a >> 16) | (b & _U32(0xFFFF0000)))
                return carry
            lax.fori_loop(0, 4, body, 0)

        def project_ahead(c, par):
            lhs = xb_v[c]
            r0 = par * (HP * SW) + c * (DC // 2)
            for t in range(3):
                for k in range(HP):
                    w = wf_v[t][pl.ds(r0 + k * SW, DC // 2), :]
                    zpre_v[par, t * HP + k] += lax.dot_general(
                        lhs, pltpu.bitcast(w, _BF16), _NN, preferred_element_type=_F32)

        def states(p):
            vr, vi = [], []
            for hf in range(2):
                ar = [pr_v[hf, pl.ds(p, 8, stride=SU), :]]
                ai = [pi_v[hf, pl.ds(p, 8, stride=SU), :]]
                for lvl in range(3):
                    mr = jnp.broadcast_to(pr_v[hf, pl.ds((8 + lvl) * SU + p, 1), :], (8, N))
                    mi = jnp.broadcast_to(pi_v[hf, pl.ds((8 + lvl) * SU + p, 1), :], (8, N))
                    for i in range(len(ar)):
                        nr, ni = _cmul(ar[i], ai[i], mr, mi)
                        ar.append(nr)
                        ai.append(ni)
                vr += ar
                vi += ai
            v = jnp.concatenate(
                [jnp.concatenate(vr, axis=0), jnp.concatenate(vi, axis=0)], axis=1).astype(_BF16)
            uf = ut_v[pl.ds(p, NC, stride=SU), :]
            lhs = jnp.concatenate([jnp.where(lo_c, uf, 0.0), jnp.where(lo_c, 0.0, uf)], axis=0)
            st = lax.dot_general(lhs, v, _NN, preferred_element_type=_F32)
            sr, si = s_buf[p // 8]
            for hf in range(2):
                rows = pl.ds(hf * 8 + p % 8, NC, stride=SG)
                sr[rows, :] = st[hf * NC:(hf + 1) * NC, :N]
                si[rows, :] = st[hf * NC:(hf + 1) * NC, N:]
            return v

        def scan(g):
            sr, si = s_buf[g]
            zr, zi = z_buf[g]
            cat = lambda i: jnp.concatenate([aux_v[i, hf, g * 8:(g + 1) * 8, :] for hf in range(2)], axis=0)
            lr, li = cat(1), cat(2)
            zr[0:16, :] = cat(4)
            zi[0:16, :] = cat(5)
            for c in range(1, NC):
                s_r = sr[pl.ds((c - 1) * SG, 16), :]
                s_i = si[pl.ds((c - 1) * SG, 16), :]
                if c == 1:
                    xr, xi = s_r, -s_i
                else:
                    xr, xi = (xr * lr + s_r) + xi * li, (xi * lr - s_i) - xr * li
                zr[pl.ds(c * SG, 16), :] = xr
                zi[pl.ds(c * SG, 16), :] = xi

        def inter(p, v):
            z = [jnp.concatenate([zb[pl.ds(hf * 8 + p % 8, NC, stride=SG), :] for hf in range(2)], axis=0)
                 for zb in z_buf[p // 8]]
            y = lax.dot_general(jnp.concatenate(z, axis=1), v, _NT, preferred_element_type=_F32)
            return jnp.where(lo_c, y[:NC], y[NC:])

        def intra(p, y):
            kk = jnp.broadcast_to(y[0:1, :], (8, _LANES))
            g1 = pltpu.roll(kk, 1, 1, stride=1, stride_axis=0)
            g1 = jnp.where((lane8 & (_T - 1)) > sub8, g1, 0.0)
            g1 = jnp.take_along_axis(g1, flip8, axis=0)
            g0 = jnp.where((lane8 & (_T - 1)) >= 8, pltpu.roll(g1, 8, 1), 0.0)
            top = pltpu.bitcast(jnp.concatenate([g0, g1], axis=0).astype(_BF16), _U32)
            gs = [(i, pltpu.roll(top, 16 * i, 1) if i else top) for i in range(_T // 16 - 1, -1, -1)]
            hs = [jnp.where((lane8 >= 16 * i) & (lane8 < _T), gv, _U32(0)) for i, gv in gs]
            hs += [jnp.where(lane8 >= _T + 16 * i, gv, _U32(0)) for i, gv in gs]
            hk = pltpu.bitcast(jnp.concatenate(hs, axis=0), _BF16)
            rows = pl.ds(p, NC, stride=SU)
            yd = lax.dot_general(ut_v[rows, :], hk, _NN, preferred_element_type=_F32)
            yt_v[rows, :] = jnp.where(first_c, 0.0, y) + yd

        def block(sb, carry):
            @pl.when(sb > 0)
            def _():
                for t in range(3):
                    w_cp(t, sb - 1).wait()

            for t in range(3):
                w_cp(t, sb).start()

            @pl.when(sb < NB - 1)
            def _():
                for cp in par_cp(sb + 1) + [u_cp(2 * sb + 2), u_cp(2 * sb + 3)]:
                    cp.start()

            @pl.when(sb == NB - 1)
            def _():
                for cp in [mem_cp] + [x_cp(i) for i in range(XR - 1)]:
                    cp.start()

            for hf in range(2):
                aux_v[0, hf] = jnp.broadcast_to(dt_v[2 * sb + hf][0:1, :], (_CB, _CB)).T

            @pl.when(sb == 0)
            def _():
                def modes(i, c, with_u):
                    for k in range(4):
                        discretise(0, i * 4 + k)
                    for k in range(NC // 2 if with_u else 0):
                        load_u(0, (i - 2) * (NC // 2) + k)
                    return c
                lax.fori_loop(0, 2, functools.partial(modes, with_u=False), 0)
                u_cp(0).wait()
                u_cp(1).wait()
                lax.fori_loop(2, 4, functools.partial(modes, with_u=True), 0)
                xpre_cp.wait()
                xpre = xpre_v[...].astype(_F32).reshape(R, Dm)
                for c in range(NB):
                    xb_v[c] = xpre[:, c * DC:(c + 1) * DC]

            @pl.when(sb > 0)
            def _():
                repack(sb - 1)
                for cp in par_cp(sb) + [u_cp(2 * sb), u_cp(2 * sb + 1)]:
                    cp.wait()

                def prepare(i, c):
                    for k in range(_CB // 16):
                        discretise(sb, i * (_CB // 16) + k)
                    for k in range(NC // 2):
                        load_u(sb, i * (NC // 2) + k)
                    project_ahead(sb - 1, i)
                    return c
                lax.fori_loop(0, 2, prepare, 0)

            for hf in range(2):
                dk_v[2 * sb + hf] = dk_v[2 * sb + hf] + aux_v[3, hf].T[0:8]

            vs, ys = {}, {}
            for p in range(_CB):
                vs[p] = states(p)
                if p % 8 == 7 and p // 8 < EARLY:
                    scan(p // 8)

            @pl.when(sb > 0)
            def _():
                y_cp(sb - 1).wait()
                wo_start(2 * sb - 1)

            wo_start(2 * sb)

            @pl.when(sb == NB - 1)
            def _():
                wo_start(2 * NB - 1)

            for g in range(NG):
                if g + EARLY < NG:
                    scan(g + EARLY)
                for p in range(g * 8, (g + 1) * 8):
                    ys[p] = inter(p, vs.pop(p))
            for p in range(_CB):
                intra(p, ys.pop(p))
            y_cp(sb).start()
            return carry
        lax.fori_loop(0, NB, block, 0)
        for t in range(3):
            w_cp(t, NB - 1).wait()
        repack(NB - 1)
        lax.fori_loop(0, 2, lambda i, c: project_ahead(NB - 1, i), None)

        mem_cp.wait()
        y_cp(NB - 1).wait()
        x_cp(0).wait()
        h_v[0][0:M, :] = mem0_v[...].astype(_F32)
        h_v[0][M:LA, :] = x_v[0, 0].astype(_F32)
        row = lax.broadcasted_iota(jnp.int32, (LA, LA), 0)
        col = lax.broadcasted_iota(jnp.int32, (LA, LA), 1)
        mask = (row < M) | (row >= col)
        wo32 = wo_v.bitcast(_U32)

        def segment(h_in, h_out, dst, side_work, pre_rows):
            def proj(hd):
                h = h_in[...] if pre_rows is None else h_in[0:LA - PRE, :]
                dot = lambda t, k0, k1: lax.dot_general(
                    h[:, k0:k1], pltpu.bitcast(wf_v[t][pl.ds(head_row(hd) + k0 // 2, (k1 - k0) // 2), :], _BF16),
                    _NN, preferred_element_type=_F32)
                if hd == 0:
                    cut, part = Dm // 2, [acc_v.at[0:h.shape[0], t * Dh:(t + 1) * Dh] for t in range(3)]
                    for t in range(3):
                        part[t][...] = dot(t, 0, cut)
                    out = [part[t][...] + dot(t, cut, Dm) for t in range(3)]
                else:
                    out = [dot(t, 0, Dm) for t in range(3)]
                if pre_rows is not None:
                    out = [jnp.concatenate([out[t], zpre_v[hd % 2, t * HP + hd // 2, pre_rows, :]], axis=0) for t in range(3)]
                return out

            qkv, prob = {}, {}

            def scores(hd):
                q, k, _ = qkv[hd]
                sc = lax.dot_general(q, k, _NT, preferred_element_type=_F32) * scale
                sc = jnp.where(mask, sc, -1e9)
                p = jnp.exp(sc - jnp.max(sc, axis=-1, keepdims=True))
                prob[hd] = p / jnp.sum(p, axis=-1, keepdims=True)

            def values(hd):
                o_v[:, hd * Dh:(hd + 1) * Dh] = lax.dot_general(
                    prob[hd], qkv[hd][2], _NN, preferred_element_type=_F32)

            for hd in range(H):
                qkv[hd] = proj(hd)
                if hd >= 1:
                    scores(hd - 1)
                if hd >= 3:
                    values(hd - 3)
                if hd in side_work:
                    side_work[hd]()
            n1 = H - H // 4
            late = [(scores, H - 1), None, (values, H - 3), (values, H - 2), (values, H - 1)]
            o = o_v[:, 0:n1 * Dh]
            for j in range(Dm // _LANES):
                w = pltpu.bitcast(wo32[j, 0:n1 * Dh // 2, :], _BF16)
                acc_v[:, j * _LANES:(j + 1) * _LANES] = lax.dot_general(o, w, _NN, preferred_element_type=_F32)
                if j < len(late) and late[j] is not None:
                    late[j][0](late[j][1])
            o = o_v[:, n1 * Dh:]
            for j in range(Dm // _LANES):
                cols = slice(j * _LANES, (j + 1) * _LANES)
                w = pltpu.bitcast(wo32[j, n1 * Dh // 2:, :], _BF16)
                res = lax.dot_general(o, w, _NN, preferred_element_type=_F32) + acc_v[:, cols]
                h_out[0:M, cols] = res[0:M]
                dst[:, cols] = res[M:].astype(_BF16)

        def out_cp(i):
            rows = pl.ds(pl.multiple_of(i * _T, _T), _T)
            return pltpu.make_async_copy(out_v.at[rows], out_hbm.at[rows], sem_out)

        def chunk(i, carry, ahead):
            rows = pl.ds(pl.multiple_of(i * _T, _T), _T)
            dst = out_v.at[rows]
            x_cp(i + 1).wait()

            def s4_epilogue(sb):
                y = ya_v[sb, pl.ds(i * SU, _CB), :].T
                for q in range(2):
                    cb = 2 * sb + q
                    skip = u_v[cb, rows, :].astype(_F32) * dk_v[cb][0:1, :]
                    dst[:, Dm + cb * _CB:Dm + (cb + 1) * _CB] = (y[q * _T:(q + 1) * _T] + skip).astype(_BF16)

            def next_rows(k):
                if k < SPC:
                    h_v[k][M:LA, :] = x_v[i & (XR - 1), k].astype(_F32)
                else:
                    h_v[0][M:LA, :] = x_v[(i + 1) & (XR - 1), 0].astype(_F32)

            def traffic():
                x_cp(i + XR - 1).start()

            for k in range(SPC):
                side = {H // 2: functools.partial(next_rows, k + 1)}
                if k == 0:
                    side[2] = traffic
                    for sb in range(NB):
                        side[4 + 2 * sb] = functools.partial(s4_epilogue, sb)
                pre_rows = pl.ds(pl.multiple_of((i * SPC + k) * PRE, PRE), PRE) if ahead else None
                segment(h_v[k], h_v[(k + 1) % SPC], dst.at[pl.ds(k * seg, seg)], side, pre_rows)
            out_cp(i).start()
            return carry

        pltpu.make_async_copy(wo_v, wo_v, sem_wo).wait()
        lax.fori_loop(0, NPRE, functools.partial(chunk, ahead=True), 0)
        lax.fori_loop(NPRE, NC, functools.partial(chunk, ahead=False), 0)

        for i in range(NC + 1, NC + XR - 1):
            x_cp(i).wait()
        pltpu.make_async_copy(out_v, out_hbm, sem_out).wait()

    scratch = [
        pltpu.VMEM((XR, SPC, seg, Dm), _BF16),
        pltpu.VMEM((NPRE * SPC, PRE, Dm), _BF16),
        pltpu.VMEM((NB, R, DC), _F32),
        pltpu.VMEM((2, 3 * HP, R, Dh), _F32),
        pltpu.VMEM((M, Dm), _BF16),
        pltpu.VMEM((3, Dm * H, Dh), _BF16),
        pltpu.VMEM((Dm // _LANES, H * Dh, _LANES), _BF16),
        pltpu.VMEM((2 * NB, L, _CB), _BF16),
        pltpu.VMEM((6, D, N), _BF16),
        pltpu.VMEM((D,), _BF16),
        pltpu.VMEM((D,), _BF16),
        pltpu.VMEM((2 * NB, 8, _CB), _F32),
        pltpu.VMEM((2 * NB, 8, _CB), _F32),
        pltpu.VMEM((NC * SU, _LANES), _F32),
        pltpu.VMEM((NC * SU, _LANES), _F32),
        pltpu.VMEM((NB, NC * SU, _LANES), _F32),
        pltpu.VMEM((2, NPOW * SU + 5, N), _F32),
        pltpu.VMEM((2, NPOW * SU + 5, N), _F32),
        pltpu.VMEM((6, 2, _CB, N), _F32),
        pltpu.VMEM((LA, H * Dh), _F32),
        pltpu.VMEM((LA, Dm), _F32),
        pltpu.VMEM((S, Dm + D), _BF16),
        pltpu.SemaphoreType.DMA((6 * NB,)),
        pltpu.SemaphoreType.DMA((4,)),
        pltpu.SemaphoreType.DMA((2 * NB,)),
        pltpu.SemaphoreType.DMA((3 * NB,)),
        pltpu.SemaphoreType.DMA(()),
        pltpu.SemaphoreType.DMA((XR,)),
        pltpu.SemaphoreType.DMA(()),
        pltpu.SemaphoreType.DMA(()),
    ]
    scratch += [pltpu.VMEM((LA, Dm), _F32)] * SPC
    scratch += [pltpu.VMEM((H * SW, Dh), _U32)] * 3
    scratch += [pltpu.VMEM((NC * SG, N), _F32)] * (4 * NG)
    return kernel, scratch


@functools.partial(jax.jit, static_argnames=("A_seg_len",))
def pallas_concat_heads__memory_aug_recurrent_mem_tr__ssm_conv_s4__prompt_kernel(
    A_x: jax.Array,
    A_mem0: jax.Array,
    A_Wq: jax.Array,
    A_Wk: jax.Array,
    A_Wv: jax.Array,
    A_Wo: jax.Array,
    A_seg_len: int,
    B_u: jax.Array,
    B_A_re: jax.Array,
    B_A_im: jax.Array,
    B_B_re: jax.Array,
    B_B_im: jax.Array,
    B_C_re: jax.Array,
    B_C_im: jax.Array,
    B_log_dt: jax.Array,
    B_Dskip: jax.Array,
):
    B, S, Dm = A_x.shape
    H, Dh = A_Wq.shape[1], A_Wq.shape[2]
    M = A_mem0.shape[1]
    seg = int(A_seg_len)
    _, L, D = B_u.shape
    N = B_A_re.shape[1]
    assert B == 1 and S == L and S % seg == 0 and Dh == _LANES and N == _LANES

    kernel, scratch = _make_kernel(S, Dm, H, Dh, M, seg, L, D, N)
    out = pl.pallas_call(
        kernel,
        out_shape=jax.ShapeDtypeStruct((S, Dm + D), _BF16),
        in_specs=[pl.BlockSpec(memory_space=pl.ANY)] * 15,
        out_specs=pl.BlockSpec(memory_space=pl.ANY),
        scratch_shapes=scratch,
        compiler_params=pltpu.CompilerParams(vmem_limit_bytes=120 * 1024 * 1024),
    )(
        A_x.reshape(S // seg, seg, Dm), A_mem0.reshape(M, Dm),
        A_Wq.reshape(Dm * H, Dh), A_Wk.reshape(Dm * H, Dh), A_Wv.reshape(Dm * H, Dh),
        A_Wo.reshape(H * Dh, Dm), B_u.reshape(L, D),
        B_A_re, B_A_im, B_B_re, B_B_im, B_C_re, B_C_im, B_log_dt, B_Dskip,
    )
    return out.reshape(B, S, Dm + D)
```

```python
import functools

import jax
import jax.numpy as jnp
from jax import lax
import jax.experimental.pallas as pl
import jax.experimental.pallas.tpu as pltpu

_NN = (((1,), (0,)), ((), ()))
_NT = (((1,), (1,)), ((), ()))
_LANES = 128
_T = 64
_CB = 128
_F32 = jnp.float32
_BF16 = jnp.bfloat16
_U32 = jnp.uint32


def _cmul(ar, ai, br, bi):
    return ar * br - ai * bi, ar * bi + ai * br


def _csqrt(x, y):
    big = jnp.sqrt(0.5 * (jnp.sqrt(x * x + y * y) + jnp.abs(x)))
    small = jnp.where(big > 0, 0.5 * y / big, 0.0)
    pos = x >= 0
    return jnp.where(pos, big, jnp.abs(small)), jnp.where(pos, small, jnp.where(y < 0, -big, big))


def _make_kernel(S, Dm, H, Dh, M, seg, L, D, N):
    LA = M + seg
    scale = Dh ** (-0.5)
    NC = L // _T
    NB = D // (2 * _CB)
    SG = 17
    DC = Dm // NB
    NG = _CB // 8
    XR = 4
    SPC = _T // seg
    EARLY = 1
    SU = _CB + 1
    SW = Dm // 2 + 1
    NPOW = 11
    HP = H // 2
    WR = H * Dh // (2 * NB)
    PRE = 8
    NPRE = 8
    R = NPRE * SPC * PRE

    def head_row(hd):
        return ((hd % 2) * HP + hd // 2) * SW

    def kernel(x_hbm, mem0_hbm, wq_hbm, wk_hbm, wv_hbm, wo_hbm, u_hbm,
               are_hbm, aim_hbm, bre_hbm, bim_hbm, cre_hbm, cim_hbm, ldt_hbm, dsk_hbm,
               out_hbm,
               x_v, xpre_v, xb_v, zpre_v, mem0_v, wraw_v, wo_v, u_v, par_v, ldt_v, dsk_v, dt_v, dk_v,
               ut_v, yt_v, ya_v, pr_v, pi_v, aux_v,
               o_v, acc_v, out_v,
               sem_par, sem_misc, sem_u, sem_w, sem_wo, sem_x, sem_out, sem_y, *bufs):
        h_v, wf_v, st_v = bufs[:SPC], bufs[SPC:SPC + 3], bufs[SPC + 3:]
        par_hbm = (are_hbm, aim_hbm, bre_hbm, bim_hbm, cre_hbm, cim_hbm)
        vec_cp = [pltpu.make_async_copy(ldt_hbm, ldt_v, sem_misc.at[0]),
                  pltpu.make_async_copy(dsk_hbm, dsk_v, sem_misc.at[1])]
        mem_cp = pltpu.make_async_copy(mem0_hbm, mem0_v, sem_misc.at[2])

        def par_cp(sb):
            rows = pl.ds(pl.multiple_of(sb * 2 * _CB, 2 * _CB), 2 * _CB)
            return [pltpu.make_async_copy(par_hbm[i].at[rows], par_v.at[i, rows], sem_par.at[sb * 6 + i])
                    for i in range(6)]

        w_hbm = (wq_hbm, wk_hbm, wv_hbm)

        def u_cp(cb):
            return pltpu.make_async_copy(
                u_hbm.at[:, pl.ds(pl.multiple_of(cb * _CB, _CB), _CB)], u_v.at[cb], sem_u.at[cb])

        def w_cp(t, cb):
            rows = pl.ds(pl.multiple_of(cb * (DC * H), DC * H), DC * H)
            return pltpu.make_async_copy(w_hbm[t].at[rows], wraw_v.at[t, rows], sem_w.at[t * NB + cb])

        def wo_start(r):
            rows = pl.ds(r * WR if isinstance(r, int) else pl.multiple_of(r * WR, WR), WR)
            for j in range(Dm // _LANES):
                pltpu.make_async_copy(wo_hbm.at[rows, pl.ds(j * _LANES, _LANES)], wo_v.at[j, rows], sem_wo).start()

        def y_cp(sb):
            return pltpu.make_async_copy(yt_v, ya_v.at[sb], sem_y)

        def x_cp(i):
            src = pl.ds(jnp.minimum(i, NC - 1) * SPC, SPC)
            return pltpu.make_async_copy(x_hbm.at[src], x_v.at[i & (XR - 1)], sem_x.at[i & (XR - 1)])

        xpre_cp = pltpu.make_async_copy(
            x_hbm.at[pl.ds(0, NPRE * SPC), pl.ds(seg - PRE, PRE)], xpre_v, sem_misc.at[3])

        for cp in par_cp(0) + vec_cp:
            cp.start()
        u_cp(0).start()
        u_cp(1).start()
        zpre_v[...] = jnp.zeros(zpre_v.shape, _F32)
        for cp in par_cp(0) + vec_cp:
            cp.wait()
        xpre_cp.start()

        dt_all = jnp.exp(ldt_v[...].astype(_F32)).astype(_BF16).astype(_F32).reshape(1, D)
        dk_all = dsk_v[...].astype(_F32).reshape(1, D)
        for cb in range(2 * NB):
            dt_v[cb] = jnp.broadcast_to(dt_all[:, cb * _CB:(cb + 1) * _CB], (8, _CB))
            dk_v[cb] = jnp.broadcast_to(dk_all[:, cb * _CB:(cb + 1) * _CB], (8, _CB))

        flip8 = 7 - lax.broadcasted_iota(jnp.int32, (8, _LANES), 0)
        lane8 = lax.broadcasted_iota(jnp.int32, (8, _LANES), 1)
        sub8 = lax.broadcasted_iota(jnp.int32, (8, _LANES), 0)
        lo_c = lax.broadcasted_iota(jnp.int32, (NC, _LANES), 1) < _T
        first_c = lax.broadcasted_iota(jnp.int32, (NC, _LANES), 0) == 0
        raw32 = wraw_v.bitcast(_U32)
        s_buf = [(st_v[4 * i], st_v[4 * i + 1]) for i in range(NG)]
        z_buf = [(st_v[4 * i + 2], st_v[4 * i + 3]) for i in range(NG)]

        def discretise(sb, g):
            hf = g // (_CB // 16)
            g16 = (g % (_CB // 16)) * 16
            r = pl.ds(pl.multiple_of(g16, 16), 16)
            rg = pl.ds(pl.multiple_of(sb * 2 * _CB + g * 16, 16), 16)
            dt = aux_v[0, hf, r, :]
            a = dt * par_v[0, rg, :].astype(_F32)
            b = dt * par_v[1, rg, :].astype(_F32)
            mag = jnp.exp(a)
            l1 = (mag * jnp.cos(b), mag * jnp.sin(b))
            w = _cmul(par_v[4, rg, :].astype(_F32), par_v[5, rg, :].astype(_F32),
                      dt * par_v[2, rg, :].astype(_F32), dt * par_v[3, rg, :].astype(_F32))
            l2 = _cmul(*l1, *l1)
            l4 = _cmul(*l2, *l2)
            l8 = _cmul(*l4, *l4)
            l16 = _cmul(*l8, *l8)
            l32 = _cmul(*l16, *l16)
            l64 = _cmul(*l32, *l32)
            pw = [_csqrt(*_cmul(*w, *l1))]
            pw.append(_cmul(*pw[0], *l1))
            pw += [_cmul(*q, *l2) for q in pw]
            pw += [_cmul(*q, *l4) for q in pw]
            pw += [l8, l16, l32]
            for j in range(NPOW):
                pr_v[hf, pl.ds(j * SU + g16, 16), :] = pw[j][0]
                pi_v[hf, pl.ds(j * SU + g16, 16), :] = pw[j][1]
            aux_v[1, hf, r, :] = l64[0]
            aux_v[2, hf, r, :] = l64[1]
            aux_v[3, hf, r, :] = jnp.broadcast_to(jnp.sum(w[0], axis=-1, keepdims=True), (16, N))
            aux_v[4, hf, r, :] = pw[0][0]
            aux_v[5, hf, r, :] = -pw[0][1]
            return pw[7][0][8:16]

        def load_u(sb, ck):
            rows = pl.ds(pl.multiple_of(ck * _T, _T), _T)
            fl = []
            for q in range(2):
                tile = u_v[2 * sb + q, rows, :].astype(_F32)
                fl += [jnp.take_along_axis(tile[_T - 8 * (i + 1):_T - 8 * i], flip8, axis=0)
                       for i in range(_T // 8)]
            ut = jnp.concatenate(fl, axis=0).T
            ut_v[pl.ds(ck * SU, _CB), :] = ut
            return ut[_CB - 8:]

        def repack(c):
            nj = DC // 2 // 4

            def body(i, carry):
                j0 = c * (DC // 2) + i * nj
                for t in range(3):
                    src = raw32.at[t, pl.ds(pl.multiple_of(j0 * H, nj * H), nj * H), :]
                    for j in range(nj):
                        for half in range(HP // 8):
                            a = src[pl.ds(j * H + half * 8, 8), :]
                            b = src[pl.ds(j * H + HP + half * 8, 8), :]
                            wf_v[t][pl.ds(j0 + (half * 8 * SW + j), 8, stride=SW), :] = (a & _U32(0xFFFF)) | (b << 16)
                            wf_v[t][pl.ds(j0 + ((HP + half * 8) * SW + j), 8, stride=SW), :] = (
                                (a >> 16) | (b & _U32(0xFFFF0000)))
                return carry
            lax.fori_loop(0, 4, body, 0)

        def project_ahead(c, par):
            lhs = xb_v[c]
            r0 = par * (HP * SW) + c * (DC // 2)
            for t in range(3):
                for k in range(HP):
                    w = wf_v[t][pl.ds(r0 + k * SW, DC // 2), :]
                    zpre_v[par, t * HP + k] += lax.dot_general(
                        lhs, pltpu.bitcast(w, _BF16), _NN, preferred_element_type=_F32)

        def states(p):
            vr, vi = [], []
            for hf in range(2):
                ar = [pr_v[hf, pl.ds(p, 8, stride=SU), :]]
                ai = [pi_v[hf, pl.ds(p, 8, stride=SU), :]]
                for lvl in range(3):
                    mr = jnp.broadcast_to(pr_v[hf, pl.ds((8 + lvl) * SU + p, 1), :], (8, N))
                    mi = jnp.broadcast_to(pi_v[hf, pl.ds((8 + lvl) * SU + p, 1), :], (8, N))
                    for i in range(len(ar)):
                        nr, ni = _cmul(ar[i], ai[i], mr, mi)
                        ar.append(nr)
                        ai.append(ni)
                vr += ar
                vi += ai
            v = jnp.concatenate(
                [jnp.concatenate(vr, axis=0), jnp.concatenate(vi, axis=0)], axis=1).astype(_BF16)
            uf = ut_v[pl.ds(p, NC, stride=SU), :]
            lhs = jnp.concatenate([jnp.where(lo_c, uf, 0.0), jnp.where(lo_c, 0.0, uf)], axis=0)
            st = lax.dot_general(lhs, v, _NN, preferred_element_type=_F32)
            sr, si = s_buf[p // 8]
            for hf in range(2):
                rows = pl.ds(hf * 8 + p % 8, NC, stride=SG)
                sr[rows, :] = st[hf * NC:(hf + 1) * NC, :N]
                si[rows, :] = st[hf * NC:(hf + 1) * NC, N:]
            return v

        def scan(g):
            sr, si = s_buf[g]
            zr, zi = z_buf[g]
            cat = lambda i: jnp.concatenate([aux_v[i, hf, g * 8:(g + 1) * 8, :] for hf in range(2)], axis=0)
            lr, li = cat(1), cat(2)
            zr[0:16, :] = cat(4)
            zi[0:16, :] = cat(5)
            for c in range(1, NC):
                s_r = sr[pl.ds((c - 1) * SG, 16), :]
                s_i = si[pl.ds((c - 1) * SG, 16), :]
                if c == 1:
                    xr, xi = s_r, -s_i
                else:
                    xr, xi = (xr * lr + s_r) + xi * li, (xi * lr - s_i) - xr * li
                zr[pl.ds(c * SG, 16), :] = xr
                zi[pl.ds(c * SG, 16), :] = xi

        def inter(p, v):
            z = [jnp.concatenate([zb[pl.ds(hf * 8 + p % 8, NC, stride=SG), :] for hf in range(2)], axis=0)
                 for zb in z_buf[p // 8]]
            y = lax.dot_general(jnp.concatenate(z, axis=1), v, _NT, preferred_element_type=_F32)
            return jnp.where(lo_c, y[:NC], y[NC:])

        def intra(p, y):
            kk = jnp.broadcast_to(y[0:1, :], (8, _LANES))
            g1 = pltpu.roll(kk, 1, 1, stride=1, stride_axis=0)
            g1 = jnp.where((lane8 & (_T - 1)) > sub8, g1, 0.0)
            g1 = jnp.take_along_axis(g1, flip8, axis=0)
            g0 = jnp.where((lane8 & (_T - 1)) >= 8, pltpu.roll(g1, 8, 1), 0.0)
            top = pltpu.bitcast(jnp.concatenate([g0, g1], axis=0).astype(_BF16), _U32)
            gs = [(i, pltpu.roll(top, 16 * i, 1) if i else top) for i in range(_T // 16 - 1, -1, -1)]
            hs = [jnp.where((lane8 >= 16 * i) & (lane8 < _T), gv, _U32(0)) for i, gv in gs]
            hs += [jnp.where(lane8 >= _T + 16 * i, gv, _U32(0)) for i, gv in gs]
            hk = pltpu.bitcast(jnp.concatenate(hs, axis=0), _BF16)
            rows = pl.ds(p, NC, stride=SU)
            yd = lax.dot_general(ut_v[rows, :], hk, _NN, preferred_element_type=_F32)
            yt_v[rows, :] = jnp.where(first_c, 0.0, y) + yd

        def block(sb, carry):
            @pl.when(sb > 0)
            def _():
                for t in range(3):
                    w_cp(t, sb - 1).wait()

            for t in range(3):
                w_cp(t, sb).start()

            @pl.when(sb < NB - 1)
            def _():
                for cp in par_cp(sb + 1) + [u_cp(2 * sb + 2), u_cp(2 * sb + 3)]:
                    cp.start()

            @pl.when(sb == NB - 1)
            def _():
                for cp in [mem_cp] + [x_cp(i) for i in range(XR - 1)]:
                    cp.start()

            for hf in range(2):
                aux_v[0, hf] = jnp.broadcast_to(dt_v[2 * sb + hf][0:1, :], (_CB, _CB)).T

            @pl.when(sb == 0)
            def _():
                def modes(i, c, with_u):
                    for k in range(4):
                        discretise(0, i * 4 + k)
                    for k in range(NC // 2 if with_u else 0):
                        load_u(0, (i - 2) * (NC // 2) + k)
                    return c
                lax.fori_loop(0, 2, functools.partial(modes, with_u=False), 0)
                u_cp(0).wait()
                u_cp(1).wait()
                lax.fori_loop(2, 4, functools.partial(modes, with_u=True), 0)
                xpre_cp.wait()
                xpre = xpre_v[...].astype(_F32).reshape(R, Dm)
                for c in range(NB):
                    xb_v[c] = xpre[:, c * DC:(c + 1) * DC]

            @pl.when(sb > 0)
            def _():
                repack(sb - 1)
                for cp in par_cp(sb) + [u_cp(2 * sb), u_cp(2 * sb + 1)]:
                    cp.wait()

                def prepare(i, c):
                    for k in range(_CB // 16):
                        discretise(sb, i * (_CB // 16) + k)
                    for k in range(NC // 2):
                        load_u(sb, i * (NC // 2) + k)
                    project_ahead(sb - 1, i)
                    return c
                lax.fori_loop(0, 2, prepare, 0)

            for hf in range(2):
                dk_v[2 * sb + hf] = dk_v[2 * sb + hf] + aux_v[3, hf].T[0:8]

            vs, ys = {}, {}
            for p in range(_CB):
                vs[p] = states(p)
                if p % 8 == 7 and p // 8 < EARLY:
                    scan(p // 8)

            @pl.when(sb > 0)
            def _():
                y_cp(sb - 1).wait()
                wo_start(2 * sb - 1)

            wo_start(2 * sb)

            @pl.when(sb == NB - 1)
            def _():
                wo_start(2 * NB - 1)

            for g in range(NG):
                if g + EARLY < NG:
                    scan(g + EARLY)
                for p in range(g * 8, (g + 1) * 8):
                    ys[p] = inter(p, vs.pop(p))
            for p in range(_CB):
                intra(p, ys.pop(p))
            y_cp(sb).start()
            return carry
        lax.fori_loop(0, NB, block, 0)
        for t in range(3):
            w_cp(t, NB - 1).wait()
        repack(NB - 1)
        lax.fori_loop(0, 2, lambda i, c: project_ahead(NB - 1, i), None)

        mem_cp.wait()
        y_cp(NB - 1).wait()
        x_cp(0).wait()
        h_v[0][0:M, :] = mem0_v[...].astype(_F32)
        h_v[0][M:LA, :] = x_v[0, 0].astype(_F32)
        row = lax.broadcasted_iota(jnp.int32, (LA, LA), 0)
        col = lax.broadcasted_iota(jnp.int32, (LA, LA), 1)
        mask = (row < M) | (row >= col)
        wo32 = wo_v.bitcast(_U32)

        def segment(h_in, h_out, dst, side_work, pre_rows):
            def proj(hd):
                h = h_in[...] if pre_rows is None else h_in[0:LA - PRE, :]
                dot = lambda t, k0, k1: lax.dot_general(
                    h[:, k0:k1], pltpu.bitcast(wf_v[t][pl.ds(head_row(hd) + k0 // 2, (k1 - k0) // 2), :], _BF16),
                    _NN, preferred_element_type=_F32)
                if hd == 0:
                    cut, part = Dm // 2, [acc_v.at[0:h.shape[0], t * Dh:(t + 1) * Dh] for t in range(3)]
                    for t in range(3):
                        part[t][...] = dot(t, 0, cut)
                    out = [part[t][...] + dot(t, cut, Dm) for t in range(3)]
                else:
                    out = [dot(t, 0, Dm) for t in range(3)]
                if pre_rows is not None:
                    out = [jnp.concatenate([out[t], zpre_v[hd % 2, t * HP + hd // 2, pre_rows, :]], axis=0) for t in range(3)]
                return out

            qkv, prob = {}, {}

            def scores(hd):
                q, k, _ = qkv[hd]
                sc = lax.dot_general(q, k, _NT, preferred_element_type=_F32) * scale
                sc = jnp.where(mask, sc, -1e9)
                p = jnp.exp(sc - jnp.max(sc, axis=-1, keepdims=True))
                prob[hd] = p / jnp.sum(p, axis=-1, keepdims=True)

            def values(hd):
                o_v[:, hd * Dh:(hd + 1) * Dh] = lax.dot_general(
                    prob[hd], qkv[hd][2], _NN, preferred_element_type=_F32)

            grp = 1 if pre_rows is None else 2
            todo_s, todo_v = list(range(H)), list(range(H))
            for hd in range(H):
                qkv[hd] = proj(hd)
                if hd % grp == 0:
                    while todo_s[0] < hd:
                        scores(todo_s.pop(0))
                    while todo_v[0] < hd - max(grp, 2):
                        values(todo_v.pop(0))
                if hd in side_work:
                    side_work[hd]()
            n1 = H - H // 4
            o = o_v[:, 0:n1 * Dh]
            for j in range(Dm // _LANES):
                w = pltpu.bitcast(wo32[j, 0:n1 * Dh // 2, :], _BF16)
                acc_v[:, j * _LANES:(j + 1) * _LANES] = lax.dot_general(o, w, _NN, preferred_element_type=_F32)
                while todo_s:
                    scores(todo_s.pop(0))
                for _ in range(grp if j >= 2 else 0):
                    if todo_v:
                        values(todo_v.pop(0))
            o = o_v[:, n1 * Dh:]
            for j in range(Dm // _LANES):
                cols = slice(j * _LANES, (j + 1) * _LANES)
                w = pltpu.bitcast(wo32[j, n1 * Dh // 2:, :], _BF16)
                res = lax.dot_general(o, w, _NN, preferred_element_type=_F32) + acc_v[:, cols]
                h_out[0:M, cols] = res[0:M]
                dst[:, cols] = res[M:].astype(_BF16)

        def out_cp(i):
            rows = pl.ds(pl.multiple_of(i * _T, _T), _T)
            return pltpu.make_async_copy(out_v.at[rows], out_hbm.at[rows], sem_out)

        def chunk(i, carry, ahead):
            rows = pl.ds(pl.multiple_of(i * _T, _T), _T)
            dst = out_v.at[rows]
            x_cp(i + 1).wait()

            def s4_epilogue(sb):
                y = ya_v[sb, pl.ds(i * SU, _CB), :].T
                for q in range(2):
                    cb = 2 * sb + q
                    skip = u_v[cb, rows, :].astype(_F32) * dk_v[cb][0:1, :]
                    dst[:, Dm + cb * _CB:Dm + (cb + 1) * _CB] = (y[q * _T:(q + 1) * _T] + skip).astype(_BF16)

            def next_rows(k):
                if k < SPC:
                    h_v[k][M:LA, :] = x_v[i & (XR - 1), k].astype(_F32)
                else:
                    h_v[0][M:LA, :] = x_v[(i + 1) & (XR - 1), 0].astype(_F32)

            def traffic():
                x_cp(i + XR - 1).start()

            for k in range(SPC):
                side = {H // 2: functools.partial(next_rows, k + 1)}
                if k == 0:
                    side[2] = traffic
                    for sb in range(NB):
                        side[4 + 2 * sb] = functools.partial(s4_epilogue, sb)
                pre_rows = pl.ds(pl.multiple_of((i * SPC + k) * PRE, PRE), PRE) if ahead else None
                segment(h_v[k], h_v[(k + 1) % SPC], dst.at[pl.ds(k * seg, seg)], side, pre_rows)
            out_cp(i).start()
            return carry

        pltpu.make_async_copy(wo_v, wo_v, sem_wo).wait()
        lax.fori_loop(0, NPRE, functools.partial(chunk, ahead=True), 0)
        lax.fori_loop(NPRE, NC, functools.partial(chunk, ahead=False), 0)

        for i in range(NC + 1, NC + XR - 1):
            x_cp(i).wait()
        pltpu.make_async_copy(out_v, out_hbm, sem_out).wait()

    scratch = [
        pltpu.VMEM((XR, SPC, seg, Dm), _BF16),
        pltpu.VMEM((NPRE * SPC, PRE, Dm), _BF16),
        pltpu.VMEM((NB, R, DC), _F32),
        pltpu.VMEM((2, 3 * HP, R, Dh), _F32),
        pltpu.VMEM((M, Dm), _BF16),
        pltpu.VMEM((3, Dm * H, Dh), _BF16),
        pltpu.VMEM((Dm // _LANES, H * Dh, _LANES), _BF16),
        pltpu.VMEM((2 * NB, L, _CB), _BF16),
        pltpu.VMEM((6, D, N), _BF16),
        pltpu.VMEM((D,), _BF16),
        pltpu.VMEM((D,), _BF16),
        pltpu.VMEM((2 * NB, 8, _CB), _F32),
        pltpu.VMEM((2 * NB, 8, _CB), _F32),
        pltpu.VMEM((NC * SU, _LANES), _F32),
        pltpu.VMEM((NC * SU, _LANES), _F32),
        pltpu.VMEM((NB, NC * SU, _LANES), _F32),
        pltpu.VMEM((2, NPOW * SU + 5, N), _F32),
        pltpu.VMEM((2, NPOW * SU + 5, N), _F32),
        pltpu.VMEM((6, 2, _CB, N), _F32),
        pltpu.VMEM((LA, H * Dh), _F32),
        pltpu.VMEM((LA, Dm), _F32),
        pltpu.VMEM((S, Dm + D), _BF16),
        pltpu.SemaphoreType.DMA((6 * NB,)),
        pltpu.SemaphoreType.DMA((4,)),
        pltpu.SemaphoreType.DMA((2 * NB,)),
        pltpu.SemaphoreType.DMA((3 * NB,)),
        pltpu.SemaphoreType.DMA(()),
        pltpu.SemaphoreType.DMA((XR,)),
        pltpu.SemaphoreType.DMA(()),
        pltpu.SemaphoreType.DMA(()),
    ]
    scratch += [pltpu.VMEM((LA, Dm), _F32)] * SPC
    scratch += [pltpu.VMEM((H * SW, Dh), _U32)] * 3
    scratch += [pltpu.VMEM((NC * SG, N), _F32)] * (4 * NG)
    return kernel, scratch


@functools.partial(jax.jit, static_argnames=("A_seg_len",))
def pallas_concat_heads__memory_aug_recurrent_mem_tr__ssm_conv_s4__prompt_kernel(
    A_x: jax.Array,
    A_mem0: jax.Array,
    A_Wq: jax.Array,
    A_Wk: jax.Array,
    A_Wv: jax.Array,
    A_Wo: jax.Array,
    A_seg_len: int,
    B_u: jax.Array,
    B_A_re: jax.Array,
    B_A_im: jax.Array,
    B_B_re: jax.Array,
    B_B_im: jax.Array,
    B_C_re: jax.Array,
    B_C_im: jax.Array,
    B_log_dt: jax.Array,
    B_Dskip: jax.Array,
):
    B, S, Dm = A_x.shape
    H, Dh = A_Wq.shape[1], A_Wq.shape[2]
    M = A_mem0.shape[1]
    seg = int(A_seg_len)
    _, L, D = B_u.shape
    N = B_A_re.shape[1]
    assert B == 1 and S == L and S % seg == 0 and Dh == _LANES and N == _LANES

    kernel, scratch = _make_kernel(S, Dm, H, Dh, M, seg, L, D, N)
    out = pl.pallas_call(
        kernel,
        out_shape=jax.ShapeDtypeStruct((S, Dm + D), _BF16),
        in_specs=[pl.BlockSpec(memory_space=pl.ANY)] * 15,
        out_specs=pl.BlockSpec(memory_space=pl.ANY),
        scratch_shapes=scratch,
        compiler_params=pltpu.CompilerParams(vmem_limit_bytes=120 * 1024 * 1024),
    )(
        A_x.reshape(S // seg, seg, Dm), A_mem0.reshape(M, Dm),
        A_Wq.reshape(Dm * H, Dh), A_Wk.reshape(Dm * H, Dh), A_Wv.reshape(Dm * H, Dh),
        A_Wo.reshape(H * Dh, Dm), B_u.reshape(L, D),
        B_A_re, B_A_im, B_B_re, B_B_im, B_C_re, B_C_im, B_log_dt, B_Dskip,
    )
    return out.reshape(B, S, Dm + D)
```

```python
import functools

import jax
import jax.numpy as jnp
from jax import lax
import jax.experimental.pallas as pl
import jax.experimental.pallas.tpu as pltpu

_NN = (((1,), (0,)), ((), ()))
_NT = (((1,), (1,)), ((), ()))
_LANES = 128
_T = 64
_CB = 128
_F32 = jnp.float32
_BF16 = jnp.bfloat16
_U32 = jnp.uint32


def _cmul(ar, ai, br, bi):
    return ar * br - ai * bi, ar * bi + ai * br


def _csqrt(x, y):
    big = jnp.sqrt(0.5 * (jnp.sqrt(x * x + y * y) + jnp.abs(x)))
    small = jnp.where(big > 0, 0.5 * y / big, 0.0)
    pos = x >= 0
    return jnp.where(pos, big, jnp.abs(small)), jnp.where(pos, small, jnp.where(y < 0, -big, big))


def _make_kernel(S, Dm, H, Dh, M, seg, L, D, N):
    LA = M + seg
    scale = Dh ** (-0.5)
    HP = H // 2
    NC = L // _T
    NB = D // (2 * _CB)
    NG = _CB // 8
    NPOW = 11
    SPC = _T // seg
    DC = Dm // NB
    WR = H * Dh // (2 * NB)
    XR = 4
    SG, SU, SW = 17, _CB + 1, Dm // 2 + 1
    PRE = 8
    NPRE = 8
    R = NPRE * SPC * PRE

    def head_row(hd):
        return ((hd % 2) * HP + hd // 2) * SW

    def kernel(x_hbm, mem0_hbm, wq_hbm, wk_hbm, wv_hbm, wo_hbm, u_hbm,
               are_hbm, aim_hbm, bre_hbm, bim_hbm, cre_hbm, cim_hbm, ldt_hbm, dsk_hbm,
               out_hbm,
               x_v, xpre_v, xb_v, zpre_v, mem0_v, wraw_v, wo_v, u_v, par_v, ldt_v, dsk_v, dt_v, dk_v,
               ut_v, yt_v, ya_v, pr_v, pi_v, aux_v,
               o_v, acc_v, out_v,
               sem_par, sem_misc, sem_u, sem_w, sem_wo, sem_x, sem_out, sem_y, *bufs):
        h_v, wf_v, st_v = bufs[:SPC], bufs[SPC:SPC + 3], bufs[SPC + 3:]
        par_hbm = (are_hbm, aim_hbm, bre_hbm, bim_hbm, cre_hbm, cim_hbm)
        vec_cp = [pltpu.make_async_copy(ldt_hbm, ldt_v, sem_misc.at[0]),
                  pltpu.make_async_copy(dsk_hbm, dsk_v, sem_misc.at[1])]
        mem_cp = pltpu.make_async_copy(mem0_hbm, mem0_v, sem_misc.at[2])

        def par_cp(sb):
            rows = pl.ds(pl.multiple_of(sb * 2 * _CB, 2 * _CB), 2 * _CB)
            return [pltpu.make_async_copy(par_hbm[i].at[rows], par_v.at[i, rows], sem_par.at[sb * 6 + i])
                    for i in range(6)]

        w_hbm = (wq_hbm, wk_hbm, wv_hbm)

        def u_cp(cb):
            return pltpu.make_async_copy(
                u_hbm.at[:, pl.ds(pl.multiple_of(cb * _CB, _CB), _CB)], u_v.at[cb], sem_u.at[cb])

        def w_cp(t, cb):
            rows = pl.ds(pl.multiple_of(cb * (DC * H), DC * H), DC * H)
            return pltpu.make_async_copy(w_hbm[t].at[rows], wraw_v.at[t, rows], sem_w.at[t * NB + cb])

        def wo_start(r):
            rows = pl.ds(r * WR if isinstance(r, int) else pl.multiple_of(r * WR, WR), WR)
            for j in range(Dm // _LANES):
                pltpu.make_async_copy(wo_hbm.at[rows, pl.ds(j * _LANES, _LANES)], wo_v.at[j, rows], sem_wo).start()

        def y_cp(sb):
            return pltpu.make_async_copy(yt_v, ya_v.at[sb], sem_y)

        def x_cp(i):
            src = pl.ds(jnp.minimum(i, NC - 1) * SPC, SPC)
            return pltpu.make_async_copy(x_hbm.at[src], x_v.at[i & (XR - 1)], sem_x.at[i & (XR - 1)])

        xpre_cp = pltpu.make_async_copy(
            x_hbm.at[pl.ds(0, NPRE * SPC), pl.ds(seg - PRE, PRE)], xpre_v, sem_misc.at[3])

        for cp in par_cp(0) + vec_cp:
            cp.start()
        u_cp(0).start()
        u_cp(1).start()
        zpre_v[...] = jnp.zeros(zpre_v.shape, _F32)
        for cp in par_cp(0) + vec_cp:
            cp.wait()
        xpre_cp.start()

        dt_all = jnp.exp(ldt_v[...].astype(_F32)).astype(_BF16).astype(_F32).reshape(1, D)
        dk_all = dsk_v[...].astype(_F32).reshape(1, D)
        for cb in range(2 * NB):
            dt_v[cb] = jnp.broadcast_to(dt_all[:, cb * _CB:(cb + 1) * _CB], (8, _CB))
            dk_v[cb] = jnp.broadcast_to(dk_all[:, cb * _CB:(cb + 1) * _CB], (8, _CB))

        flip8 = 7 - lax.broadcasted_iota(jnp.int32, (8, _LANES), 0)
        lane8 = lax.broadcasted_iota(jnp.int32, (8, _LANES), 1)
        sub8 = lax.broadcasted_iota(jnp.int32, (8, _LANES), 0)
        lo_c = lax.broadcasted_iota(jnp.int32, (NC, _LANES), 1) < _T
        first_c = lax.broadcasted_iota(jnp.int32, (NC, _LANES), 0) == 0
        raw32 = wraw_v.bitcast(_U32)
        s_buf = [(st_v[4 * i], st_v[4 * i + 1]) for i in range(NG)]
        z_buf = [(st_v[4 * i + 2], st_v[4 * i + 3]) for i in range(NG)]

        def discretise(sb, g):
            hf = g // (_CB // 16)
            g16 = (g % (_CB // 16)) * 16
            r = pl.ds(pl.multiple_of(g16, 16), 16)
            rg = pl.ds(pl.multiple_of(sb * 2 * _CB + g * 16, 16), 16)
            dt = aux_v[0, hf, r, :]
            a = dt * par_v[0, rg, :].astype(_F32)
            b = dt * par_v[1, rg, :].astype(_F32)
            mag = jnp.exp(a)
            l1 = (mag * jnp.cos(b), mag * jnp.sin(b))
            w = _cmul(par_v[4, rg, :].astype(_F32), par_v[5, rg, :].astype(_F32),
                      dt * par_v[2, rg, :].astype(_F32), dt * par_v[3, rg, :].astype(_F32))
            l2 = _cmul(*l1, *l1)
            l4 = _cmul(*l2, *l2)
            l8 = _cmul(*l4, *l4)
            l16 = _cmul(*l8, *l8)
            l32 = _cmul(*l16, *l16)
            l64 = _cmul(*l32, *l32)
            pw = [_csqrt(*_cmul(*w, *l1))]
            pw.append(_cmul(*pw[0], *l1))
            pw += [_cmul(*q, *l2) for q in pw]
            pw += [_cmul(*q, *l4) for q in pw]
            pw += [l8, l16, l32]
            for j in range(NPOW):
                pr_v[hf, pl.ds(j * SU + g16, 16), :] = pw[j][0]
                pi_v[hf, pl.ds(j * SU + g16, 16), :] = pw[j][1]
            aux_v[1, hf, r, :] = l64[0]
            aux_v[2, hf, r, :] = l64[1]
            aux_v[3, hf, r, :] = jnp.broadcast_to(jnp.sum(w[0], axis=-1, keepdims=True), (16, N))
            aux_v[4, hf, r, :] = pw[0][0]
            aux_v[5, hf, r, :] = -pw[0][1]

        def load_u(sb, ck):
            rows = pl.ds(pl.multiple_of(ck * _T, _T), _T)
            fl = []
            for q in range(2):
                tile = u_v[2 * sb + q, rows, :].astype(_F32)
                fl += [jnp.take_along_axis(tile[_T - 8 * (i + 1):_T - 8 * i], flip8, axis=0)
                       for i in range(_T // 8)]
            ut_v[pl.ds(ck * SU, _CB), :] = jnp.concatenate(fl, axis=0).T

        def repack(c):
            nj = DC // 2 // 4

            def body(i, carry):
                j0 = c * (DC // 2) + i * nj
                for t in range(3):
                    src = raw32.at[t, pl.ds(pl.multiple_of(j0 * H, nj * H), nj * H), :]
                    for j in range(nj):
                        for half in range(HP // 8):
                            a = src[pl.ds(j * H + half * 8, 8), :]
                            b = src[pl.ds(j * H + HP + half * 8, 8), :]
                            wf_v[t][pl.ds(j0 + (half * 8 * SW + j), 8, stride=SW), :] = (a & _U32(0xFFFF)) | (b << 16)
                            wf_v[t][pl.ds(j0 + ((HP + half * 8) * SW + j), 8, stride=SW), :] = (
                                (a >> 16) | (b & _U32(0xFFFF0000)))
                return carry
            lax.fori_loop(0, 4, body, 0)

        def project_ahead(c, par):
            lhs = xb_v[c]
            r0 = par * (HP * SW) + c * (DC // 2)
            for t in range(3):
                for k in range(HP):
                    w = wf_v[t][pl.ds(r0 + k * SW, DC // 2), :]
                    zpre_v[par, t * HP + k] += lax.dot_general(
                        lhs, pltpu.bitcast(w, _BF16), _NN, preferred_element_type=_F32)

        def states(p):
            vr, vi = [], []
            for hf in range(2):
                ar = [pr_v[hf, pl.ds(p, 8, stride=SU), :]]
                ai = [pi_v[hf, pl.ds(p, 8, stride=SU), :]]
                for lvl in range(3):
                    mr = jnp.broadcast_to(pr_v[hf, pl.ds((8 + lvl) * SU + p, 1), :], (8, N))
                    mi = jnp.broadcast_to(pi_v[hf, pl.ds((8 + lvl) * SU + p, 1), :], (8, N))
                    for i in range(len(ar)):
                        nr, ni = _cmul(ar[i], ai[i], mr, mi)
                        ar.append(nr)
                        ai.append(ni)
                vr += ar
                vi += ai
            v = jnp.concatenate(
                [jnp.concatenate(vr, axis=0), jnp.concatenate(vi, axis=0)], axis=1).astype(_BF16)
            uf = ut_v[pl.ds(p, NC, stride=SU), :]
            lhs = jnp.concatenate([jnp.where(lo_c, uf, 0.0), jnp.where(lo_c, 0.0, uf)], axis=0)
            st = lax.dot_general(lhs, v, _NN, preferred_element_type=_F32)
            sr, si = s_buf[p // 8]
            for hf in range(2):
                rows = pl.ds(hf * 8 + p % 8, NC, stride=SG)
                sr[rows, :] = st[hf * NC:(hf + 1) * NC, :N]
                si[rows, :] = st[hf * NC:(hf + 1) * NC, N:]
            return v

        def scan(g):
            sr, si = s_buf[g]
            zr, zi = z_buf[g]
            cat = lambda i: jnp.concatenate([aux_v[i, hf, g * 8:(g + 1) * 8, :] for hf in range(2)], axis=0)
            lr, li = cat(1), cat(2)
            zr[0:16, :] = cat(4)
            zi[0:16, :] = cat(5)
            for c in range(1, NC):
                s_r = sr[pl.ds((c - 1) * SG, 16), :]
                s_i = si[pl.ds((c - 1) * SG, 16), :]
                if c == 1:
                    xr, xi = s_r, -s_i
                else:
                    xr, xi = (xr * lr + s_r) + xi * li, (xi * lr - s_i) - xr * li
                zr[pl.ds(c * SG, 16), :] = xr
                zi[pl.ds(c * SG, 16), :] = xi

        def inter(p, v):
            z = [jnp.concatenate([zb[pl.ds(hf * 8 + p % 8, NC, stride=SG), :] for hf in range(2)], axis=0)
                 for zb in z_buf[p // 8]]
            y = lax.dot_general(jnp.concatenate(z, axis=1), v, _NT, preferred_element_type=_F32)
            return jnp.where(lo_c, y[:NC], y[NC:])

        def intra(p, y):
            kk = jnp.broadcast_to(y[0:1, :], (8, _LANES))
            g1 = pltpu.roll(kk, 1, 1, stride=1, stride_axis=0)
            g1 = jnp.where((lane8 & (_T - 1)) > sub8, g1, 0.0)
            g1 = jnp.take_along_axis(g1, flip8, axis=0)
            g0 = jnp.where((lane8 & (_T - 1)) >= 8, pltpu.roll(g1, 8, 1), 0.0)
            top = pltpu.bitcast(jnp.concatenate([g0, g1], axis=0).astype(_BF16), _U32)
            gs = [(i, pltpu.roll(top, 16 * i, 1) if i else top) for i in range(_T // 16 - 1, -1, -1)]
            hs = [jnp.where((lane8 >= 16 * i) & (lane8 < _T), gv, _U32(0)) for i, gv in gs]
            hs += [jnp.where(lane8 >= _T + 16 * i, gv, _U32(0)) for i, gv in gs]
            hk = pltpu.bitcast(jnp.concatenate(hs, axis=0), _BF16)
            rows = pl.ds(p, NC, stride=SU)
            yd = lax.dot_general(ut_v[rows, :], hk, _NN, preferred_element_type=_F32)
            yt_v[rows, :] = jnp.where(first_c, 0.0, y) + yd

        def block(sb, carry):
            @pl.when(sb > 0)
            def _():
                for t in range(3):
                    w_cp(t, sb - 1).wait()

            for t in range(3):
                w_cp(t, sb).start()

            @pl.when(sb < NB - 1)
            def _():
                for cp in par_cp(sb + 1) + [u_cp(2 * sb + 2), u_cp(2 * sb + 3)]:
                    cp.start()

            @pl.when(sb == NB - 1)
            def _():
                for cp in [mem_cp] + [x_cp(i) for i in range(XR - 1)]:
                    cp.start()

            for hf in range(2):
                aux_v[0, hf] = jnp.broadcast_to(dt_v[2 * sb + hf][0:1, :], (_CB, _CB)).T

            @pl.when(sb == 0)
            def _():
                def modes(i, c, with_u):
                    for k in range(4):
                        discretise(0, i * 4 + k)
                    for k in range(NC // 2 if with_u else 0):
                        load_u(0, (i - 2) * (NC // 2) + k)
                    return c
                lax.fori_loop(0, 2, functools.partial(modes, with_u=False), 0)
                u_cp(0).wait()
                u_cp(1).wait()
                lax.fori_loop(2, 4, functools.partial(modes, with_u=True), 0)
                xpre_cp.wait()
                xpre = xpre_v[...].astype(_F32).reshape(R, Dm)
                for c in range(NB):
                    xb_v[c] = xpre[:, c * DC:(c + 1) * DC]

            @pl.when(sb > 0)
            def _():
                repack(sb - 1)
                for cp in par_cp(sb) + [u_cp(2 * sb), u_cp(2 * sb + 1)]:
                    cp.wait()

                def prepare(i, c):
                    for k in range(_CB // 16):
                        discretise(sb, i * (_CB // 16) + k)
                    for k in range(NC // 2):
                        load_u(sb, i * (NC // 2) + k)
                    project_ahead(sb - 1, i)
                    return c
                lax.fori_loop(0, 2, prepare, 0)

            for hf in range(2):
                dk_v[2 * sb + hf] = dk_v[2 * sb + hf] + aux_v[3, hf].T[0:8]

            vs, ys = {}, {}
            for p in range(_CB):
                vs[p] = states(p)
                if p == 7:
                    scan(0)

            @pl.when(sb > 0)
            def _():
                y_cp(sb - 1).wait()
                wo_start(2 * sb - 1)

            wo_start(2 * sb)

            @pl.when(sb == NB - 1)
            def _():
                wo_start(2 * NB - 1)

            for g in range(NG):
                if g + 1 < NG:
                    scan(g + 1)
                for p in range(g * 8, (g + 1) * 8):
                    ys[p] = inter(p, vs.pop(p))
            for p in range(_CB):
                intra(p, ys.pop(p))
            y_cp(sb).start()
            return carry
        lax.fori_loop(0, NB, block, 0)
        for t in range(3):
            w_cp(t, NB - 1).wait()
        repack(NB - 1)
        lax.fori_loop(0, 2, lambda i, c: project_ahead(NB - 1, i), None)

        mem_cp.wait()
        y_cp(NB - 1).wait()
        x_cp(0).wait()
        h_v[0][0:M, :] = mem0_v[...].astype(_F32)
        h_v[0][M:LA, :] = x_v[0, 0].astype(_F32)
        row = lax.broadcasted_iota(jnp.int32, (LA, LA), 0)
        col = lax.broadcasted_iota(jnp.int32, (LA, LA), 1)
        mask = (row < M) | (row >= col)
        wo32 = wo_v.bitcast(_U32)

        def segment(h_in, h_out, dst, side_work, pre_rows):
            def proj(hd):
                h = h_in[...] if pre_rows is None else h_in[0:LA - PRE, :]
                dot = lambda t, k0, k1: lax.dot_general(
                    h[:, k0:k1], pltpu.bitcast(wf_v[t][pl.ds(head_row(hd) + k0 // 2, (k1 - k0) // 2), :], _BF16),
                    _NN, preferred_element_type=_F32)
                if hd == 0:
                    cut, part = Dm // 2, [acc_v.at[0:h.shape[0], t * Dh:(t + 1) * Dh] for t in range(3)]
                    for t in range(3):
                        part[t][...] = dot(t, 0, cut)
                    out = [part[t][...] + dot(t, cut, Dm) for t in range(3)]
                else:
                    out = [dot(t, 0, Dm) for t in range(3)]
                if pre_rows is not None:
                    out = [jnp.concatenate([out[t], zpre_v[hd % 2, t * HP + hd // 2, pre_rows, :]], axis=0)
                           for t in range(3)]
                return out

            qkv, prob = {}, {}

            def scores(hd):
                q, k, _ = qkv[hd]
                sc = lax.dot_general(q, k, _NT, preferred_element_type=_F32) * scale
                sc = jnp.where(mask, sc, -1e9)
                p = jnp.exp(sc - jnp.max(sc, axis=-1, keepdims=True))
                prob[hd] = p / jnp.sum(p, axis=-1, keepdims=True)

            def values(hd):
                o_v[:, hd * Dh:(hd + 1) * Dh] = lax.dot_general(
                    prob[hd], qkv[hd][2], _NN, preferred_element_type=_F32)

            grp = 1 if pre_rows is None else 2
            todo_s, todo_v = list(range(H)), list(range(H))
            for hd in range(H):
                qkv[hd] = proj(hd)
                if hd % grp == 0:
                    while todo_s[0] < hd:
                        scores(todo_s.pop(0))
                    while todo_v[0] < hd - max(grp, 2):
                        values(todo_v.pop(0))
                if hd in side_work:
                    side_work[hd]()
            n1 = H - H // 4
            o = o_v[:, 0:n1 * Dh]
            for j in range(Dm // _LANES):
                w = pltpu.bitcast(wo32[j, 0:n1 * Dh // 2, :], _BF16)
                acc_v[:, j * _LANES:(j + 1) * _LANES] = lax.dot_general(o, w, _NN, preferred_element_type=_F32)
                while todo_s:
                    scores(todo_s.pop(0))
                for _ in range(grp if j >= 2 else 0):
                    if todo_v:
                        values(todo_v.pop(0))
            o = o_v[:, n1 * Dh:]
            for j in range(Dm // _LANES):
                cols = slice(j * _LANES, (j + 1) * _LANES)
                w = pltpu.bitcast(wo32[j, n1 * Dh // 2:, :], _BF16)
                res = lax.dot_general(o, w, _NN, preferred_element_type=_F32) + acc_v[:, cols]
                h_out[0:M, cols] = res[0:M]
                dst[:, cols] = res[M:].astype(_BF16)

        def out_cp(i):
            rows = pl.ds(pl.multiple_of(i * _T, _T), _T)
            return pltpu.make_async_copy(out_v.at[rows], out_hbm.at[rows], sem_out)

        def chunk(i, carry, ahead):
            rows = pl.ds(pl.multiple_of(i * _T, _T), _T)
            dst = out_v.at[rows]
            x_cp(i + 1).wait()

            def s4_epilogue(sb):
                y = ya_v[sb, pl.ds(i * SU, _CB), :].T
                for q in range(2):
                    cb = 2 * sb + q
                    skip = u_v[cb, rows, :].astype(_F32) * dk_v[cb][0:1, :]
                    dst[:, Dm + cb * _CB:Dm + (cb + 1) * _CB] = (y[q * _T:(q + 1) * _T] + skip).astype(_BF16)

            def next_rows(k):
                if k < SPC:
                    h_v[k][M:LA, :] = x_v[i & (XR - 1), k].astype(_F32)
                else:
                    h_v[0][M:LA, :] = x_v[(i + 1) & (XR - 1), 0].astype(_F32)

            for k in range(SPC):
                side = {H // 2: functools.partial(next_rows, k + 1)}
                if k == 0:
                    side[2] = x_cp(i + XR - 1).start
                    for sb in range(NB):
                        side[4 + 2 * sb] = functools.partial(s4_epilogue, sb)
                pre_rows = pl.ds(pl.multiple_of((i * SPC + k) * PRE, PRE), PRE) if ahead else None
                segment(h_v[k], h_v[(k + 1) % SPC], dst.at[pl.ds(k * seg, seg)], side, pre_rows)
            out_cp(i).start()
            return carry

        pltpu.make_async_copy(wo_v, wo_v, sem_wo).wait()
        lax.fori_loop(0, NPRE, functools.partial(chunk, ahead=True), 0)
        lax.fori_loop(NPRE, NC, functools.partial(chunk, ahead=False), 0)

        for i in range(NC + 1, NC + XR - 1):
            x_cp(i).wait()
        pltpu.make_async_copy(out_v, out_hbm, sem_out).wait()

    scratch = [
        pltpu.VMEM((XR, SPC, seg, Dm), _BF16),
        pltpu.VMEM((NPRE * SPC, PRE, Dm), _BF16),
        pltpu.VMEM((NB, R, DC), _F32),
        pltpu.VMEM((2, 3 * HP, R, Dh), _F32),
        pltpu.VMEM((M, Dm), _BF16),
        pltpu.VMEM((3, Dm * H, Dh), _BF16),
        pltpu.VMEM((Dm // _LANES, H * Dh, _LANES), _BF16),
        pltpu.VMEM((2 * NB, L, _CB), _BF16),
        pltpu.VMEM((6, D, N), _BF16),
        pltpu.VMEM((D,), _BF16),
        pltpu.VMEM((D,), _BF16),
        pltpu.VMEM((2 * NB, 8, _CB), _F32),
        pltpu.VMEM((2 * NB, 8, _CB), _F32),
        pltpu.VMEM((NC * SU, _LANES), _F32),
        pltpu.VMEM((NC * SU, _LANES), _F32),
        pltpu.VMEM((NB, NC * SU, _LANES), _F32),
        pltpu.VMEM((2, NPOW * SU + 5, N), _F32),
        pltpu.VMEM((2, NPOW * SU + 5, N), _F32),
        pltpu.VMEM((6, 2, _CB, N), _F32),
        pltpu.VMEM((LA, H * Dh), _F32),
        pltpu.VMEM((LA, Dm), _F32),
        pltpu.VMEM((S, Dm + D), _BF16),
        pltpu.SemaphoreType.DMA((6 * NB,)),
        pltpu.SemaphoreType.DMA((4,)),
        pltpu.SemaphoreType.DMA((2 * NB,)),
        pltpu.SemaphoreType.DMA((3 * NB,)),
        pltpu.SemaphoreType.DMA(()),
        pltpu.SemaphoreType.DMA((XR,)),
        pltpu.SemaphoreType.DMA(()),
        pltpu.SemaphoreType.DMA(()),
    ]
    scratch += [pltpu.VMEM((LA, Dm), _F32)] * SPC
    scratch += [pltpu.VMEM((H * SW, Dh), _U32)] * 3
    scratch += [pltpu.VMEM((NC * SG, N), _F32)] * (4 * NG)
    return kernel, scratch


@functools.partial(jax.jit, static_argnames=("A_seg_len",))
def pallas_concat_heads__memory_aug_recurrent_mem_tr__ssm_conv_s4__prompt_kernel(
    A_x: jax.Array,
    A_mem0: jax.Array,
    A_Wq: jax.Array,
    A_Wk: jax.Array,
    A_Wv: jax.Array,
    A_Wo: jax.Array,
    A_seg_len: int,
    B_u: jax.Array,
    B_A_re: jax.Array,
    B_A_im: jax.Array,
    B_B_re: jax.Array,
    B_B_im: jax.Array,
    B_C_re: jax.Array,
    B_C_im: jax.Array,
    B_log_dt: jax.Array,
    B_Dskip: jax.Array,
):
    B, S, Dm = A_x.shape
    H, Dh = A_Wq.shape[1], A_Wq.shape[2]
    M = A_mem0.shape[1]
    seg = int(A_seg_len)
    _, L, D = B_u.shape
    N = B_A_re.shape[1]
    assert B == 1 and S == L and Dh == N == _LANES and H % 16 == 0
    assert seg % 16 == 0 and _T % seg == 0 and M % 8 == 0 and D % (4 * _CB) == 0 and L % (2 * _T) == 0

    kernel, scratch = _make_kernel(S, Dm, H, Dh, M, seg, L, D, N)
    out = pl.pallas_call(
        kernel,
        out_shape=jax.ShapeDtypeStruct((S, Dm + D), _BF16),
        in_specs=[pl.BlockSpec(memory_space=pl.ANY)] * 15,
        out_specs=pl.BlockSpec(memory_space=pl.ANY),
        scratch_shapes=scratch,
        compiler_params=pltpu.CompilerParams(vmem_limit_bytes=120 * 1024 * 1024),
    )(
        A_x.reshape(S // seg, seg, Dm), A_mem0.reshape(M, Dm),
        A_Wq.reshape(Dm * H, Dh), A_Wk.reshape(Dm * H, Dh), A_Wv.reshape(Dm * H, Dh),
        A_Wo.reshape(H * Dh, Dm), B_u.reshape(L, D),
        B_A_re, B_A_im, B_B_re, B_B_im, B_C_re, B_C_im, B_log_dt, B_Dskip,
    )
    return out.reshape(B, S, Dm + D)
```
